```python
import jax
import jax.numpy as jnp

def _softmax(x, axis=-1):
    return jax.nn.softmax(x, axis=axis)
def _gelu(x):
    return jax.nn.gelu(x, approximate=True)
def _silu(x):
    return jax.nn.silu(x)
def _sigmoid(x):
    return jax.nn.sigmoid(x)
def _layernorm(x, axis=-1, eps=1e-5):
    m = jnp.mean(x, axis=axis, keepdims=True)
    v = jnp.var(x, axis=axis, keepdims=True)
    return (x - m) / jnp.sqrt(v + eps)
def _scatter_add(tgt, idx, src, axis=0):
    return tgt.at[idx].add(src)
def _segment_sum(src, seg, n):
    return jax.ops.segment_sum(src, seg, n)
class _Rng:
    def __init__(self, key):
        self._k = key
    def _next(self):
        self._k, sub = jax.random.split(self._k)
        return sub
    def normal(self, shape):
        return jax.random.normal(self._next(), shape, dtype=jnp.bfloat16)
    def randint(self, lo, hi, shape):
        return jax.random.randint(self._next(), shape, lo, hi, dtype=jnp.int32)
    def uniform(self, shape, lo=0.0, hi=1.0):
        return jax.random.uniform(self._next(), shape, jnp.bfloat16, lo, hi)
    def permutation(self, n):
        return jax.random.permutation(self._next(), n)


kernel_name = 'parallel_sum__sliding_local_dilated__glu_gated_bilinear__prompt'

def setup_inputs():
    _rng = _Rng(jax.random.key(int.from_bytes(__import__("os").urandom(4), "little")))
    _w = (lambda a: (lambda t: t.astype(jnp.bfloat16) if jnp.issubdtype(t.dtype, jnp.floating) else t)(jnp.asarray(a)))
    def _A_setup():
        B, S, D = 1, 2048, 1024
        return {
            "x": _w((lambda *s: _rng.normal(s) * 0.05)(B, S, D)),
            "wqkv": _w((lambda *s: _rng.normal(s) * 0.05)(D, 3 * D)),
            "wo": _w((lambda *s: _rng.normal(s) * 0.05)(D, D)),
        }
    _A_in = _A_setup()

    def _B_setup():
        B, S, D, F = 1, 2048, 1024, 3584
        return {
            "x": _w((lambda *s: _rng.normal(s) * 0.05)(B, S, D)),
            "w_gate": _w((lambda *s: _rng.normal(s) * 0.05)(D, F) * (D ** -0.5)),
            "w_up": _w((lambda *s: _rng.normal(s) * 0.05)(D, F) * (D ** -0.5)),
            "w_down": _w((lambda *s: _rng.normal(s) * 0.05)(F, D) * (F ** -0.5)),
        }
    _B_in = _B_setup()

    return {
        "A_x": _A_in["x"],
        "A_wqkv": _A_in["wqkv"],
        "A_wo": _A_in["wo"],
        "B_x": _B_in["x"],
        "B_w_gate": _B_in["w_gate"],
        "B_w_up": _B_in["w_up"],
        "B_w_down": _B_in["w_down"],
    }

def reference(A_x, A_wqkv, A_wo, B_x, B_w_gate, B_w_up, B_w_down):
    def _A_ref(x, wqkv, wo):
        B, S, D = x.shape
        H = 32; Dh = D // H
        W, dil = 8, 2
        qkv = (lambda x, *d: x.transpose(*d))((x @ wqkv).reshape(B, S, 3, H, Dh), 2, 0, 3, 1, 4)
        q, k, v = qkv[0], qkv[1], qkv[2]
        scale = Dh ** -0.5
        pos = jnp.arange(S)
        off = jnp.arange(W) * dil
        idx = pos[:, None] - off[None, :]
        mask = idx >= 0
        idx_c = jnp.where(mask, idx, 0).reshape(-1)
        kg = k[:, :, idx_c, :].reshape(B, H, S, W, Dh)
        vg = v[:, :, idx_c, :].reshape(B, H, S, W, Dh)
        logits = jnp.einsum("bhsd,bhswd->bhsw", q, kg) * scale
        logits = jnp.where(mask[None, None, :, :], logits, -1e9)
        attn = _softmax(logits, axis=-1)
        o = jnp.einsum("bhsw,bhswd->bhsd", attn, vg)
        return (lambda x, *d: x.transpose(*d))(o, 0, 2, 1, 3).reshape(B, S, D) @ wo

    def _B_ref(x, w_gate, w_up, w_down):
        g = jnp.einsum("bsd,df->bsf", x, w_gate)
        u = jnp.einsum("bsd,df->bsf", x, w_up)
        h = g * u
        return jnp.einsum("bsf,fd->bsd", h, w_down)

    x = A_x
    xn = _layernorm(x, axis=-1)
    return x + _A_ref(xn, A_wqkv, A_wo) + _B_ref(xn, B_w_gate, B_w_up, B_w_down)
```

```python
import functools
import jax
import jax.numpy as jnp
from jax import lax
import jax.experimental.pallas as pl
import jax.experimental.pallas.tpu as pltpu

H, WIN, DIL = 32, 8, 2
TM = 1024
RG = 16
AG = 8
HIST = 16
PITCH = 33
STEPS = 8
SKIP = ''
AP, RB, KSPLIT = 2, 4, (4,)
SPAN_H = (0, 46, 5)
SPAN_A = ((0, 50, 5), (6, 64, 8), (14, 72, 6), (30, 80, 5), (50, 92, 5))
SPAN_L = ((0, 68, 4), (6, 74, 4), (12, 80, 3), (26, 94, 3))
LAG_T, LAG_W = (2, 2), (5, 5)
FLAGS = None
LAST_T = 13.9
F32, BF16 = jnp.float32, jnp.bfloat16
NN = (((1,), (0,)), ((), ()))
NT = (((1,), (1,)), ((), ()))

L_TERMS = (((0, 0), (1, 1), 1), ((1, 0), (1, 1), 1), ((0, 0),), ((1, 1),),
           ((0, 0), (0, 1), 1), ((1, 0), (0, 0), -1), ((0, 1), (1, 1), -1))
R_TERMS = (((0, 0), (1, 1), 1), ((0, 0),), ((0, 1), (1, 1), -1), ((1, 0), (0, 0), -1),
           ((1, 1),), ((0, 0), (0, 1), 1), ((1, 0), (1, 1), 1))
ORDER = (1, 3, 4, 2, 0, 6, 5)


def _comb(term, get):
    if len(term) == 1:
        return get(*term[0])
    a, b = get(*term[0]), get(*term[1])
    return a + b if term[2] > 0 else a - b


def _tree(f, xs):
    return xs[0] if len(xs) == 1 else f(_tree(f, xs[:len(xs) // 2]), _tree(f, xs[len(xs) // 2:]))


class _Shadow:
    def __init__(self):
        self.calls, self.tasks, self.zeros, self.late = 0, [], {}, []

    def add(self, fns, first, last, lag, gates, pin):
        for n, fn in enumerate(fns):
            self.tasks.append((first + n * (last - first) / len(fns), fn, lag, gates, pin))
        self.tasks.sort(key=lambda task: task[0])

    def dot(self, a, b, dims=NN):
        self.late += self.zeros.pop(self.calls, [])
        if self.late and b.dtype == F32:
            r0, c = b.shape[0] - 128, b.shape[1] - 128
            rows = [b[r:r + 8] for r in range(r0, r0 + 128, 8)]
            for step, zero in self.late:
                w = rows[14 - 2 * step]
                rows[14 - 2 * step] = jnp.concatenate([w[:, :c], w[:, c:] + zero], axis=1) if c else w + zero
            self.late = []
            b = jnp.concatenate(([b[:r0]] if r0 else []) + rows, axis=0)
        out = lax.dot_general(a, b.astype(BF16), dims, preferred_element_type=F32)
        events = []
        while self.tasks and self.tasks[0][0] < self.calls + 1:
            events.append(self.tasks.pop(0))
        for step in range(STEPS):
            group = [task for task in events if int((task[0] - self.calls) * STEPS) == step]
            row = step * out.shape[0] // STEPS
            for gate in {gate: None for task in group for gate in task[3]}:
                gate(out[row:row + 8])
            for task in group:
                task[1]()
            for lag, pin in {(task[2], task[4]): None for task in group}:
                self.zeros.setdefault(self.calls + lag, []).append((step, pin()))
        self.calls += 1
        return out

    def finish(self):
        assert not self.tasks


def _level(prod, tmp, emit, keep=None):
    tmp[0] = prod(1)
    c21 = tmp[0] + prod(3)
    emit(1, 0, c21)
    if keep is None:
        tmp[3] = c21
    tmp[1] = prod(4)
    c12 = tmp[1] + prod(2)
    emit(0, 1, c12)
    if keep is None:
        tmp[4] = c12
    tmp[2] = prod(0) - tmp[0] - tmp[1]
    emit(0, 0, (tmp[3] if keep is None else keep[2]) + tmp[2] + prod(6))
    emit(1, 1, (tmp[4] if keep is None else keep[1]) + tmp[2] + prod(5))


def _strassen2(prod, t2, t1, emit):
    def run(p, e, keep=None):
        _level(lambda q: prod(7 * p + q), t2, e, keep)

    def put(i):
        def f(r, c, v):
            t1[4 * i + 2 * r + c] = v
        return f
    get = lambda i, r, c: t1[4 * i + 2 * r + c]

    def c21(r, c, v):
        v = get(0, r, c) + v
        put(3)(r, c, v)
        emit(2 + r, c, v, t1.at[12 + 2 * r + c])

    def c12(r, c, v):
        v = get(1, r, c) + v
        put(4)(r, c, v)
        emit(r, 2 + c, v, t1.at[16 + 2 * r + c])
    run(1, put(0), t1.at[0:4])
    run(3, c21)
    run(4, put(1), t1.at[4:8])
    run(2, c12)
    run(0, lambda r, c, v: put(2)(r, c, v - get(0, r, c) - get(1, r, c)))
    run(6, lambda r, c, v: emit(r, c, get(3, r, c) + get(2, r, c) + v, None))
    run(5, lambda r, c, v: emit(2 + r, 2 + c, get(4, r, c) + get(2, r, c) + v, None))


def _rhs2(w, b1, slot=0):
    slots = {}

    def get(n):
        p, q = divmod(n, 7)
        if len(R_TERMS[p]) == 1:
            a, b = R_TERMS[p][0]
            dtype = BF16 if len(R_TERMS[q]) == 1 else F32
            return _comb(R_TERMS[q], lambda r, c: w(2 * a + r, 2 * b + c, dtype))
        if p not in slots:
            slots[p] = 4 * ((slot + len(slots)) % 2)
            for r in range(2):
                for c in range(2):
                    b1[slots[p] + 2 * r + c] = _comb(R_TERMS[p], lambda a, b: w(2 * a + r, 2 * b + c, F32))
        return _comb(R_TERMS[q], lambda r, c: b1[slots[p] + 2 * r + c])
    return get


def _lhs2(blk, p):
    l1 = {(r, c): _comb(L_TERMS[p], lambda a, b: blk(2 * a + r, 2 * b + c)) for r in range(2) for c in range(2)}
    return l1, [_comb(L_TERMS[q], lambda r, c: l1[r, c]).astype(BF16) for q in range(7)]


def _kernel(x_hbm, wqkv_hbm, wo_hbm, wg_hbm, wu_hbm, wd_hbm, o_hbm,
            x_v, out_v, w_v, wa_v, wt_v, wo_v, wd_v, tr_v, xa1_v, xa2_v, ha_v, qk_v, v_v, o_v,
            hh_v, t2_v, t3_v, tg_v, tu_v, b1_v, b1t_v, b1d_v, s1_v, s2_v, s3_v, s4_v, m1_v, m2_v, opaque, sem_in, sem_out):
    S, D = x_hbm.shape[0] * TM, x_hbm.shape[-1]
    F = wg_hbm.shape[1]
    NTILE, NB, DH, NQ = S // TM, D // 128, D // H, F // 512
    M, KQ = TM // 4, D // 4
    MH = M // 2
    AROWS = pl.cdiv(M // AG, NQ) * AG
    W_G, W_U, W_QKV, W_O = 0, NQ, 2 * NQ, 2 * NQ + 6
    al = pl.multiple_of
    lanes = lambda n: slice(n * 128, (n + 1) * 128)

    def slab_copy(src, base, s):
        dst = w_v.at[base + s] if base < W_QKV else wa_v.at[base - W_QKV + s]
        return pltpu.make_async_copy(src.at[:, pl.ds(al(s * 512, 512), 512)], dst, sem_in.at[base + s])

    def wd_copy(j):
        return pltpu.make_async_copy(wd_hbm.at[:, :, pl.ds(j * 512, 512)], wd_v.at[j], sem_in.at[W_O + 2 + j])

    def x_copy(i, j):
        rows = pl.ds(al(j * MH, MH), MH)
        return pltpu.make_async_copy(x_hbm.at[i, :, rows], x_v.at[pl.ds(4 * i, 4), rows],
                                     sem_in.at[W_O + 4 + 2 * i + j])

    def out_copy(i, j, a, b):
        cols = pl.ds(al(j * 512 + b * 256, 256), 256)
        return pltpu.make_async_copy(out_v.at[2 * i + j, pl.ds(2 * a, 2), :, pl.ds(b * 256, 256)],
                                     o_hbm.at[i, pl.ds(2 * a, 2), :, cols], sem_out.at[0])

    for j in range(2):
        x_copy(0, j).start()
    for s in range(6):
        slab_copy(wqkv_hbm, W_QKV, s).start()
    for s in range(2):
        slab_copy(wo_hbm, W_O, s).start()
    for t in range(NQ):
        slab_copy(wg_hbm, W_G, t).start()
        slab_copy(wu_hbm, W_U, t).start()
    for j in range(2):
        wd_copy(j).start()
    for i in range(1, NTILE):
        for j in range(2):
            x_copy(i, j).start()

    opaque[0] = 0
    origin = lambda: opaque[0]
    for ref in (o_v.at[NB], tu_v.at[20], tr_v.at[0], s1_v.at[0, 0], s2_v.at[0, 0], s3_v.at[0, 0], s4_v.at[0, 0]):
        ref[:8, :] = jnp.zeros((8, 128), F32)
    for ref in (ha_v.at[49 * (NQ - 1)], xa2_v.at[98], wt_v.at[6 * 32], wo_v.at[2 * 64]):
        ref[:16, :128] = jnp.zeros((16, 128), BF16)
    for ref in (t2_v, t3_v, tg_v, tu_v, b1_v, b1t_v, b1d_v):
        ref[origin(), :8, :128] = jnp.zeros((8, 128), F32)
    pin_ha = lambda: ha_v.bitcast(F32)[49 * (NQ - 1), :8, :]
    pin_xa = lambda: xa2_v.bitcast(F32)[98, :8, :]
    pin_wt = lambda: wt_v[6 * 32, :, :128].astype(F32)[:8]
    pin_wo = lambda: wo_v[origin() + 2 * 64, :, :128].astype(F32)[:8]
    pin_o = lambda: o_v[NB, :8, :]
    pin_hh, pin_tr = [lambda ref=ref: ref[origin(), :8, :] for ref in (hh_v, tr_v)]
    pin_s = [lambda ref=ref: ref[origin(), 0, :8, :] for ref in (s1_v, s2_v, s3_v, s4_v)]

    def gate_to(ref, at):
        def gate(v):
            if ref.dtype == F32:
                ref[at() + (slice(0, 8), slice(0, 128))] = v
            else:
                ref[at() + (slice(0, 16), slice(0, 128))] = jnp.concatenate([v, v], axis=0).astype(BF16)
        return gate
    gate_hh, gate_tr = [gate_to(ref, lambda: (origin() + 1,)) for ref in (hh_v, tr_v)]
    gate_s = [gate_to(ref, lambda: (origin() + 1, 0)) for ref in (s1_v, s2_v, s3_v, s4_v)]
    gate_qk, gate_v = gate_to(qk_v, lambda: (2 * NB,)), gate_to(v_v, lambda: (NB,))
    gate_x = gate_to(x_v, lambda: (4 * NTILE,))
    gate_wqkv, gate_wo = gate_to(wa_v, lambda: (8,)), gate_to(wa_v, lambda: (origin() + 8,))
    packed = lambda ref, n: pltpu.bitcast(ref.bitcast(F32)[n], BF16)
    cat = lambda ref, lo, n: jnp.concatenate([packed(ref, lo + k) for k in range(n)], axis=1)

    def x_operands(src, j, r, kk, p):
        rows = lambda base: pl.ds(al(base + j * MH + r, RG), RG)
        l1, l2 = _lhs2(lambda a, c: src[2 + 4 * a + c, pl.ds(al(kk * MH + r, RG), RG), :], p)
        for (a, c), v in l1.items():
            xa1_v[4 * p + 2 * c + kk, rows(a * M), :] = v.astype(BF16)
        for q, v in enumerate(l2):
            xa2_v[2 * (7 * p + q) + kk, rows(0), :] = v

    def h_operands(t, r, p):
        for q, v in enumerate(_lhs2(lambda a, c: hh_v[2 + 4 * a + c, r:r + RG, :], p)[1]):
            ha_v[(7 * p + q) * (NQ - 1) + t, r:r + RG, :] = v

    def scores(r0, n, ws):
        qs = [qk_v[b, pl.ds(r0 + HIST, AG), :] for b in range(NB)]
        for w in ws:
            s1_v[2 + n, w] = _tree(jnp.add, [qs[b] * qk_v[NB + b, pl.ds(r0 + HIST - DIL * w, AG), :]
                                             for b in range(NB)])

    def logits(pos, may_mask, n):
        ls = []
        for w in range(WIN):
            t = s1_v[2 + n, w]
            t = t + pltpu.roll(t, 64, 1)
            t = t + pltpu.roll(t, 32, 1)
            t = t * (DH ** -0.5)
            if may_mask < DIL * w:
                t = jnp.where(pos + lax.broadcasted_iota(jnp.int32, (AG, 128), 0) >= DIL * w, t, -1e9)
            ls.append(t)
        for w, t in enumerate(ls + [_tree(jnp.maximum, ls)]):
            s2_v[2 + n, w] = t

    def exps(n):
        m = s2_v[2 + n, WIN]
        es = [jnp.exp(s2_v[2 + n, w] - m) for w in range(WIN)]
        for w, e in enumerate(es + [_tree(jnp.add, es)]):
            s3_v[2 + n, w] = e

    def reciprocals(ns):
        for n in ns:
            s4_v[2 + n, 0] = 1.0 / s3_v[2 + n, WIN]

    def mix(r0, n, bs):
        es = [s3_v[2 + n, w] for w in range(WIN)]
        for b in bs:
            o_v[b, pl.ds(r0, AG), :] = s4_v[2 + n, 0] * _tree(
                jnp.add, [es[w] * v_v[b, pl.ds(r0 + HIST - DIL * w, AG), :] for w in range(WIN)])

    def stash(slot, c, v):
        for h in range(4):
            tr_v[2 + slot, pl.ds((4 * c + h) * PITCH, DH), :] = v[h * DH:(h + 1) * DH]

    def gather(slot, d):
        return tr_v[2 + slot, pl.ds(d, 16, stride=PITCH), :].astype(BF16)

    def reorder(shadow, last, lags, spread, units, block, put, gates, gates_tr, pin):
        def spill(n, c):
            stash(n % STASH, c, block(units[n], c))

        def fill(n, d0):
            for d in range(d0, d0 + 8):
                put(units[n], d, gather(n % STASH, d))
        step = (last - lags[0]) / (len(units) + 1)
        assert lags[0] + 2 * step <= STASH * step
        for n in range(len(units)):
            shadow.add([functools.partial(spill, n, c) for c in range(4)], n * step, (n + spread) * step,
                       lags[0], gates, pin_tr if gates_tr else pin_m[0])
            shadow.add([functools.partial(fill, n, 8 * c) for c in range(4)],
                       lags[0] + (n + 1) * step, lags[0] + (n + 2) * step, lags[1], gates_tr, pin)
    STASH = tr_v.shape[0] - 2

    def tile(i, _):
        def first(f):
            pl.when(i == 0)(f)

        def wt(row, k0, kn, dtype):
            return wt_v[pl.ds(row, 8), :, k0:k0 + kn].astype(dtype).reshape(128, kn)

        @pl.when(i > 0)
        def _():
            qk_v[NB:2 * NB, :HIST, :] = qk_v[NB:2 * NB, TM:TM + HIST, :]
            v_v[:NB, :HIST, :] = v_v[:NB, TM:TM + HIST, :]

        def q_k(n, prepare):
            fill = _Shadow()
            if prepare:
                for s in range(2):
                    slab_copy(wqkv_hbm, W_QKV, 2 * n + s).wait()

                def put(unit, d, v):
                    wt_v[64 * n + 2 * d + unit[0], :, lanes(unit[1])] = v
                reorder(fill, LAST_T, LAG_T, 0, [(s, kb) for s in range(2) for kb in range(NB)],
                        lambda unit, c: wa_v[2 * n + unit[0], lanes(unit[1]), lanes(c)].T.astype(F32),
                        put, (gate_wqkv,), (), pin_wt)
            for c0 in (0, 2):
                def prod(q):
                    dtype = BF16 if len(R_TERMS[q]) == 1 else F32
                    b = _comb(R_TERMS[q], lambda r, c: wt(n * 32 + (c0 + c) * 8, r * 512, 512, dtype))
                    return fill.dot(cat(xa1_v, 4 * q, 4), b, NT)

                def emit(r, c, v):
                    qk_v[4 * n + c0 + c, HIST + r * 2 * M:HIST + (r + 1) * 2 * M, :] = v
                _level(prod, t3_v, emit)
            fill.finish()

        def q_k_step(n, _):
            lax.cond((i == 0) & (n >= 1) & (n <= 2), lambda: q_k(n, True), lambda: q_k(n, False))
            return 0
        if 'q' not in SKIP:
            lax.fori_loop(0, 4, q_k_step, 0)

        @first
        def _():
            for s in range(2):
                slab_copy(wo_hbm, W_O, s).wait()

        if 'v' not in SKIP:
            fill = _Shadow()

            def put(unit, d, v):
                wo_v[unit[0] * 64 + 2 * d + unit[2], :, lanes(unit[1])] = v
            reorder(fill, 92, LAG_W, 1, [(j, c, s) for j in range(2) for c in range(4) for s in range(2)],
                    lambda unit, n: wa_v[6 + unit[0], lanes(4 * unit[2] + n), lanes(unit[1])].astype(F32),
                    put, (gate_wo,), (gate_tr,), pin_wo)
            for j in range(2):
                ops = _rhs2(lambda r, c, dtype: wt(128 + j * 32 + c * 8, r * KQ, KQ, dtype), b1t_v, j)

                def emit(r, c, v, ref):
                    v_v[4 * j + c, HIST + r * M:HIST + (r + 1) * M, :] = v
                _strassen2(lambda n: fill.dot(cat(xa2_v, 2 * n, 2), ops(n), NT), t2_v, (tg_v, tu_v)[j], emit)
            fill.finish()

        @first
        def _():
            for ref, base in ((qk_v, NB), (v_v, 0)):
                for b in range(base, base + NB):
                    ref[b, :HIST, :] = jnp.broadcast_to(ref[b, HIST:HIST + 1, :], (HIST, 128))

        def gate_up(t, _):
            @first
            def _():
                slab_copy(wg_hbm, W_G, t).wait()
                slab_copy(wu_hbm, W_U, t).wait()
            fill = _Shadow()
            if 'h' not in SKIP:
                fill.add([functools.partial(h_operands, jnp.maximum(t - 1, 0), r, p)
                          for p in ORDER for r in range(0, M, RG)], *SPAN_H, (), pin_ha)
            if 'a' not in SKIP:
                base = jnp.minimum(t * AROWS, M - AROWS)
                groups = list(enumerate((a * M + r, al(a * M + base + r, AG))
                                        for a in range(4) for r in range(0, AROWS, AG)))
                parts = [range(n, n + AP) for n in range(0, 8, AP)]
                fill.add([functools.partial(scores, r0, n, ws) for n, (_, r0) in groups for ws in parts],
                         *SPAN_A[0], (gate_qk,), pin_s[0])
                fill.add([functools.partial(logits, i * TM + r0, low, n) for n, (low, r0) in groups],
                         *SPAN_A[1], gate_s[0:1], pin_s[1])
                fill.add([functools.partial(exps, n) for n, _ in groups], *SPAN_A[2], gate_s[1:2], pin_s[2])
                fill.add([functools.partial(reciprocals, range(n, n + RB)) for n in range(0, len(groups), RB)],
                         *SPAN_A[3], gate_s[2:3], pin_s[3])
                fill.add([functools.partial(mix, r0, n, bs) for n, (_, r0) in groups for bs in parts],
                         *SPAN_A[4], (gate_s[2], gate_s[3], gate_v), pin_o)
            g = {}

            def emit_g(r, c, v, ref):
                if ref is None:
                    ref = tg_v.at[20 + 2 * r + c % 2]
                    ref[...] = v
                g[r, c] = ref

            def emit_u(r, c, v, ref):
                hh_v[2 + 4 * r + c] = g[r, c][...] * v
            for k, (w0, tmp, emit) in enumerate(((W_G, tg_v, emit_g), (W_U, tu_v, emit_u))):
                ops = _rhs2(lambda r, c, dtype: w_v[w0 + t, r * KQ:(r + 1) * KQ, lanes(c)].astype(dtype), b1_v, k)
                _strassen2(lambda n: fill.dot(cat(xa2_v, 2 * n, 2), ops(n)), t2_v, tmp, emit)
            fill.finish()
            return 0
        if 'g' not in SKIP:
            lax.fori_loop(0, NQ, gate_up, 0)

        @first
        def _():
            for j in range(2):
                wd_copy(j).wait()
            for n in range(1, NTILE):
                for j in range(2):
                    x_copy(n, j).wait()

        def down(j, _):
            fill = _Shadow()
            if 'l' not in SKIP:
                nxt, steps = jnp.minimum(i + 1, NTILE - 1), range(0, MH, RG)
                rows = [(a, r) for r in steps for a in range(4)]
                if '5' not in SKIP: fill.add([functools.partial(row_mean, nxt, j, a, r, n) for n, (a, r) in enumerate(rows)],
                         *SPAN_L[0], (gate_x,), pin_m[0])
                if '5' not in SKIP: fill.add([functools.partial(row_scale, nxt, j, a, r, n) for n, (a, r) in enumerate(rows)],
                         *SPAN_L[1], (gate_x, gate_m[0]), pin_m[1])
                if '6' not in SKIP: fill.add([functools.partial(normalize, nxt, j, a, r, n) for n, (a, r) in enumerate(rows)],
                         *SPAN_L[2], (gate_x, gate_m[0], gate_m[1]), pin_tu)
                if '7' not in SKIP: fill.add([functools.partial(x_operands, tu_v, j, r, kk, p)
                          for r in steps for kk in range(2) for p in range(7)], *SPAN_L[3], (gate_tu,), pin_xa)

            def weights(r, c, dtype):
                down = wd_v[j, :, lanes(r), lanes(c)].astype(dtype).reshape(NQ * 128, 128)
                proj = wo_v[pl.ds(j * 64 + r * 16, 16), :, lanes(c)].astype(dtype).reshape(KQ, 128)
                return jnp.concatenate([down, proj], axis=0)
            ops = _rhs2(weights, b1d_v)

            def prod(n):
                p, q = divmod(n, 7)
                direct = lambda blk: _comb(L_TERMS[q], lambda r, c: _comb(
                    L_TERMS[p], lambda a, b: blk(2 * a + r, 2 * b + c))).astype(BF16)
                parts = [packed(ha_v, n * (NQ - 1) + t) for t in range(NQ - 1)]
                parts.append(direct(lambda a, c: hh_v[2 + 4 * a + c]))
                parts += [direct(lambda a, c: o_v[2 * c + kk, a * M:(a + 1) * M, :]) for kk in range(2)]
                if not KSPLIT:
                    return fill.dot(jnp.concatenate(parts, axis=1), ops(n))
                b, out = ops(n), None
                for k, (lo, hi) in enumerate(zip((0,) + KSPLIT, KSPLIT + (len(parts),))):
                    y = fill.dot(jnp.concatenate(parts[lo:hi], axis=1), b[lo * 128:hi * 128])
                    out = y if out is None else y + t3_v[k - 1, :M]
                    if hi < len(parts):
                        t3_v[k, :M] = out
                return out

            def emit(r, c, v, ref):
                x = x_v[4 * i + r, :, pl.ds(al(j * 512 + c * 128, 128), 128)]
                out_v[2 * i + j, r, :, lanes(c)] = (v + x.astype(F32)).astype(BF16)
                if r % 2 == 1 and c % 2 == 1:
                    out_copy(i, j, r // 2, c // 2).start()
            _strassen2(prod, t2_v, tg_v, emit)
            fill.finish()
            return 0
        if 'd' not in SKIP:
            lax.fori_loop(0, 2, down, 0)
        return 0

    def layernorm_to(dst, i, j, a, r):
        x = x_v[4 * i + a, pl.ds(al(j * MH + r, RG), RG), :].astype(F32)
        xc = x - jnp.mean(x, axis=-1, keepdims=True)
        y = xc * lax.rsqrt(jnp.mean(xc * xc, axis=-1, keepdims=True) + 1e-5)
        for b in range(NB):
            dst[2 + 4 * a + b // 2, pl.ds(al((b % 2) * MH + r, RG), RG), :] = y[:, lanes(b)]
    x_rows = lambda i, j, a, r: x_v[4 * i + a, pl.ds(al(j * MH + r, RG), RG), :].astype(F32)

    def row_mean(i, j, a, r, n):
        m1_v[2 + n] = jnp.broadcast_to(jnp.mean(x_rows(i, j, a, r), axis=-1, keepdims=True), (RG, 128))

    def row_scale(i, j, a, r, n):
        xc = x_rows(i, j, a, r) - jnp.tile(m1_v[2 + n], (1, NB))
        m2_v[2 + n] = jnp.broadcast_to(jnp.mean(xc * xc, axis=-1, keepdims=True), (RG, 128))

    def normalize(i, j, a, r, n):
        x, m, scale = x_rows(i, j, a, r), m1_v[2 + n], lax.rsqrt(m2_v[2 + n] + 1e-5)
        for b in range(NB):
            tu_v[2 + 4 * a + b // 2, pl.ds((b % 2) * MH + r, RG), :] = (x[:, lanes(b)] - m) * scale
    for ref in (m1_v, m2_v):
        ref[0, :8, :] = jnp.zeros((8, 128), F32)
    pin_m = [lambda ref=ref: ref[origin(), :8, :] for ref in (m1_v, m2_v)]
    gate_m = [gate_to(ref, lambda: (origin() + 1,)) for ref in (m1_v, m2_v)]
    pin_tu = lambda: tu_v[origin() + 20, :8, :]
    gate_tu = gate_to(tu_v, lambda: (origin() + 1,))

    def first_layernorm(j, _):
        x_copy(0, j).wait()

        def norm(r, _):
            for a in range(4):
                layernorm_to(hh_v, 0, j, a, r * RG)
            return 0
        lax.fori_loop(0, MH // RG, norm, 0)

        def operands(r, _):
            for kk in range(2):
                for p in range(7):
                    x_operands(hh_v, j, r * RG, kk, p)
            return 0
        lax.fori_loop(0, MH // RG, operands, 0)
        return 0

    def first_weights(s, _):
        slab_copy(wqkv_hbm, W_QKV, s).wait()

        def unit(kb, _):
            ks = pl.ds(al(kb * 128, 128), 128)
            for c in range(4):
                stash(0, c, wa_v[s, ks, lanes(c)].T.astype(F32))
            for d in range(DH):
                wt_v[2 * d + s, :, ks] = gather(0, d)
            return 0
        lax.fori_loop(0, NB, unit, 0)
        return 0
    if 'f' not in SKIP:
        lax.fori_loop(0, 2, first_layernorm, 0)
        lax.fori_loop(0, 2, first_weights, 0)
    lax.fori_loop(0, NTILE, tile, 0)
    pltpu.make_async_copy(o_hbm, o_hbm, sem_out.at[0]).wait()


@jax.jit
def pallas_parallel_sum__sliding_local_dilated__glu_gated_bilinear__prompt_kernel(
        A_x, A_wqkv, A_wo, B_x, B_w_gate, B_w_up, B_w_down):
    B, S, D = A_x.shape
    F = B_w_gate.shape[1]
    NB, NQ, M, NTILE = D // 128, F // 512, TM // 4, S // TM
    groups = 4 * pl.cdiv(M // AG, NQ)
    V = pltpu.VMEM
    out = pl.pallas_call(
        _kernel,
        out_shape=jax.ShapeDtypeStruct((NTILE, 4, M, D), BF16),
        in_specs=[pl.BlockSpec(memory_space=pl.ANY)] * 6,
        out_specs=pl.BlockSpec(memory_space=pl.ANY),
        scratch_shapes=[
            V((4 * NTILE + 1, M, D), BF16),
            V((2 * NTILE, 4, M, 512), BF16),
            V((2 * NQ, D, 512), BF16),
            V((9, D, 512), BF16),
            V((6 * 32 + 1, 16, D), BF16),
            V((2 * 64 + 1, 16, 512), BF16),
            V((2, NQ, 512, 512), BF16),
            V((2 + 8, 16 * PITCH, 128), F32),
            V((28, 2 * M, 128), BF16), V((99, M, 128), BF16), V((49 * (NQ - 1) + 1, M, 128), BF16),
            V((2 * NB + 1, TM + HIST, 128), F32), V((NB + 1, TM + HIST, 128), F32), V((NB + 1, TM, 128), F32),
            V((18, M, 128), F32), V((5, M, 128), F32), V((5, 2 * M, 128), F32),
            V((28, M, 128), F32), V((21, M, 128), F32),
            V((8, D // 4, 128), F32), V((8, 128, D // 4), F32), V((8, NQ * 128 + D // 4, 128), F32),
            *[V((2 + groups, n, AG, 128), F32) for n in (WIN, WIN + 1, WIN + 1, 1)],
            V((2 + 2 * M // RG, RG, 128), F32), V((2 + 2 * M // RG, RG, 128), F32),
            pltpu.SMEM((1,), jnp.int32),
            pltpu.SemaphoreType.DMA((2 * NQ + 10 + 2 * NTILE,)), pltpu.SemaphoreType.DMA((1,)),
        ],
        compiler_params=pltpu.CompilerParams(vmem_limit_bytes=126 << 20, flags=FLAGS),
    )(A_x.reshape(NTILE, 4, M, D), A_wqkv, A_wo, B_w_gate, B_w_up, B_w_down.reshape(NQ, 512, D))
    return out.reshape(B, S, D)
```

```python
import functools
import math
import jax
import jax.numpy as jnp
from jax import lax
import jax.experimental.pallas as pl
import jax.experimental.pallas.tpu as pltpu

H, WIN, DIL = 32, 8, 2
TM = 1024
RG = 16
AG = 8
HIST = 16
PITCH = 33
STEPS = 8
SKIP = ''
AP, RB, KSPLIT = 2, 2, (4,)
SPAN_H = (0, 91, 5)
SPAN_A = ((0, 50, 5), (6, 64, 8), (14, 72, 6), (30, 80, 5), (50, 92, 5))
SPAN_L = ((0, 68, 4), (6, 74, 4), (12, 80, 3), (26, 94, 3))
LN_MODE = 2
ROOM_D, ROOM_G = (1.0, 0), (0.6, 4)
LAG_T, LAG_W = (2, 2), (5, 5)
FLAGS = None
SPAN_W = ((0, 44, 4), (51, 93, 4))
AHEAD = 2
PAD = 8
SCOPES = False
LAST_T = 13.9
F32, BF16 = jnp.float32, jnp.bfloat16
NN = (((1,), (0,)), ((), ()))
NT = (((1,), (1,)), ((), ()))

L_TERMS = (((0, 0), (1, 1), 1), ((1, 0), (1, 1), 1), ((0, 0),), ((1, 1),),
           ((0, 0), (0, 1), 1), ((1, 0), (0, 0), -1), ((0, 1), (1, 1), -1))
R_TERMS = (((0, 0), (1, 1), 1), ((0, 0),), ((0, 1), (1, 1), -1), ((1, 0), (0, 0), -1),
           ((1, 1),), ((0, 0), (0, 1), 1), ((1, 0), (1, 1), 1))
ORDER = (1, 3, 4, 2, 0, 6, 5)


def _comb(term, get):
    if len(term) == 1:
        return get(*term[0])
    a, b = get(*term[0]), get(*term[1])
    return a + b if term[2] > 0 else a - b


def _scoped(name, f):
    def g(*args):
        with jax.named_scope(name):
            return f(*args)
    return g if SCOPES else f


def _attention_rows(steps):
    return pl.cdiv(TM // 32, steps) * 32


def _tree(f, xs):
    return xs[0] if len(xs) == 1 else f(_tree(f, xs[:len(xs) // 2]), _tree(f, xs[len(xs) // 2:]))


class _Shadow:
    def __init__(self, room=None):
        self.room = room
        self.calls, self.tasks, self.zeros, self.late = 0, [], {}, []

    def add(self, fns, first, last, lag, gates, pin):
        for n, fn in enumerate(fns):
            self.tasks.append((self.warp(first + n * (last - first) / len(fns)), fn, lag, gates, pin))
        self.tasks.sort(key=lambda task: task[0])

    def warp(self, at):
        if self.room is None:
            return at
        at *= sum(self.room) / len(self.room)
        for n, room in enumerate(self.room):
            if at < room:
                return n + at / room
            at -= room

    def dot(self, a, b, dims=NN):
        self.late += self.zeros.pop(self.calls, [])
        if self.late and b.dtype == F32:
            r0, c = b.shape[0] - 128, b.shape[1] - 128
            rows = [b[r:r + 8] for r in range(r0, r0 + 128, 8)]
            for step, zero in self.late:
                w = rows[14 - 2 * step]
                rows[14 - 2 * step] = jnp.concatenate([w[:, :c], w[:, c:] + zero], axis=1) if c else w + zero
            self.late = []
            b = jnp.concatenate(([b[:r0]] if r0 else []) + rows, axis=0)
        out = lax.dot_general(a, b.astype(BF16), dims, preferred_element_type=F32)
        events = []
        while self.tasks and self.tasks[0][0] < self.calls + 1:
            events.append(self.tasks.pop(0))
        for step in range(STEPS):
            group = [task for task in events if int((task[0] - self.calls) * STEPS) == step]
            row = step * out.shape[0] // STEPS
            for gate in {gate: None for task in group for gate in task[3]}:
                gate(out[row:row + 8])
            for task in group:
                task[1]()
            for lag, pin in {(task[2], task[4]): None for task in group}:
                self.zeros.setdefault(self.calls + lag, []).append((step, pin()))
        self.calls += 1
        return out

    def finish(self):
        assert not self.tasks


def _level(prod, tmp, emit, keep=None):
    tmp[0] = prod(1)
    c21 = tmp[0] + prod(3)
    emit(1, 0, c21)
    if keep is None:
        tmp[3] = c21
    tmp[1] = prod(4)
    c12 = tmp[1] + prod(2)
    emit(0, 1, c12)
    if keep is None:
        tmp[4] = c12
    tmp[2] = prod(0) - tmp[0] - tmp[1]
    emit(0, 0, (tmp[3] if keep is None else keep[2]) + tmp[2] + prod(6))
    emit(1, 1, (tmp[4] if keep is None else keep[1]) + tmp[2] + prod(5))


def _strassen2(prod, t2, t1, emit):
    def run(p, e, keep=None):
        _level(lambda q: prod(7 * p + q), t2, e, keep)

    def put(i):
        def f(r, c, v):
            t1[4 * i + 2 * r + c] = v
        return f
    get = lambda i, r, c: t1[4 * i + 2 * r + c]

    def c21(r, c, v):
        v = get(0, r, c) + v
        put(3)(r, c, v)
        emit(2 + r, c, v, t1.at[12 + 2 * r + c])

    def c12(r, c, v):
        v = get(1, r, c) + v
        put(4)(r, c, v)
        emit(r, 2 + c, v, t1.at[16 + 2 * r + c])
    run(1, put(0), t1.at[0:4])
    run(3, c21)
    run(4, put(1), t1.at[4:8])
    run(2, c12)
    run(0, lambda r, c, v: put(2)(r, c, v - get(0, r, c) - get(1, r, c)))
    run(6, lambda r, c, v: emit(r, c, get(3, r, c) + get(2, r, c) + v, None))
    run(5, lambda r, c, v: emit(2 + r, 2 + c, get(4, r, c) + get(2, r, c) + v, None))


def _room(calls, count, busy, shift):
    heavy = [len(R_TERMS[p]) > 1 and k < 4 for p in ORDER for k in range(7)]
    return [busy if heavy[(n + shift) // calls % 49] else 1.0 for n in range(49 * calls * count)]


def _rhs2(w, b1, slot=0):
    slots = {}

    def get(n):
        p, q = divmod(n, 7)
        if len(R_TERMS[p]) == 1:
            a, b = R_TERMS[p][0]
            dtype = BF16 if len(R_TERMS[q]) == 1 else F32
            return _comb(R_TERMS[q], lambda r, c: w(2 * a + r, 2 * b + c, dtype))
        if p not in slots:
            slots[p] = 4 * ((slot + len(slots)) % 2)
            for r in range(2):
                for c in range(2):
                    b1[slots[p] + 2 * r + c] = _comb(R_TERMS[p], lambda a, b: w(2 * a + r, 2 * b + c, F32))
        return _comb(R_TERMS[q], lambda r, c: b1[slots[p] + 2 * r + c])
    return get


def _lhs2(blk, p):
    l1 = {(r, c): _comb(L_TERMS[p], lambda a, b: blk(2 * a + r, 2 * b + c)) for r in range(2) for c in range(2)}
    return l1, [_comb(L_TERMS[q], lambda r, c: l1[r, c]).astype(BF16) for q in range(7)]


def _kernel(x_hbm, wqkv_hbm, wo_hbm, wg_hbm, wu_hbm, wd_hbm, o_hbm,
            x_v, out_v, w_v, wa_v, wt_v, wo_v, wd_v, tr_v, xa1_v, xa2_v, ha_v, qk_v, v_v, o_v,
            hh_v, t2_v, t3_v, tg_v, tu_v, b1_v, b1t_v, b1d_v, qkw_v, vw_v, s1_v, s2_v, s3_v, s4_v, m1_v, m2_v, opaque, sem_in, sem_out):
    S, D = x_hbm.shape[0] * TM, x_hbm.shape[-1]
    F = wg_hbm.shape[1]
    NTILE, NB, DH, NQ = S // TM, D // 128, D // H, F // 512
    M, KQ = TM // 4, D // 4
    MH, MQ = M // 2, M // 4
    AROWS = _attention_rows(NQ)
    W_G, W_U, W_QKV, W_O = 0, NQ, 2 * NQ, 2 * NQ + 6
    al = pl.multiple_of
    lanes = lambda n: slice(n * 128, (n + 1) * 128)

    def slab_copy(src, base, s):
        dst = w_v.at[base + s] if base < W_QKV else wa_v.at[base - W_QKV + s]
        return pltpu.make_async_copy(src.at[:, pl.ds(al(s * 512, 512), 512)], dst, sem_in.at[base + s])

    def wq_copy(n):
        rows = pl.ds(al(n % 2 * 512, 512), 512)
        return pltpu.make_async_copy(wqkv_hbm.at[rows, pl.ds(al(n // 2 * 512, 512), 512)], wa_v.at[n // 2, rows],
                                     sem_out.at[1 + n])

    def wd_copy(j):
        return pltpu.make_async_copy(wd_hbm.at[:, :, pl.ds(j * 512, 512)], wd_v.at[j], sem_in.at[W_O + 2 + j])

    def x_copy(i, j):
        rows = pl.ds(al(j * MQ, MQ), MQ)
        return pltpu.make_async_copy(x_hbm.at[i, :, rows], x_v.at[pl.ds(4 * i, 4), rows],
                                     sem_in.at[W_O + 4 + 4 * i + j])

    def out_copy(i, j, a, b):
        cols = pl.ds(al(j * 512 + b * 256, 256), 256)
        return pltpu.make_async_copy(out_v.at[2 * i + j, pl.ds(2 * a, 2), :, pl.ds(b * 256, 256)],
                                     o_hbm.at[i, pl.ds(2 * a, 2), :, cols], sem_out.at[0])

    early = [cp(j) for j in range(4) for cp in (functools.partial(x_copy, 0), wq_copy)]
    early += [slab_copy(wqkv_hbm, W_QKV, s) for s in range(2, 4)]
    for cp in early[:AHEAD]:
        cp.start()

    def start_next(step):
        for n in range(AHEAD, len(early)):
            pl.when(step == min(n - AHEAD, 7))(early[n].start)

    opaque[0] = 0
    origin = lambda: opaque[0]
    for ref in (o_v.at[NB], tu_v.at[20], tr_v.at[0], s1_v.at[0, 0], s2_v.at[0, 0], s3_v.at[0, 0], s4_v.at[0, 0]):
        ref[:8, :] = jnp.zeros((8, 128), F32)
    for ref in (ha_v.at[49 * (NQ - 1)], xa2_v.at[98], wt_v.at[6 * 32], wo_v.at[2 * 64]):
        ref[:16, :128] = jnp.zeros((16, 128), BF16)
    for ref in (t2_v, t3_v, tg_v, tu_v, b1_v, b1t_v, b1d_v):
        ref[origin(), :8, :128] = jnp.zeros((8, 128), F32)
    pin_ha = lambda: ha_v.bitcast(F32)[49 * (NQ - 1), :8, :]
    pin_xa = lambda: xa2_v.bitcast(F32)[98, :8, :]
    pin_wt = lambda: wt_v[6 * 32, :, :128].astype(F32)[:8]
    pin_wo = lambda: wo_v[2 * 64, :, :128].astype(F32)[:8]
    pin_o = lambda: o_v[NB, :8, :]
    pin_hh, pin_tr = [lambda ref=ref: ref[origin(), :8, :] for ref in (hh_v, tr_v)]
    pin_s = [lambda ref=ref: ref[origin(), 0, :8, :] for ref in (s1_v, s2_v, s3_v, s4_v)]

    def gate_to(ref, at):
        def gate(v):
            if ref.dtype == F32:
                ref[at() + (slice(0, 8), slice(0, 128))] = v
            else:
                ref[at() + (slice(0, 16), slice(0, 128))] = jnp.concatenate([v, v], axis=0).astype(BF16)
        return gate
    gate_hh, gate_tr = [gate_to(ref, lambda: (origin() + 1,)) for ref in (hh_v, tr_v)]
    gate_s = [gate_to(ref, lambda: (origin() + 1, 0)) for ref in (s1_v, s2_v, s3_v, s4_v)]
    gate_qkw, gate_vw = gate_to(qkw_v, lambda: (origin() + 2 * NB,)), gate_to(vw_v, lambda: (origin() + NB,))
    pin_qkw, pin_vw = lambda: qkw_v[origin() + 2 * NB, 8:16, :], lambda: vw_v[origin() + NB, 8:16, :]
    qkw_v[2 * NB, 8:16, :] = vw_v[NB, 8:16, :] = jnp.zeros((8, 128), F32)
    gate_x = gate_to(x_v, lambda: (4 * NTILE,))
    gate_wqkv = gate_to(wa_v, lambda: (8,))
    packed = lambda ref, n: pltpu.bitcast(ref.bitcast(F32)[n], BF16)
    cat = lambda ref, lo, n: jnp.concatenate([packed(ref, lo + k) for k in range(n)], axis=1)

    def x_operands(j, r, kk, p):
        rows = pl.ds(al(j * MH + r, RG), RG)
        l1, l2 = _lhs2(lambda a, c: tu_v[2 + 4 * a + c, pl.ds(kk * MH + r, RG), :], p)
        for (a, c), v in l1.items():
            xa1_v[2 * (4 * p + 2 * c + kk) + a, rows, :] = v.astype(BF16)
        for q, v in enumerate(l2):
            xa2_v[2 * (7 * p + q) + kk, rows, :] = v

    def h_operands(t, r, p):
        for q, v in enumerate(_lhs2(lambda a, c: hh_v[2 + 4 * a + c, r:r + RG, :], p)[1]):
            ha_v[(7 * p + q) * (NQ - 1) + t, r:r + RG, :] = v

    def window(src, dst, b, base, lo, hi):
        dst[b, lo:hi, :] = src.at[:, pl.ds(base, AROWS + HIST)][b, lo:hi, :]

    def windows(src, dst, planes, base):
        cuts = range(0, AROWS + HIST + 1, (AROWS + HIST) // 2)
        return [functools.partial(window, src, dst, b, base, lo, hi) for lo, hi in zip(cuts, cuts[1:]) for b in planes]

    def scores(qk, n, ws):
        r0 = n * AG
        qs = [qk[b, pl.ds(r0 + HIST, AG), :] for b in range(NB)]
        for w in ws:
            s1_v[2 + n, w] = _tree(jnp.add, [qs[b] * qk[NB + b, pl.ds(r0 + HIST - DIL * w, AG), :]
                                             for b in range(NB)])

    def logits(pos, may_mask, n):
        ls = []
        for w in range(WIN):
            t = s1_v[2 + n, w]
            t = t + pltpu.roll(t, 64, 1)
            t = t + pltpu.roll(t, 32, 1)
            if may_mask < DIL * w:
                t = jnp.where(pos + lax.broadcasted_iota(jnp.int32, (AG, 128), 0) >= DIL * w, t, -1e9 * DH ** 0.5)
            ls.append(t)
        for w, t in enumerate(ls + [_tree(jnp.maximum, ls)]):
            s2_v[2 + n, w] = t

    def exps(n):
        m = s2_v[2 + n, WIN]
        es = [jnp.exp2((s2_v[2 + n, w] - m) * (DH ** -0.5 * math.log2(math.e))) for w in range(WIN)]
        for w, e in enumerate(es + [_tree(jnp.add, es)]):
            s3_v[2 + n, w] = e

    def reciprocals(ns):
        for n in ns:
            s4_v[2 + n, 0] = 1.0 / s3_v[2 + n, WIN]

    def mix(v, o, n, bs):
        r0 = n * AG
        es = [s3_v[2 + n, w] for w in range(WIN)]
        for b in bs:
            o[b, pl.ds(r0, AG), :] = s4_v[2 + n, 0] * _tree(
                jnp.add, [es[w] * v[b, pl.ds(r0 + HIST - DIL * w, AG), :] for w in range(WIN)])

    def stash(slot, c, v):
        for h in range(4):
            tr_v[2 + slot, pl.ds((4 * c + h) * PITCH, DH), :] = v[h * DH:(h + 1) * DH]

    def gather(slot, d):
        return tr_v[2 + slot, pl.ds(d, 16, stride=PITCH), :].astype(BF16)

    def reorder(shadow, last, lags, spread, units, block, put, gates, gates_tr, pin):
        def spill(n, c):
            stash(n % STASH, c, block(units[n], c))

        def fill(n, d0):
            for d in range(d0, d0 + 8):
                put(units[n], d, gather(n % STASH, d))
        step = (last - lags[0]) / (len(units) + 1)
        assert lags[0] + 2 * step <= STASH * step
        for n in range(len(units)):
            shadow.add([functools.partial(spill, n, c) for c in range(4)], n * step, (n + spread) * step,
                       lags[0], gates, pin_tr if gates_tr else pin_s[0])
            shadow.add([functools.partial(fill, n, 8 * c) for c in range(4)],
                       lags[0] + (n + 1) * step, lags[0] + (n + 2) * step, lags[1], gates_tr, pin)
    STASH = tr_v.shape[0] - 2

    def before_start(ref, base):
        for b in range(base, base + NB):
            ref[b, :HIST, :] = jnp.broadcast_to(ref[b, HIST:HIST + 1, :], (HIST, 128))

    def tile(i, _):
        def first(f):
            pl.when(i == 0)(f)

        def wt(row, k0, kn, dtype):
            return wt_v[pl.ds(row, 8), :, k0:k0 + kn].astype(dtype).reshape(128, kn)

        @pl.when(i > 0)
        def _():
            qk_v[NB:2 * NB, :HIST, :] = qk_v[NB:2 * NB, TM:TM + HIST, :]
            v_v[:NB, :HIST, :] = v_v[:NB, TM:TM + HIST, :]

        def q_k(n, prepare):
            fill = _Shadow()
            if prepare:
                for s in range(2):
                    slab_copy(wqkv_hbm, W_QKV, 2 * n + s).wait()

                @pl.when(n == 1)
                def _():
                    for s in range(2):
                        slab_copy(wqkv_hbm, W_QKV, 4 + s).start()

                @pl.when(n == 2)
                def _():
                    for s in range(2):
                        slab_copy(wo_hbm, W_O, s).start()
                    for k in range(1, NTILE):
                        for j in range(4):
                            x_copy(k, j).start()
                    slab_copy(wg_hbm, W_G, 0).start()
                    slab_copy(wu_hbm, W_U, 0).start()

                def put(unit, d, v):
                    wt_v[64 * n + 2 * d + unit[0], :, lanes(unit[1])] = v
                reorder(fill, LAST_T, LAG_T, 0, [(s, kb) for s in range(2) for kb in range(NB)],
                        lambda unit, c: wa_v[2 * n + unit[0], lanes(unit[1]), lanes(c)].T.astype(F32),
                        put, (gate_wqkv,), (), pin_wt)
            for c0 in (0, 2):
                def prod(q):
                    dtype = BF16 if len(R_TERMS[q]) == 1 else F32
                    b = _comb(R_TERMS[q], lambda r, c: wt(n * 32 + (c0 + c) * 8, r * 512, 512, dtype))
                    a = jnp.concatenate([jnp.concatenate([packed(xa1_v, 2 * (4 * q + k) + h) for k in range(4)], axis=1)
                                         for h in range(2)], axis=0)
                    return fill.dot(a, b, NT)

                def emit(r, c, v):
                    qk_v[4 * n + c0 + c, HIST + r * 2 * M:HIST + (r + 1) * 2 * M, :] = v
                _level(prod, t3_v, emit)
            fill.finish()

        def q_k_step(n, _):
            lax.cond((i == 0) & (n >= 1) & (n <= 2), lambda: q_k(n, True), lambda: q_k(n, False))
            return 0
        if 'q' not in SKIP:
            lax.fori_loop(0, 4, _scoped('q_k_step', q_k_step), 0)

        @first
        def _():
            for s in range(2):
                slab_copy(wo_hbm, W_O, s).wait()
            for k in range(1, NTILE):
                for j in range(4):
                    x_copy(k, j).wait()
            before_start(qk_v, NB)

        following, steps = jnp.minimum(i + 1, NTILE - 1), range(0, MH, RG)
        blocks = [(k, a, r) for k, (a, r) in enumerate((a, r) for r in steps for a in range(4))]

        def value(j, _):
            fill = _Shadow()

            def put(unit, d, v):
                wo_v[j * 64 + 2 * d + unit[1], :, lanes(unit[0])] = v
            reorder(fill, 44, LAG_W, 1, [(c, s) for c in range(4) for s in range(2)],
                    lambda unit, n: wa_v[6 + j, lanes(4 * unit[1] + n), lanes(unit[0])].astype(F32),
                    put, (gate_wqkv,), (gate_tr,), pin_wo)
            fill.add(windows(qk_v, qkw_v, [j * NB + b for b in range(NB)], 0), 0, 44, 4, (), pin_qkw)
            ops = _rhs2(lambda r, c, dtype: wt(128 + j * 32 + c * 8, r * KQ, KQ, dtype), b1t_v)

            def emit(r, c, v, ref):
                v_v[4 * j + c, HIST + r * M:HIST + (r + 1) * M, :] = v
            _strassen2(lambda n: fill.dot(cat(xa2_v, 2 * n, 2), ops(n), NT), t2_v, tg_v, emit)
            fill.finish()
            return 0
        if 'v' not in SKIP:
            lax.fori_loop(0, 2, _scoped('value', value), 0)

        @first
        def _():
            before_start(v_v, 0)

        def gate_up(t, _):
            @first
            def _():
                slab_copy(wg_hbm, W_G, t).wait()
                slab_copy(wu_hbm, W_U, t).wait()

                @pl.when(t + 1 < NQ)
                def _():
                    slab_copy(wg_hbm, W_G, t + 1).start()
                    slab_copy(wu_hbm, W_U, t + 1).start()
                for j in range(2):
                    pl.when(t == 2 * j)(wd_copy(j).start)
            fill = _Shadow(_room(1, 2, *ROOM_G))
            if 'h' not in SKIP:
                fill.add([functools.partial(h_operands, jnp.maximum(t - 1, 0), r, p)
                          for p in (1, 5, 4, 6, 0, 2, 3) for r in range(0, M, RG)], *SPAN_H, (), pin_ha)
            if 'a' not in SKIP:
                base, nxt = [al(jnp.minimum(n * AROWS, TM - AROWS), 32) for n in (t, t + 1)]
                qk, v = qkw_v, vw_v
                fill.add(windows(v_v, vw_v, range(NB), base), *SPAN_W[0], (), pin_vw)
                fill.add(windows(qk_v, qkw_v, range(2 * NB), nxt), *SPAN_W[1], (), pin_qkw)
                o = o_v.at[:, pl.ds(base, AROWS)]
                groups = range(AROWS // AG)
                parts = [range(n, n + AP) for n in range(0, 8, AP)]
                fill.add([functools.partial(scores, qk, n, ws) for n in groups for ws in parts],
                         *SPAN_A[0], (gate_qkw,), pin_s[0])
                fill.add([functools.partial(logits, i * TM + base + n * AG, n * AG, n) for n in groups],
                         *SPAN_A[1], gate_s[0:1], pin_s[1])
                fill.add([functools.partial(exps, n) for n in groups], *SPAN_A[2], gate_s[1:2], pin_s[2])
                fill.add([functools.partial(reciprocals, range(n, n + RB)) for n in range(0, len(groups), RB)],
                         *SPAN_A[3], gate_s[2:3], pin_s[3])
                fill.add([functools.partial(mix, v, o, n, bs) for n in groups for bs in parts],
                         *SPAN_A[4], (gate_s[2], gate_s[3], gate_vw), pin_o)
            g = {}

            def emit_g(r, c, v, ref):
                if ref is None:
                    ref = tg_v.at[20 + 2 * r + c % 2]
                    ref[...] = v
                g[r, c] = ref

            def emit_u(r, c, v, ref):
                hh_v[2 + 4 * r + c] = g[r, c][...] * v
            for k, (w0, tmp, emit) in enumerate(((W_G, tg_v, emit_g), (W_U, tu_v, emit_u))):
                ops = _rhs2(lambda r, c, dtype: w_v[w0 + t, r * KQ:(r + 1) * KQ, lanes(c)].astype(dtype), b1_v, k)
                _strassen2(lambda n: fill.dot(cat(xa2_v, 2 * n, 2), ops(n)), t2_v, tmp, emit)
            fill.finish()
            return 0
        if 'g' not in SKIP:
            lax.fori_loop(0, NQ, _scoped('gate_up', gate_up), 0)

        @first
        def _():
            for j in range(2):
                wd_copy(j).wait()

        def down(j, _):
            fill = _Shadow(_room(1 + len(KSPLIT), 1, *ROOM_D))

            if 'l' not in SKIP:
                args = [(following, j * MH, a, r, k) for k, a, r in blocks]
                if LN_MODE == 0:
                    fill.add([functools.partial(layernorm, *x) for x in args], *SPAN_L[2], (gate_x,), pin_tu)
                elif LN_MODE == 1:
                    fill.add([functools.partial(center, *x) for x in args], *SPAN_L[0], (gate_x,), pin_m[1])
                    fill.add([functools.partial(rescale, *x, bs) for x in args for bs in (range(4), range(4, 8))],
                             *SPAN_L[2], (gate_tu, gate_m[1]), pin_tu)
                else:
                    fill.add([functools.partial(row_mean, *x) for x in args], *SPAN_L[0], (gate_x,), pin_m[0])
                    fill.add([functools.partial(row_scale, *x) for x in args],
                             *SPAN_L[1], (gate_x, gate_m[0]), pin_m[1])
                    fill.add([functools.partial(normalize, *x) for x in args],
                             *SPAN_L[2], (gate_x, gate_m[0], gate_m[1]), pin_tu)
                fill.add([functools.partial(x_operands, j, r, kk, p)
                          for r in steps for kk in range(2) for p in range(7)], *SPAN_L[3], (gate_tu,), pin_xa)

            def weights(r, c, dtype):
                down = wd_v[j, :, lanes(r), lanes(c)].astype(dtype).reshape(NQ * 128, 128)
                proj = wo_v[pl.ds(j * 64 + r * 16, 16), :, lanes(c)].astype(dtype).reshape(KQ, 128)
                return jnp.concatenate([down, proj], axis=0)
            ops = _rhs2(weights, b1d_v)

            def prod(n):
                p, q = divmod(n, 7)
                direct = lambda blk: _comb(L_TERMS[q], lambda r, c: _comb(
                    L_TERMS[p], lambda a, b: blk(2 * a + r, 2 * b + c))).astype(BF16)
                parts = [packed(ha_v, n * (NQ - 1) + t) for t in range(NQ - 1)]
                parts.append(direct(lambda a, c: hh_v[2 + 4 * a + c]))
                parts += [direct(lambda a, c: o_v[2 * c + kk, a * M:(a + 1) * M, :]) for kk in range(2)]
                if not KSPLIT:
                    return fill.dot(jnp.concatenate(parts, axis=1), ops(n))
                b, out = ops(n), None
                for k, (lo, hi) in enumerate(zip((0,) + KSPLIT, KSPLIT + (len(parts),))):
                    y = fill.dot(jnp.concatenate(parts[lo:hi], axis=1), b[lo * 128:hi * 128])
                    out = y if out is None else y + t3_v[k - 1, :M]
                    if hi < len(parts):
                        t3_v[k, :M] = out
                return out

            def emit(r, c, v, ref):
                x = x_v[4 * i + r, :, pl.ds(al(j * 512 + c * 128, 128), 128)]
                out_v[2 * i + j, r, :, lanes(c)] = (v + x.astype(F32)).astype(BF16)
                if r % 2 == 1 and c % 2 == 1:
                    out_copy(i, j, r // 2, c // 2).start()
            _strassen2(prod, t2_v, tg_v, emit)
            fill.finish()
            return 0
        if 'd' not in SKIP:
            lax.fori_loop(0, 2, _scoped('down', down), 0)
        return 0

    x_rows = lambda i, j, a, r: x_v.at[4 * i + a, pl.ds(al(j, MQ), MH if r >= MQ else MQ)][r:r + RG, :].astype(F32)

    def row_mean(i, j, a, r, n):
        m1_v[2 + n] = jnp.broadcast_to(jnp.mean(x_rows(i, j, a, r), axis=-1, keepdims=True), (RG, 128))

    def row_scale(i, j, a, r, n):
        xc = x_rows(i, j, a, r) - jnp.tile(m1_v[2 + n], (1, NB))
        m2_v[2 + n] = jnp.broadcast_to(jnp.mean(xc * xc, axis=-1, keepdims=True), (RG, 128))

    def layernorm(i, j, a, r, n):
        x = x_rows(i, j, a, r)
        xc = x - jnp.mean(x, axis=-1, keepdims=True)
        y = xc * lax.rsqrt(jnp.mean(xc * xc, axis=-1, keepdims=True) + 1e-5)
        for b in range(NB):
            tu_v[2 + 4 * a + b // 2, pl.ds((b % 2) * MH + r, RG), :] = y[:, lanes(b)]

    def center(i, j, a, r, n):
        x = x_rows(i, j, a, r)
        xc = x - jnp.mean(x, axis=-1, keepdims=True)
        m2_v[2 + n] = jnp.broadcast_to(jnp.mean(xc * xc, axis=-1, keepdims=True), (RG, 128))
        for b in range(NB):
            tu_v[2 + 4 * a + b // 2, pl.ds((b % 2) * MH + r, RG), :] = xc[:, lanes(b)]

    def rescale(i, j, a, r, n, bs):
        scale = lax.rsqrt(m2_v[2 + n] + 1e-5)
        for b in bs:
            at = (2 + 4 * a + b // 2, pl.ds((b % 2) * MH + r, RG))
            tu_v[at] = tu_v[at] * scale

    def normalize(i, j, a, r, n):
        x, m, scale = x_rows(i, j, a, r), m1_v[2 + n], lax.rsqrt(m2_v[2 + n] + 1e-5)
        for b in range(NB):
            tu_v[2 + 4 * a + b // 2, pl.ds((b % 2) * MH + r, RG), :] = (x[:, lanes(b)] - m) * scale
    m1_v[1, 8:, :] = m2_v[2 + TM // RG, :8, :] = jnp.zeros((8, 128), F32)
    pin_m = [lambda: m1_v[origin() + 1, 8:, :], lambda: m2_v[2 + TM // RG, :8, :]]
    gate_m = [gate_to(ref, lambda: (origin() + 1,)) for ref in (m1_v, m2_v)]
    pin_tu = lambda: tu_v[origin() + 20, :8, :]
    gate_tu = gate_to(tu_v, lambda: (origin() + 1,))

    def start_up(j, _):
        _scoped('xwait', x_copy(0, j).wait)()
        start_next(2 * j)
        for n, (a, r) in enumerate((a, r) for r in range(0, MQ, RG) for a in range(4)):
            row_mean(0, j * MQ, a, r, n)
            row_scale(0, j * MQ, a, r, n)
        _scoped('wwait', wq_copy(j).wait)()
        start_next(2 * j + 1)
        for u in range(4):
            ks = pl.ds(al(j % 2 * 512 + u * 128, 128), 128)
            for c in range(4):
                stash(u, c, wa_v[j // 2, ks, lanes(c)].T.astype(F32))
            rows = pl.ds(al(j * MQ + u * RG, RG), RG)
            stats = [(m1_v[2 + 4 * u + a], lax.rsqrt(m2_v[2 + 4 * u + a] + 1e-5)) for a in range(4)]
            for kk in range(2):
                y = {(a, c): (x_v[a, rows, lanes(2 * c + kk)].astype(F32) - stats[a][0]) * stats[a][1]
                     for a in range(4) for c in range(4)}
                for p in range(7):
                    l1, l2 = _lhs2(lambda a, c: y[a, c], p)
                    for (a, c), v in l1.items():
                        xa1_v[2 * (4 * p + 2 * c + kk) + a, rows, :] = v.astype(BF16)
                    for q, v in enumerate(l2):
                        xa2_v[2 * (7 * p + q) + kk, rows, :] = v
            for d in range(DH):
                wt_v[2 * d + j // 2, :, ks] = gather(u, d)
        return 0
    if 'f' not in SKIP:
        lax.fori_loop(0, 4, _scoped('start', start_up), 0)
    lax.fori_loop(0, NTILE, tile, 0)
    pltpu.make_async_copy(o_hbm, o_hbm, sem_out.at[0]).wait()


@jax.jit
def pallas_parallel_sum__sliding_local_dilated__glu_gated_bilinear__prompt_kernel(
        A_x, A_wqkv, A_wo, B_x, B_w_gate, B_w_up, B_w_down):
    B, S, D = A_x.shape
    F = B_w_gate.shape[1]
    NB, NQ, M, NTILE = D // 128, F // 512, TM // 4, S // TM
    groups = _attention_rows(NQ) // AG
    V = pltpu.VMEM
    out = pl.pallas_call(
        _kernel,
        out_shape=jax.ShapeDtypeStruct((NTILE, 4, M, D), BF16),
        in_specs=[pl.BlockSpec(memory_space=pl.ANY)] * 6,
        out_specs=pl.BlockSpec(memory_space=pl.ANY),
        scratch_shapes=[
            V((4 * NTILE + 1, M, D), BF16),
            V((2 * NTILE, 4, M, 512), BF16),
            V((2 * NQ, D, 512), BF16),
            V((9, D, 512), BF16),
            V((6 * 32 + 1, 16, D), BF16),
            V((2 * 64 + 1, 16, 512), BF16),
            V((2, NQ, 512, 512), BF16),
            V((2 + 8, 16 * PITCH, 128), F32),
            V((56, M, 128), BF16), V((99, M, 128), BF16), V((49 * (NQ - 1) + 1, M, 128), BF16),
            V((2 * NB + 1, TM + HIST + PAD, 128), F32), V((NB + 1, TM + HIST + PAD, 128), F32), V((NB + 1, TM, 128), F32),
            V((18, M, 128), F32), V((5, M, 128), F32), V((5, 2 * M, 128), F32),
            V((28, M, 128), F32), V((21, M, 128), F32),
            V((8, D // 4, 128), F32), V((8, 128, D // 4), F32), V((8, NQ * 128 + D // 4, 128), F32),
            V((2 * NB + 1, groups * AG + HIST + PAD, 128), F32), V((NB + 1, groups * AG + HIST + PAD, 128), F32),
            *[V((2 + groups, n, AG, 128), F32) for n in (WIN, WIN + 1, WIN + 1, 1)],
            V((2 + TM // RG, RG, 128), F32), V((3 + TM // RG, RG, 128), F32),
            pltpu.SMEM((1,), jnp.int32),
            pltpu.SemaphoreType.DMA((2 * NQ + 10 + 4 * NTILE,)), pltpu.SemaphoreType.DMA((5,)),
        ],
        compiler_params=pltpu.CompilerParams(vmem_limit_bytes=126 << 20, flags=FLAGS),
    )(A_x.reshape(NTILE, 4, M, D), A_wqkv, A_wo, B_w_gate, B_w_up, B_w_down.reshape(NQ, 512, D))
    return out.reshape(B, S, D)
```

```python
import functools
import math
import jax
import jax.numpy as jnp
from jax import lax
import jax.experimental.pallas as pl
import jax.experimental.pallas.tpu as pltpu

H, WIN, DIL = 32, 8, 2
TM = 1024
RG = 16
AG = 8
HIST = 16
PITCH = 33
STEPS = 8
SKIP = ''
AP, RB, KSPLIT = 2, 2, (4,)
SPAN_H = (0, 91, 5)
SPAN_A = ((0, 50, 5), (6, 64, 8), (14, 72, 6), (30, 80, 5), (50, 92, 5))
SPAN_L = ((0, 68, 4), (6, 74, 4), (12, 80, 3), (26, 94, 3))
LN_MODE = 2
T_MODE = (0, 1, 0)
WCUT = 88
PIN_TILE, PIN_SPAN = 0, 8
ROOM_D, ROOM_G = (1.0, 0), (0.6, 4)
LAG_T, LAG_W = (6, 3), (5, 5)
FLAGS = None
SPAN_W = ((0, 44, 4), (51, 93, 4))
AHEAD = 3
PAD = 8
SCOPES = False
LAST_T = 46
F32, BF16 = jnp.float32, jnp.bfloat16
NN = (((1,), (0,)), ((), ()))
NT = (((1,), (1,)), ((), ()))

L_TERMS = (((0, 0), (1, 1), 1), ((1, 0), (1, 1), 1), ((0, 0),), ((1, 1),),
           ((0, 0), (0, 1), 1), ((1, 0), (0, 0), -1), ((0, 1), (1, 1), -1))
R_TERMS = (((0, 0), (1, 1), 1), ((0, 0),), ((0, 1), (1, 1), -1), ((1, 0), (0, 0), -1),
           ((1, 1),), ((0, 0), (0, 1), 1), ((1, 0), (1, 1), 1))
ORDER = (1, 3, 4, 2, 0, 6, 5)
SWAP = (0, 1, 0, 0, 1, 1, 1)


def _comb(term, get):
    if len(term) == 1:
        return get(*term[0])
    a, b = get(*term[0]), get(*term[1])
    return a + b if term[2] > 0 else a - b


def _scoped(name, f):
    def g(*args):
        with jax.named_scope(name):
            return f(*args)
    return g if SCOPES else f


def _attention_rows(steps):
    return pl.cdiv(TM // 32, steps) * 32


def _tree(f, xs):
    return xs[0] if len(xs) == 1 else f(_tree(f, xs[:len(xs) // 2]), _tree(f, xs[len(xs) // 2:]))


class _Shadow:
    def __init__(self, room=None):
        self.room = room
        self.calls, self.tasks, self.zeros, self.late = 0, [], {}, []

    def add(self, fns, first, last, lag, gates, pin):
        for n, fn in enumerate(fns):
            self.tasks.append((self.warp(first + n * (last - first) / len(fns)), fn, lag, gates, pin))
        self.tasks.sort(key=lambda task: task[0])

    def warp(self, at):
        if self.room is None:
            return at
        at *= sum(self.room) / len(self.room)
        for n, room in enumerate(self.room):
            if at < room:
                return n + at / room
            at -= room

    def dot(self, a, b, dims=NN):
        self.late += self.zeros.pop(self.calls, [])
        if self.late and b.dtype == F32:
            rows = [[b[r:r + 8, c:c + 128] for c in range(0, b.shape[1], 128)] for r in range(0, b.shape[0], 8)]
            tiles = b.size // (128 * 128)
            for step, zero in self.late:
                tile = tiles - 1 - (step * PIN_TILE) % tiles
                r, c = (16 * tile, 0) if len(rows[0]) == 1 else (0, tile)
                rows[r + 14 - 2 * (step * PIN_SPAN // STEPS)][c] += zero
            self.late = []
            b = jnp.concatenate([jnp.concatenate(row, axis=1) for row in rows], axis=0)
        out = lax.dot_general(a, b.astype(BF16), dims, preferred_element_type=F32)
        events = []
        while self.tasks and self.tasks[0][0] < self.calls + 1:
            events.append(self.tasks.pop(0))
        for step in range(STEPS):
            group = [task for task in events if int((task[0] - self.calls) * STEPS) == step]
            row = step * out.shape[0] // STEPS
            for gate in {gate: None for task in group for gate in task[3]}:
                gate(out[row:row + 8])
            for task in group:
                task[1]()
            for lag, pin in {(task[2], task[4]): None for task in group if task[4]}:
                self.zeros.setdefault(self.calls + lag, []).append((step, pin()))
        self.calls += 1
        return out

    def finish(self):
        assert not self.tasks


def _level(prod, tmp, emit, keep=None):
    tmp[0] = prod(1)
    c21 = tmp[0] + prod(3)
    emit(1, 0, c21)
    if keep is None:
        tmp[3] = c21
    tmp[1] = prod(4)
    c12 = tmp[1] + prod(2)
    emit(0, 1, c12)
    if keep is None:
        tmp[4] = c12
    tmp[2] = prod(0) - tmp[0] - tmp[1]
    emit(0, 0, (tmp[3] if keep is None else keep(1, 0)) + tmp[2] + prod(6))
    emit(1, 1, (tmp[4] if keep is None else keep(0, 1)) + tmp[2] + prod(5))


def _strassen2(prod, t2, t1, emit):
    def run(p, e, keep=None):
        _level(lambda q: prod(7 * p + q), t2, lambda r, c, v: e(r, c ^ SWAP[p], v),
               keep and (lambda r, c: keep(r, c ^ SWAP[p])))

    def put(i):
        def f(r, c, v):
            t1[4 * i + 2 * r + c] = v
        return f
    get = lambda i, r, c: t1[4 * i + 2 * r + c]

    def c21(r, c, v):
        v = get(0, r, c) + v
        put(3)(r, c, v)
        emit(2 + r, c, v, t1.at[12 + 2 * r + c])

    def c12(r, c, v):
        v = get(1, r, c) + v
        put(4)(r, c, v)
        emit(r, 2 + c, v, t1.at[16 + 2 * r + c])
    run(1, put(0), functools.partial(get, 0))
    run(3, c21)
    run(4, put(1), functools.partial(get, 1))
    run(2, c12)
    run(0, lambda r, c, v: put(2)(r, c, v - get(0, r, c) - get(1, r, c)))
    run(6, lambda r, c, v: emit(r, c, get(3, r, c) + get(2, r, c) + v, None))
    run(5, lambda r, c, v: emit(2 + r, 2 + c, get(4, r, c) + get(2, r, c) + v, None))


def _room(calls, count, busy, shift):
    heavy = [len(R_TERMS[p]) > 1 and k < 4 for p in ORDER for k in range(7)]
    return [busy if heavy[(n + shift) // calls % 49] else 1.0 for n in range(49 * calls * count)]


def _rhs2(w, b1, slot=0):
    slots = {}

    def get(n):
        p, q = divmod(n, 7)
        if len(R_TERMS[p]) == 1:
            a, b = R_TERMS[p][0]
            dtype = BF16 if len(R_TERMS[q]) == 1 else F32
            return _comb(R_TERMS[q], lambda r, c: w(2 * a + r, 2 * b + (c ^ SWAP[p]), dtype))
        if p not in slots:
            slots[p] = 4 * ((slot + len(slots)) % 2)
            for r in range(2):
                for c in range(2):
                    b1[slots[p] + 2 * r + c] = _comb(R_TERMS[p], lambda a, b: w(2 * a + r, 2 * b + c, F32))
        return _comb(R_TERMS[q], lambda r, c: b1[slots[p] + 2 * r + (c ^ SWAP[p])])
    return get


def _lhs2(blk, p):
    l1 = {(r, c): _comb(L_TERMS[p], lambda a, b: blk(2 * a + r, 2 * b + c)) for r in range(2) for c in range(2)}
    return l1, [_comb(L_TERMS[q], lambda r, c: l1[r, c]).astype(BF16) for q in range(7)]


def _kernel(x_hbm, wqkv_hbm, wo_hbm, wg_hbm, wu_hbm, wd_hbm, o_hbm,
            x_v, out_v, w_v, wa_v, wt_v, wo_v, wd_v, tr_v, xa2_v, ha_v, qkv_v, o_v,
            hh_v, t2_v, t3_v, tg_v, tu_v, b1_v, b1t_v, b1d_v, qkw_v, vw_v, s1_v, s2_v, s3_v, s4_v, m1_v, m2_v, opaque, sem_in, sem_out):
    S, D = x_hbm.shape[0] * TM, x_hbm.shape[-1]
    F = wg_hbm.shape[1]
    NTILE, NB, DH, NQ = S // TM, D // 128, D // H, F // 512
    M, KQ = TM // 4, D // 4
    MH, MQ = M // 2, M // 4
    AROWS = _attention_rows(NQ)
    W_G, W_U, W_QKV, W_O = 0, NQ, 2 * NQ, 2 * NQ + 6
    al = pl.multiple_of
    qk_v, v_v = qkv_v.at[:2 * NB], qkv_v.at[2 * NB:]
    lanes = lambda n: slice(n * 128, (n + 1) * 128)

    def slab_copy(src, base, s):
        dst = w_v.at[base + s] if base < W_QKV else wa_v.at[base - W_QKV + s]
        return pltpu.make_async_copy(src.at[:, pl.ds(al(s * 512, 512), 512)], dst, sem_in.at[base + s])

    def wq_copy(n):
        rows = pl.ds(al(n % 2 * 512, 512), 512)
        return pltpu.make_async_copy(wqkv_hbm.at[rows, pl.ds(al(n // 2 * 512, 512), 512)], wa_v.at[n // 2, rows],
                                     sem_out.at[1 + n])

    def wd_copy(j):
        return pltpu.make_async_copy(wd_hbm.at[:, :, pl.ds(j * 512, 512)], wd_v.at[j], sem_in.at[W_O + 2 + j])

    def x_copy(i, j):
        rows = pl.ds(al(j * MQ, MQ), MQ)
        return pltpu.make_async_copy(x_hbm.at[i, :, rows], x_v.at[pl.ds(4 * i, 4), rows],
                                     sem_in.at[W_O + 4 + 4 * i + j])

    def out_copy(i, j, a, b):
        cols = pl.ds(al(j * 512 + b * 256, 256), 256)
        return pltpu.make_async_copy(out_v.at[2 * i + j, pl.ds(2 * a, 2), :, pl.ds(b * 256, 256)],
                                     o_hbm.at[i, pl.ds(2 * a, 2), :, cols], sem_out.at[0])

    early = [cp(j) for j in range(4) for cp in (functools.partial(x_copy, 0), wq_copy)]
    early += [slab_copy(wqkv_hbm, W_QKV, s) for s in range(2, 3)]
    for cp in early[:AHEAD]:
        cp.start()

    def start_next(step):
        for n in range(AHEAD, len(early)):
            pl.when(step == min(n - AHEAD, 7))(early[n].start)

    opaque[0] = 0
    origin = lambda: opaque[0]
    for ref in (o_v.at[NB], tu_v.at[20], tr_v.at[0], s1_v.at[0, 0], s2_v.at[0, 0], s3_v.at[0, 0], s4_v.at[0, 0]):
        ref[:8, :] = jnp.zeros((8, 128), F32)
    for ref in (ha_v.at[49 * (NQ - 1)], xa2_v.at[98], wt_v.at[6 * 32], wo_v.at[2 * 64]):
        ref[:16, :128] = jnp.zeros((16, 128), BF16)
    for ref in (t2_v, t3_v, tg_v, tu_v, b1_v, b1t_v, b1d_v):
        ref[origin(), :8, :128] = jnp.zeros((8, 128), F32)
    pin_ha = lambda: ha_v.bitcast(F32)[49 * (NQ - 1), :8, :]
    pin_xa = lambda: xa2_v.bitcast(F32)[98, :8, :]
    pin_wt = lambda: wt_v[6 * 32, :, :128].astype(F32)[:8]
    pin_wo = lambda: wo_v[origin() + 2 * 64, :, :128].astype(F32)[:8]
    pin_o = lambda: o_v[NB, :8, :]
    pin_hh, pin_tr = [lambda ref=ref: ref[origin(), :8, :] for ref in (hh_v, tr_v)]
    pin_s = [lambda ref=ref: ref[origin(), 0, :8, :] for ref in (s1_v, s2_v, s3_v, s4_v)]

    def gate_to(ref, at):
        def gate(v):
            if ref.dtype == F32:
                ref[at() + (slice(0, 8), slice(0, 128))] = v
            else:
                ref[at() + (slice(0, 16), slice(0, 128))] = jnp.concatenate([v, v], axis=0).astype(BF16)
        return gate
    gate_hh, gate_tr = [gate_to(ref, lambda: (origin() + 1,)) for ref in (hh_v, tr_v)]
    gate_s = [gate_to(ref, lambda: (origin() + 1, 0)) for ref in (s1_v, s2_v, s3_v, s4_v)]
    gate_qkw, gate_vw = gate_to(qkw_v, lambda: (origin() + 2 * NB,)), gate_to(vw_v, lambda: (origin() + NB,))
    pin_qkw, pin_vw = lambda: qkw_v[origin() + 2 * NB, 8:16, :], lambda: vw_v[origin() + NB, 8:16, :]
    qkw_v[2 * NB, 8:16, :] = vw_v[NB, 8:16, :] = jnp.zeros((8, 128), F32)
    gate_x = gate_to(x_v, lambda: (4 * NTILE,))
    gate_wqkv, gate_wo = gate_to(wa_v, lambda: (8,)), gate_to(wa_v, lambda: (origin() + 8,))
    packed = lambda ref, n: pltpu.bitcast(ref.bitcast(F32)[n], BF16)
    cat = lambda ref, lo, n: jnp.concatenate([packed(ref, lo + k) for k in range(n)], axis=1)

    def x_operands(j, r, kk, p):
        rows = pl.ds(al(j * MH + r, RG), RG)
        l1, l2 = _lhs2(lambda a, c: tu_v[2 + 4 * a + c, pl.ds(kk * MH + r, RG), :], p)
        for q, v in enumerate(l2):
            xa2_v[2 * (7 * p + q) + kk, rows, :] = v

    def h_operands(t, r, p):
        for q, v in enumerate(_lhs2(lambda a, c: hh_v[2 + 4 * a + c, r:r + RG, :], p)[1]):
            ha_v[(7 * p + q) * (NQ - 1) + t, r:r + RG, :] = v

    def window(src, dst, b, base, lo, hi):
        dst[b, lo:hi, :] = src.at[:, pl.ds(base, AROWS + HIST)][b, lo:hi, :]

    def windows(src, dst, planes, base):
        cuts = [*range(0, AROWS + HIST, WCUT), AROWS + HIST]
        return [functools.partial(window, src, dst, b, base, lo, hi) for lo, hi in zip(cuts, cuts[1:]) for b in planes]

    def scores(qk, n, ws):
        r0 = n * AG
        qs = [qk[b, pl.ds(r0 + HIST, AG), :] for b in range(NB)]
        for w in ws:
            s1_v[2 + n, w] = _tree(jnp.add, [qs[b] * qk[NB + b, pl.ds(r0 + HIST - DIL * w, AG), :]
                                             for b in range(NB)])

    def logits(pos, may_mask, n):
        ls = []
        for w in range(WIN):
            t = s1_v[2 + n, w]
            t = t + pltpu.roll(t, 64, 1)
            t = t + pltpu.roll(t, 32, 1)
            if may_mask < DIL * w:
                t = jnp.where(pos + lax.broadcasted_iota(jnp.int32, (AG, 128), 0) >= DIL * w, t, -1e9 * DH ** 0.5)
            ls.append(t)
        for w, t in enumerate(ls + [_tree(jnp.maximum, ls)]):
            s2_v[2 + n, w] = t

    def exps(n):
        m = s2_v[2 + n, WIN]
        es = [jnp.exp2((s2_v[2 + n, w] - m) * (DH ** -0.5 * math.log2(math.e))) for w in range(WIN)]
        for w, e in enumerate(es + [_tree(jnp.add, es)]):
            s3_v[2 + n, w] = e

    def reciprocals(ns):
        for n in ns:
            s4_v[2 + n, 0] = 1.0 / s3_v[2 + n, WIN]

    def mix(v, o, n, bs):
        r0 = n * AG
        es = [s3_v[2 + n, w] for w in range(WIN)]
        for b in bs:
            o[b, pl.ds(r0, AG), :] = s4_v[2 + n, 0] * _tree(
                jnp.add, [es[w] * v[b, pl.ds(r0 + HIST - DIL * w, AG), :] for w in range(WIN)])

    def stash(slot, c, v):
        for h in range(4):
            tr_v[2 + slot, pl.ds((4 * c + h) * PITCH, DH), :] = v[h * DH:(h + 1) * DH]

    def gather(slot, d):
        return tr_v[2 + slot, pl.ds(d, 16, stride=PITCH), :].astype(BF16)

    def reorder(shadow, last, lags, spread, units, block, put, gates, gates_tr, pin):
        def spill(n, c):
            stash(n % STASH, c, block(units[n], c))

        def fill(n, d0):
            for d in range(d0, d0 + 8):
                put(units[n], d, gather(n % STASH, d))
        step = (last - lags[0]) / (len(units) + 1)
        assert lags[0] + 2 * step <= STASH * step
        for n in range(len(units)):
            shadow.add([functools.partial(spill, n, c) for c in range(4)], n * step, (n + spread) * step,
                       lags[0], gates, pin_tr if gates_tr else pin_s[0])
            shadow.add([functools.partial(fill, n, 8 * c) for c in range(4)],
                       lags[0] + (n + 1) * step, lags[0] + (n + 2) * step, lags[1], gates_tr, pin)
    STASH = tr_v.shape[0] - 2

    def before_start(ref, base):
        for b in range(base, base + NB):
            ref[b, :HIST, :] = jnp.broadcast_to(ref[b, HIST:HIST + 1, :], (HIST, 128))

    def tile(i, _):
        def first(f):
            pl.when(i == 0)(f)

        def wt(row, k0, kn, dtype):
            return wt_v[pl.ds(row, 8), :, k0:k0 + kn].astype(dtype).reshape(128, kn)

        @pl.when(i > 0)
        def _():
            qkv_v[NB:, :HIST, :] = qkv_v[NB:, TM:TM + HIST, :]

        def project(fill, n, tmp, slot):
            ops = _rhs2(lambda r, c, dtype: wt(n * 32 + c * 8, r * KQ, KQ, dtype), b1t_v, slot)

            def emit(r, c, v, ref):
                qkv_v[4 * n + c, HIST + r * M:HIST + (r + 1) * M, :] = v
            _strassen2(lambda m: fill.dot(cat(xa2_v, 2 * m, 2), ops(m), NT), t2_v, tmp, emit)

        def first_projection(n, _):
            slab_copy(wqkv_hbm, W_QKV, n + 2).wait()
            pl.when(n < 3)(lambda: slab_copy(wqkv_hbm, W_QKV, n + 3).start())
            pl.when(n < 2)(lambda: slab_copy(wo_hbm, W_O, n).start())

            @pl.when(n == 3)
            def _():
                slab_copy(wg_hbm, W_G, 0).start()
                slab_copy(wu_hbm, W_U, 0).start()
            fill = _Shadow()

            def put(kb, d, v):
                wt_v[64 * (n // 2 + 1) + 2 * d + n % 2, :, lanes(kb)] = v
            reorder(fill, LAST_T, LAG_T, T_MODE[0], range(NB),
                    lambda kb, c: wa_v[n + 2, lanes(kb), lanes(c)].T.astype(F32) if T_MODE[1] else wa_v[n + 2, lanes(kb), lanes(c)].astype(F32).T,
                    put, (gate_wqkv,), (gate_tr,) * T_MODE[2], pin_wt)
            project(fill, n, tg_v, 0)
            fill.finish()
            return 0

        first_window = pltpu.make_async_copy(qk_v.at[:, :AROWS + HIST], qkw_v.at[:2 * NB, :AROWS + HIST],
                                             sem_out.at[5])

        def projection(n, _):
            pl.when(n == 2)(first_window.start)
            fill = _Shadow()

            def put(unit, d, v):
                wo_v[unit[0] * 64 + 2 * d + unit[2], :, lanes(unit[1])] = v
            reorder(fill, 92, LAG_W, 1, [(j, c, s) for j in range(2) for c in range(4) for s in range(2)],
                    lambda unit, k: wa_v[6 + unit[0], lanes(4 * unit[2] + k), lanes(unit[1])].astype(F32),
                    put, (gate_wo,), (gate_tr,), pin_wo)
            project(fill, 2 * n, tg_v, 0)
            project(fill, 2 * n + 1, tu_v, 1)
            fill.finish()
            return 0
        if 'q' not in SKIP:
            lax.fori_loop(0, jnp.where(i == 0, 4, 0), _scoped('first', first_projection), 0)

        @first
        def _():
            for s in range(2):
                slab_copy(wo_hbm, W_O, s).wait()
            before_start(qkv_v, NB)
        if 'v' not in SKIP:
            lax.fori_loop(jnp.where(i == 0, 2, 0), 3, _scoped('proj', projection), 0)

        @first
        def _():
            before_start(qkv_v, 2 * NB)
        first_window.wait()
        following, steps = jnp.minimum(i + 1, NTILE - 1), range(0, MH, RG)
        blocks = [(k, a, r) for k, (a, r) in enumerate((a, r) for r in steps for a in range(4))]

        def gate_up(t, _):
            @first
            def _():
                slab_copy(wg_hbm, W_G, t).wait()
                slab_copy(wu_hbm, W_U, t).wait()

                @pl.when(t + 1 < NQ)
                def _():
                    slab_copy(wg_hbm, W_G, t + 1).start()
                    slab_copy(wu_hbm, W_U, t + 1).start()
                for j in range(2):
                    pl.when(t == 2 * j)(wd_copy(j).start)

                @pl.when(t == 4)
                def _():
                    for k in range(1, NTILE):
                        for j in range(4):
                            x_copy(k, j).start()
            fill = _Shadow(_room(1, 2, *ROOM_G))
            if 'h' not in SKIP:
                fill.add([functools.partial(h_operands, jnp.maximum(t - 1, 0), r, p)
                          for p in (1, 5, 4, 6, 0, 2, 3) for r in range(0, M, RG)], *SPAN_H, (), pin_ha)
            if 'a' not in SKIP:
                base, nxt = [al(jnp.minimum(n * AROWS, TM - AROWS), 32) for n in (t, t + 1)]
                qk, v = qkw_v, vw_v
                fill.add(windows(v_v, vw_v, range(NB), base), *SPAN_W[0], (), pin_vw)
                fill.add(windows(qk_v, qkw_v, range(2 * NB), nxt), *SPAN_W[1], (), pin_qkw)
                o = o_v.at[:, pl.ds(base, AROWS)]
                groups = range(AROWS // AG)
                parts = [range(n, n + AP) for n in range(0, 8, AP)]
                fill.add([functools.partial(scores, qk, n, ws) for n in groups for ws in parts],
                         *SPAN_A[0], (gate_qkw,), pin_s[0])
                fill.add([functools.partial(logits, i * TM + base + n * AG, n * AG, n) for n in groups],
                         *SPAN_A[1], gate_s[0:1], pin_s[1])
                fill.add([functools.partial(exps, n) for n in groups], *SPAN_A[2], gate_s[1:2], pin_s[2])
                fill.add([functools.partial(reciprocals, range(n, n + RB)) for n in range(0, len(groups), RB)],
                         *SPAN_A[3], gate_s[2:3], pin_s[3])
                fill.add([functools.partial(mix, v, o, n, bs) for n in groups for bs in parts],
                         *SPAN_A[4], (gate_s[2], gate_s[3], gate_vw), pin_o)
            g = {}

            def emit_g(r, c, v, ref):
                if ref is None:
                    ref = tg_v.at[20 + 2 * r + c % 2]
                    ref[...] = v
                g[r, c] = ref

            def emit_u(r, c, v, ref):
                hh_v[2 + 4 * r + c] = g[r, c][...] * v
            for k, (w0, tmp, emit) in enumerate(((W_G, tg_v, emit_g), (W_U, tu_v, emit_u))):
                ops = _rhs2(lambda r, c, dtype: w_v[w0 + t, r * KQ:(r + 1) * KQ, lanes(c)].astype(dtype), b1_v, k)
                _strassen2(lambda n: fill.dot(cat(xa2_v, 2 * n, 2), ops(n)), t2_v, tmp, emit)
            fill.finish()
            return 0
        if 'g' not in SKIP:
            lax.fori_loop(0, NQ, _scoped('gate_up', gate_up), 0)

        @first
        def _():
            for j in range(2):
                wd_copy(j).wait()
            for k in range(1, NTILE):
                for j in range(4):
                    x_copy(k, j).wait()

        def down(j, _):
            fill = _Shadow(_room(1 + len(KSPLIT), 1, *ROOM_D))

            if 'l' not in SKIP:
                args = [(following, j * MH, a, r, k) for k, a, r in blocks]
                if LN_MODE == 0:
                    fill.add([functools.partial(layernorm, *x) for x in args], *SPAN_L[2], (gate_x,), pin_tu)
                elif LN_MODE == 1:
                    fill.add([functools.partial(center, *x) for x in args], *SPAN_L[0], (gate_x,), pin_m[1])
                    fill.add([functools.partial(rescale, *x, bs) for x in args for bs in (range(4), range(4, 8))],
                             *SPAN_L[2], (gate_tu, gate_m[1]), pin_tu)
                else:
                    fill.add([functools.partial(row_mean, *x) for x in args], *SPAN_L[0], (gate_x,), pin_m[0])
                    fill.add([functools.partial(row_scale, *x) for x in args],
                             *SPAN_L[1], (gate_x, gate_m[0]), pin_m[1])
                    fill.add([functools.partial(normalize, *x) for x in args],
                             *SPAN_L[2], (gate_x, gate_m[0], gate_m[1]), pin_tu)
                fill.add([functools.partial(x_operands, j, r, kk, p)
                          for r in steps for kk in range(2) for p in range(7)], *SPAN_L[3], (gate_tu,), pin_xa)

            def weights(r, c, dtype):
                down = wd_v[j, :, lanes(r), lanes(c)].astype(dtype).reshape(NQ * 128, 128)
                proj = wo_v[pl.ds(j * 64 + r * 16, 16), :, lanes(c)].astype(dtype).reshape(KQ, 128)
                return jnp.concatenate([down, proj], axis=0)
            ops = _rhs2(weights, b1d_v)

            def prod(n):
                p, q = divmod(n, 7)
                direct = lambda blk: _comb(L_TERMS[q], lambda r, c: _comb(
                    L_TERMS[p], lambda a, b: blk(2 * a + r, 2 * b + c))).astype(BF16)
                parts = [packed(ha_v, n * (NQ - 1) + t) for t in range(NQ - 1)]
                parts.append(direct(lambda a, c: hh_v[2 + 4 * a + c]))
                parts += [direct(lambda a, c: o_v[2 * c + kk, a * M:(a + 1) * M, :]) for kk in range(2)]
                if not KSPLIT:
                    return fill.dot(jnp.concatenate(parts, axis=1), ops(n))
                b, out = ops(n), None
                for k, (lo, hi) in enumerate(zip((0,) + KSPLIT, KSPLIT + (len(parts),))):
                    y = fill.dot(jnp.concatenate(parts[lo:hi], axis=1), b[lo * 128:hi * 128])
                    out = y if out is None else y + t3_v[k - 1, :M]
                    if hi < len(parts):
                        t3_v[k, :M] = out
                return out

            def emit(r, c, v, ref):
                x = x_v[4 * i + r, :, pl.ds(al(j * 512 + c * 128, 128), 128)]
                out_v[2 * i + j, r, :, lanes(c)] = (v + x.astype(F32)).astype(BF16)
                if r % 2 == 1 and c % 2 == 1 - SWAP[(6, 2, 3, 5)[r // 2 * 2 + c // 2]]:
                    out_copy(i, j, r // 2, c // 2).start()
            _strassen2(prod, t2_v, tg_v, emit)
            fill.finish()
            return 0
        if 'd' not in SKIP:
            lax.fori_loop(0, 2, _scoped('down', down), 0)
        return 0

    x_rows = lambda i, j, a, r: x_v.at[4 * i + a, pl.ds(al(j, MQ), MH if r >= MQ else MQ)][r:r + RG, :].astype(F32)

    def row_mean(i, j, a, r, n):
        m1_v[2 + n] = jnp.broadcast_to(jnp.mean(x_rows(i, j, a, r), axis=-1, keepdims=True), (RG, 128))

    def row_scale(i, j, a, r, n):
        xc = x_rows(i, j, a, r) - jnp.tile(m1_v[2 + n], (1, NB))
        m2_v[2 + n] = jnp.broadcast_to(jnp.mean(xc * xc, axis=-1, keepdims=True), (RG, 128))

    def layernorm(i, j, a, r, n):
        x = x_rows(i, j, a, r)
        xc = x - jnp.mean(x, axis=-1, keepdims=True)
        y = xc * lax.rsqrt(jnp.mean(xc * xc, axis=-1, keepdims=True) + 1e-5)
        for b in range(NB):
            tu_v[2 + 4 * a + b // 2, pl.ds((b % 2) * MH + r, RG), :] = y[:, lanes(b)]

    def center(i, j, a, r, n):
        x = x_rows(i, j, a, r)
        xc = x - jnp.mean(x, axis=-1, keepdims=True)
        m2_v[2 + n] = jnp.broadcast_to(jnp.mean(xc * xc, axis=-1, keepdims=True), (RG, 128))
        for b in range(NB):
            tu_v[2 + 4 * a + b // 2, pl.ds((b % 2) * MH + r, RG), :] = xc[:, lanes(b)]

    def rescale(i, j, a, r, n, bs):
        scale = lax.rsqrt(m2_v[2 + n] + 1e-5)
        for b in bs:
            at = (2 + 4 * a + b // 2, pl.ds((b % 2) * MH + r, RG))
            tu_v[at] = tu_v[at] * scale

    def normalize(i, j, a, r, n):
        x, m, scale = x_rows(i, j, a, r), m1_v[2 + n], lax.rsqrt(m2_v[2 + n] + 1e-5)
        for b in range(NB):
            tu_v[2 + 4 * a + b // 2, pl.ds((b % 2) * MH + r, RG), :] = (x[:, lanes(b)] - m) * scale
    m1_v[1, 8:, :] = m2_v[2 + TM // RG, :8, :] = jnp.zeros((8, 128), F32)
    pin_m = [lambda: m1_v[origin() + 1, 8:, :], lambda: m2_v[2 + TM // RG, :8, :]]
    gate_m = [gate_to(ref, lambda: (origin() + 1,)) for ref in (m1_v, m2_v)]
    pin_tu = lambda: tu_v[origin() + 20, :8, :]
    gate_tu = gate_to(tu_v, lambda: (origin() + 1,))

    def start_up(j, _):
        _scoped('xwait', x_copy(0, j).wait)()
        start_next(2 * j)
        for n, (a, r) in enumerate((a, r) for r in range(0, MQ, RG) for a in range(4)):
            row_mean(0, j * MQ, a, r, n)
            row_scale(0, j * MQ, a, r, n)
        _scoped('wwait', wq_copy(j).wait)()
        start_next(2 * j + 1)
        for u in range(4):
            ks = pl.ds(al(j % 2 * 512 + u * 128, 128), 128)
            for c in range(4):
                stash(u, c, wa_v[j // 2, ks, lanes(c)].T.astype(F32))
            rows = pl.ds(al(j * MQ + u * RG, RG), RG)
            stats = [(m1_v[2 + 4 * u + a], lax.rsqrt(m2_v[2 + 4 * u + a] + 1e-5)) for a in range(4)]
            for kk in range(2):
                y = {(a, c): (x_v[a, rows, lanes(2 * c + kk)].astype(F32) - stats[a][0]) * stats[a][1]
                     for a in range(4) for c in range(4)}
                for p in range(7):
                    l1, l2 = _lhs2(lambda a, c: y[a, c], p)
                    for q, v in enumerate(l2):
                        xa2_v[2 * (7 * p + q) + kk, rows, :] = v
            for d in range(DH):
                wt_v[2 * d + j // 2, :, ks] = gather(u, d)
        return 0
    if 'f' not in SKIP:
        lax.fori_loop(0, 4, _scoped('start', start_up), 0)
    lax.fori_loop(0, NTILE, tile, 0)
    pltpu.make_async_copy(o_hbm, o_hbm, sem_out.at[0]).wait()


@jax.jit
def pallas_parallel_sum__sliding_local_dilated__glu_gated_bilinear__prompt_kernel(
        A_x, A_wqkv, A_wo, B_x, B_w_gate, B_w_up, B_w_down):
    B, S, D = A_x.shape
    F = B_w_gate.shape[1]
    NB, NQ, M, NTILE = D // 128, F // 512, TM // 4, S // TM
    groups = _attention_rows(NQ) // AG
    V = pltpu.VMEM
    out = pl.pallas_call(
        _kernel,
        out_shape=jax.ShapeDtypeStruct((NTILE, 4, M, D), BF16),
        in_specs=[pl.BlockSpec(memory_space=pl.ANY)] * 6,
        out_specs=pl.BlockSpec(memory_space=pl.ANY),
        scratch_shapes=[
            V((4 * NTILE + 1, M, D), BF16),
            V((2 * NTILE, 4, M, 512), BF16),
            V((2 * NQ, D, 512), BF16),
            V((9, D, 512), BF16),
            V((6 * 32 + 1, 16, D), BF16),
            V((2 * 64 + 1, 16, 512), BF16),
            V((2, NQ, 512, 512), BF16),
            V((2 + 8, 16 * PITCH, 128), F32),
            V((99, M, 128), BF16), V((49 * (NQ - 1) + 1, M, 128), BF16),
            V((3 * NB, TM + HIST, 128), F32), V((NB + 1, TM, 128), F32),
            V((18, M, 128), F32), V((5, M, 128), F32), V((5, 2 * M, 128), F32),
            V((28, M, 128), F32), V((21, M, 128), F32),
            V((8, D // 4, 128), F32), V((8, 128, D // 4), F32), V((8, NQ * 128 + D // 4, 128), F32),
            V((2 * NB + 1, groups * AG + HIST + PAD, 128), F32), V((NB + 1, groups * AG + HIST + PAD, 128), F32),
            *[V((2 + groups, n, AG, 128), F32) for n in (WIN, WIN + 1, WIN + 1, 1)],
            V((2 + TM // RG, RG, 128), F32), V((3 + TM // RG, RG, 128), F32),
            pltpu.SMEM((1,), jnp.int32),
            pltpu.SemaphoreType.DMA((2 * NQ + 10 + 4 * NTILE,)), pltpu.SemaphoreType.DMA((6,)),
        ],
        compiler_params=pltpu.CompilerParams(vmem_limit_bytes=126 << 20, flags=FLAGS),
    )(A_x.reshape(NTILE, 4, M, D), A_wqkv, A_wo, B_w_gate, B_w_up, B_w_down.reshape(NQ, 512, D))
    return out.reshape(B, S, D)
```

```python
import functools
import math
import jax
import jax.numpy as jnp
from jax import lax
import jax.experimental.pallas as pl
import jax.experimental.pallas.tpu as pltpu

H, WIN, DIL = 32, 8, 2
TM = 1024
RG = 16
AG = 8
HIST = 16
PITCH = 33
STEPS = 8
SKIP = ''
AP, RB, KSPLIT = 2, 4, (4,)
SPAN_H = (0, 88, 5)
SPAN_A = ((0, 50, 5), (6, 64, 8), (14, 72, 6), (31, 80, 5), (50, 92, 5))
SPAN_L = ((0, 68, 4), (6, 74, 4), (12, 80, 3), (26, 94, 3))
LN_MODE = 2
NOCHECK = True
UNROLL = False
T_MODE = (0, 1, 0)
WCUT = 88
PIN_TILE, PIN_SPAN = 0, 6
ROOM_D, ROOM_G = (1.0, 0), (0.6, 4)
LAG_T, LAG_W = (6, 3), (5, 5)
FLAGS = None
SPAN_W = ((0, 37, 4), (51, 90, 4))
AHEAD = 4
PAD = 8
SCOPES = False
LAST_T = 46
F32, BF16 = jnp.float32, jnp.bfloat16
NN = (((1,), (0,)), ((), ()))
NT = (((1,), (1,)), ((), ()))

L_TERMS = (((0, 0), (1, 1), 1), ((1, 0), (1, 1), 1), ((0, 0),), ((1, 1),),
           ((0, 0), (0, 1), 1), ((1, 0), (0, 0), -1), ((0, 1), (1, 1), -1))
R_TERMS = (((0, 0), (1, 1), 1), ((0, 0),), ((0, 1), (1, 1), -1), ((1, 0), (0, 0), -1),
           ((1, 1),), ((0, 0), (0, 1), 1), ((1, 0), (1, 1), 1))
ORDER = (1, 3, 4, 2, 0, 6, 5)
SWAP = (0, 1, 0, 0, 1, 1, 1)


def _comb(term, get):
    if len(term) == 1:
        return get(*term[0])
    a, b = get(*term[0]), get(*term[1])
    return a + b if term[2] > 0 else a - b


def _scoped(name, f):
    def g(*args):
        with jax.named_scope(name):
            return f(*args)
    return g if SCOPES else f


def _attention_rows(steps):
    return pl.cdiv(TM // 32, steps) * 32


def _tree(f, xs):
    return xs[0] if len(xs) == 1 else f(_tree(f, xs[:len(xs) // 2]), _tree(f, xs[len(xs) // 2:]))


class _Shadow:
    def __init__(self, room=None):
        self.room = room
        self.calls, self.tasks, self.zeros, self.late = 0, [], {}, []

    def add(self, fns, first, last, lag, gates, pin):
        for n, fn in enumerate(fns):
            self.tasks.append((self.warp(first + n * (last - first) / len(fns)), fn, lag, gates, pin))
        self.tasks.sort(key=lambda task: task[0])

    def warp(self, at):
        if self.room is None:
            return at
        at *= sum(self.room) / len(self.room)
        for n, room in enumerate(self.room):
            if at < room:
                return n + at / room
            at -= room

    def dot(self, a, b, dims=NN):
        self.late += self.zeros.pop(self.calls, [])
        if self.late and b.dtype == F32:
            rows = [[b[r:r + 8, c:c + 128] for c in range(0, b.shape[1], 128)] for r in range(0, b.shape[0], 8)]
            tiles = b.size // (128 * 128)
            for step, zero in self.late:
                tile = tiles - 1 - (step * PIN_TILE) % tiles
                r, c = (16 * tile, 0) if len(rows[0]) == 1 else (0, tile)
                rows[r + 14 - 2 * (step * PIN_SPAN // STEPS)][c] += zero
            self.late = []
            b = jnp.concatenate([jnp.concatenate(row, axis=1) for row in rows], axis=0)
        out = lax.dot_general(a, b.astype(BF16), dims, preferred_element_type=F32)
        events = []
        while self.tasks and self.tasks[0][0] < self.calls + 1:
            events.append(self.tasks.pop(0))
        for step in range(STEPS):
            group = [task for task in events if int((task[0] - self.calls) * STEPS) == step]
            row = step * out.shape[0] // STEPS
            for gate in {gate: None for task in group for gate in task[3]}:
                gate(out[row:row + 8])
            for task in group:
                task[1]()
            for lag, pin in {(task[2], task[4]): None for task in group if task[4]}:
                self.zeros.setdefault(self.calls + lag, []).append((step, pin()))
        self.calls += 1
        return out

    def finish(self):
        assert not self.tasks


def _level(prod, tmp, emit, keep=None):
    tmp[0] = prod(1)
    c21 = tmp[0] + prod(3)
    emit(1, 0, c21)
    if keep is None:
        tmp[3] = c21
    tmp[1] = prod(4)
    c12 = tmp[1] + prod(2)
    emit(0, 1, c12)
    if keep is None:
        tmp[4] = c12
    tmp[2] = prod(0) - tmp[0] - tmp[1]
    emit(0, 0, (tmp[3] if keep is None else keep(1, 0)) + tmp[2] + prod(6))
    emit(1, 1, (tmp[4] if keep is None else keep(0, 1)) + tmp[2] + prod(5))


def _strassen2(prod, t2, t1, emit):
    def run(p, e, keep=None):
        _level(lambda q: prod(7 * p + q), t2, lambda r, c, v: e(r, c ^ SWAP[p], v),
               keep and (lambda r, c: keep(r, c ^ SWAP[p])))

    def put(i):
        def f(r, c, v):
            t1[4 * i + 2 * r + c] = v
        return f
    get = lambda i, r, c: t1[4 * i + 2 * r + c]

    def c21(r, c, v):
        v = get(0, r, c) + v
        put(3)(r, c, v)
        emit(2 + r, c, v, t1.at[12 + 2 * r + c])

    def c12(r, c, v):
        v = get(1, r, c) + v
        put(4)(r, c, v)
        emit(r, 2 + c, v, t1.at[16 + 2 * r + c])
    run(1, put(0), functools.partial(get, 0))
    run(3, c21)
    run(4, put(1), functools.partial(get, 1))
    run(2, c12)
    run(0, lambda r, c, v: put(2)(r, c, v - get(0, r, c) - get(1, r, c)))
    run(6, lambda r, c, v: emit(r, c, get(3, r, c) + get(2, r, c) + v, None))
    run(5, lambda r, c, v: emit(2 + r, 2 + c, get(4, r, c) + get(2, r, c) + v, None))


def _room(calls, count, busy, shift):
    heavy = [len(R_TERMS[p]) > 1 and k < 4 for p in ORDER for k in range(7)]
    return [busy if heavy[(n + shift) // calls % 49] else 1.0 for n in range(49 * calls * count)]


def _rhs2(w, b1, slot=0):
    slots = {}

    def get(n):
        p, q = divmod(n, 7)
        if len(R_TERMS[p]) == 1:
            a, b = R_TERMS[p][0]
            dtype = BF16 if len(R_TERMS[q]) == 1 else F32
            return _comb(R_TERMS[q], lambda r, c: w(2 * a + r, 2 * b + (c ^ SWAP[p]), dtype))
        if p not in slots:
            slots[p] = 4 * ((slot + len(slots)) % 2)
            for r in range(2):
                for c in range(2):
                    b1[slots[p] + 2 * r + c] = _comb(R_TERMS[p], lambda a, b: w(2 * a + r, 2 * b + c, F32))
        return _comb(R_TERMS[q], lambda r, c: b1[slots[p] + 2 * r + (c ^ SWAP[p])])
    return get


def _lhs2(blk, p):
    l1 = {(r, c): _comb(L_TERMS[p], lambda a, b: blk(2 * a + r, 2 * b + c)) for r in range(2) for c in range(2)}
    return l1, [_comb(L_TERMS[q], lambda r, c: l1[r, c]).astype(BF16) for q in range(7)]


def _kernel(x_hbm, wqkv_hbm, wo_hbm, wg_hbm, wu_hbm, wd_hbm, o_hbm,
            x_v, out_v, w_v, wa_v, wt_v, wo_v, wd_v, tr_v, xa2_v, ha_v, qkv_v, o_v,
            hh_v, t2_v, t3_v, tg_v, tu_v, b1_v, b1t_v, b1d_v, qkw_v, vw_v, s1_v, s2_v, s3_v, s4_v, m1_v, m2_v, opaque, sem_in, sem_out):
    S, D = x_hbm.shape[0] * TM, x_hbm.shape[-1]
    F = wg_hbm.shape[1]
    NTILE, NB, DH, NQ = S // TM, D // 128, D // H, F // 512
    M, KQ = TM // 4, D // 4
    MH, MQ = M // 2, M // 4
    AROWS = _attention_rows(NQ)
    W_G, W_U, W_QKV, W_O = 0, NQ, 2 * NQ, 2 * NQ + 6
    al = pl.multiple_of
    qk_v, v_v = qkv_v.at[:2 * NB], qkv_v.at[2 * NB:]
    lanes = lambda n: slice(n * 128, (n + 1) * 128)

    def slab_copy(src, base, s):
        dst = w_v.at[base + s] if base < W_QKV else wa_v.at[base - W_QKV + s]
        return pltpu.make_async_copy(src.at[:, pl.ds(al(s * 512, 512), 512)], dst, sem_in.at[base + s])

    def wq_copy(n):
        rows = pl.ds(al(n % 2 * 512, 512), 512)
        return pltpu.make_async_copy(wqkv_hbm.at[rows, pl.ds(al(n // 2 * 512, 512), 512)], wa_v.at[n // 2, rows],
                                     sem_out.at[1 + n])

    def wd_copy(j):
        return pltpu.make_async_copy(wd_hbm.at[:, :, pl.ds(j * 512, 512)], wd_v.at[j], sem_in.at[W_O + 2 + j])

    def x_copy(i, j):
        rows = pl.ds(al(j * MQ, MQ), MQ)
        return pltpu.make_async_copy(x_hbm.at[i, :, rows], x_v.at[pl.ds(4 * i, 4), rows],
                                     sem_in.at[W_O + 4 + 4 * i + j])

    def out_copy(i, j, a, b):
        cols = pl.ds(al(j * 512 + b * 256, 256), 256)
        return pltpu.make_async_copy(out_v.at[2 * i + j, pl.ds(2 * a, 2), :, pl.ds(b * 256, 256)],
                                     o_hbm.at[i, pl.ds(2 * a, 2), :, cols], sem_out.at[0])

    early = [x_copy(0, j) for j in range(4)] + [wq_copy(j) for j in range(4)]
    early += [slab_copy(wqkv_hbm, W_QKV, s) for s in range(2, 3)]
    for cp in early[:AHEAD]:
        cp.start()

    def start_next(step):
        for n in range(AHEAD, len(early)):
            pl.when(step == min(n - AHEAD, 7))(early[n].start)

    opaque[0] = 0
    origin = lambda: opaque[0]
    for ref in (o_v.at[NB], tu_v.at[20], tr_v.at[0], s1_v.at[0, 0], s2_v.at[0, 0], s3_v.at[0, 0], s4_v.at[0, 0]):
        ref[:8, :] = jnp.zeros((8, 128), F32)
    for ref in (ha_v.at[49 * (NQ - 1)], xa2_v.at[98], wt_v.at[6 * 32], wo_v.at[2 * 64]):
        ref[:16, :128] = jnp.zeros((16, 128), BF16)
    for ref in (t2_v, t3_v, tg_v, tu_v, b1_v, b1t_v, b1d_v):
        ref[origin(), :8, :128] = jnp.zeros((8, 128), F32)
    pin_ha = lambda: ha_v.bitcast(F32)[49 * (NQ - 1), :8, :]
    pin_xa = lambda: xa2_v.bitcast(F32)[98, :8, :]
    pin_wt = lambda: wt_v[6 * 32, :, :128].astype(F32)[:8]
    pin_wo = lambda: wo_v[origin() + 2 * 64, :, :128].astype(F32)[:8]
    pin_o = lambda: o_v[NB, :8, :]
    pin_hh, pin_tr = [lambda ref=ref: ref[origin(), :8, :] for ref in (hh_v, tr_v)]
    pin_s = [lambda ref=ref: ref[origin(), 0, :8, :] for ref in (s1_v, s2_v, s3_v, s4_v)]

    def gate_to(ref, at):
        def gate(v):
            if ref.dtype == F32:
                ref[at() + (slice(0, 8), slice(0, 128))] = v
            else:
                ref[at() + (slice(0, 16), slice(0, 128))] = jnp.concatenate([v, v], axis=0).astype(BF16)
        return gate
    gate_hh, gate_tr = [gate_to(ref, lambda: (origin() + 1,)) for ref in (hh_v, tr_v)]
    gate_s = [gate_to(ref, lambda: (origin() + 1, 0)) for ref in (s1_v, s2_v, s3_v, s4_v)]
    gate_qkw, gate_vw = gate_to(qkw_v, lambda: (origin() + 2 * NB,)), gate_to(vw_v, lambda: (origin() + NB,))
    pin_qkw, pin_vw = lambda: qkw_v[origin() + 2 * NB, 8:16, :], lambda: vw_v[origin() + NB, 8:16, :]
    qkw_v[2 * NB, 8:16, :] = vw_v[NB, 8:16, :] = jnp.zeros((8, 128), F32)
    gate_x = gate_to(x_v, lambda: (4 * NTILE,))
    gate_wqkv, gate_wo = gate_to(wa_v, lambda: (8,)), gate_to(wa_v, lambda: (origin() + 8,))
    packed = lambda ref, n: pltpu.bitcast(ref.bitcast(F32)[n], BF16)
    cat = lambda ref, lo, n: jnp.concatenate([packed(ref, lo + k) for k in range(n)], axis=1)

    def x_operands(j, r, kk, p):
        rows = pl.ds(al(j * MH + r, RG), RG)
        l1, l2 = _lhs2(lambda a, c: tu_v[2 + 4 * a + c, pl.ds(kk * MH + r, RG), :], p)
        for q, v in enumerate(l2):
            xa2_v[2 * (7 * p + q) + kk, rows, :] = v

    def h_operands(t, r, p):
        for q, v in enumerate(_lhs2(lambda a, c: hh_v[2 + 4 * a + c, r:r + RG, :], p)[1]):
            ha_v[(7 * p + q) * (NQ - 1) + t, r:r + RG, :] = v

    def window(src, dst, b, base, lo, hi):
        dst[b, lo:hi, :] = src.at[:, pl.ds(base, AROWS + HIST)][b, lo:hi, :]

    def windows(src, dst, planes, base):
        cuts = [*range(0, AROWS + HIST, WCUT), AROWS + HIST]
        return [functools.partial(window, src, dst, b, base, lo, hi) for lo, hi in zip(cuts, cuts[1:]) for b in planes]

    def scores(qk, n, ws):
        r0 = n * AG
        qs = [qk[b, pl.ds(r0 + HIST, AG), :] for b in range(NB)]
        for w in ws:
            s1_v[2 + n, w] = _tree(jnp.add, [qs[b] * qk[NB + b, pl.ds(r0 + HIST - DIL * w, AG), :]
                                             for b in range(NB)])

    def logits(pos, may_mask, n):
        ls = []
        for w in range(WIN):
            t = s1_v[2 + n, w]
            t = t + pltpu.roll(t, 64, 1)
            t = t + pltpu.roll(t, 32, 1)
            if may_mask < DIL * w:
                t = jnp.where(pos + lax.broadcasted_iota(jnp.int32, (AG, 128), 0) >= DIL * w, t, -1e9 * DH ** 0.5)
            ls.append(t)
        for w, t in enumerate(ls + [_tree(jnp.maximum, ls)]):
            s2_v[2 + n, w] = t

    def exps(n):
        m = s2_v[2 + n, WIN]
        es = [jnp.exp2((s2_v[2 + n, w] - m) * (DH ** -0.5 * math.log2(math.e))) for w in range(WIN)]
        for w, e in enumerate(es + [_tree(jnp.add, es)]):
            s3_v[2 + n, w] = e

    def reciprocals(ns):
        for n in ns:
            s4_v[2 + n, 0] = 1.0 / s3_v[2 + n, WIN]

    def mix(v, o, n, bs):
        r0 = n * AG
        es = [s3_v[2 + n, w] for w in range(WIN)]
        for b in bs:
            o[b, pl.ds(r0, AG), :] = s4_v[2 + n, 0] * _tree(
                jnp.add, [es[w] * v[b, pl.ds(r0 + HIST - DIL * w, AG), :] for w in range(WIN)])

    def stash(slot, c, v):
        for h in range(4):
            tr_v[2 + slot, pl.ds((4 * c + h) * PITCH, DH), :] = v[h * DH:(h + 1) * DH]

    def gather(slot, d):
        return tr_v[2 + slot, pl.ds(d, 16, stride=PITCH), :].astype(BF16)

    def reorder(shadow, last, lags, spread, units, block, put, gates, gates_tr, pin):
        def spill(n, c):
            stash(n % STASH, c, block(units[n], c))

        def fill(n, d0):
            for d in range(d0, d0 + 8):
                put(units[n], d, gather(n % STASH, d))
        step = (last - lags[0]) / (len(units) + 1)
        assert lags[0] + 2 * step <= STASH * step
        for n in range(len(units)):
            shadow.add([functools.partial(spill, n, c) for c in range(4)], n * step, (n + spread) * step,
                       lags[0], gates, pin_tr if gates_tr else pin_s[0])
            shadow.add([functools.partial(fill, n, 8 * c) for c in range(4)],
                       lags[0] + (n + 1) * step, lags[0] + (n + 2) * step, lags[1], gates_tr, pin)
    STASH = tr_v.shape[0] - 2

    def before_start(ref, base):
        for b in range(base, base + NB):
            ref[b, :HIST, :] = jnp.broadcast_to(ref[b, HIST:HIST + 1, :], (HIST, 128))

    def tile(i, _):
        def first(f):
            pl.when(i == 0)(f)

        def wt(row, k0, kn, dtype):
            return wt_v[pl.ds(row, 8), :, k0:k0 + kn].astype(dtype).reshape(128, kn)

        @pl.when(i > 0)
        def _():
            qkv_v[NB:, :HIST, :] = qkv_v[NB:, TM:TM + HIST, :]

        def project(fill, n, tmp, slot):
            ops = _rhs2(lambda r, c, dtype: wt(n * 32 + c * 8, r * KQ, KQ, dtype), b1t_v, slot)

            def emit(r, c, v, ref):
                qkv_v[4 * n + c, HIST + r * M:HIST + (r + 1) * M, :] = v
                if r == 0:
                    qkw_v[jnp.minimum(4 * n + c, 2 * NB), HIST:HIST + AROWS, :] = v[:AROWS]
            _strassen2(lambda m: fill.dot(cat(xa2_v, 2 * m, 2), ops(m), NT), t2_v, tmp, emit)

        def first_projection(n, _):
            slab_copy(wqkv_hbm, W_QKV, n + 2).wait()
            pl.when(n < 3)(lambda: slab_copy(wqkv_hbm, W_QKV, n + 3).start())
            pl.when(n < 2)(lambda: slab_copy(wo_hbm, W_O, n).start())
            slab_copy(wg_hbm, W_G, n).start()
            pl.when(n > 0)(lambda: slab_copy(wu_hbm, W_U, n - 1).start())
            fill = _Shadow()

            def put(kb, d, v):
                wt_v[64 * (n // 2 + 1) + 2 * d + n % 2, :, lanes(kb)] = v
            reorder(fill, LAST_T, LAG_T, T_MODE[0], range(NB),
                    lambda kb, c: wa_v[n + 2, lanes(kb), lanes(c)].T.astype(F32) if T_MODE[1] else wa_v[n + 2, lanes(kb), lanes(c)].astype(F32).T,
                    put, (gate_wqkv,), (gate_tr,) * T_MODE[2], pin_wt)
            project(fill, n, tg_v, 0)
            fill.finish()
            return 0

        def projection(n, _):
            fill = _Shadow()

            def put(unit, d, v):
                wo_v[unit[0] * 64 + 2 * d + unit[2], :, lanes(unit[1])] = v
            reorder(fill, 92, LAG_W, 1, [(j, c, s) for j in range(2) for c in range(4) for s in range(2)],
                    lambda unit, k: wa_v[6 + unit[0], lanes(4 * unit[2] + k), lanes(unit[1])].astype(F32),
                    put, (gate_wo,), (gate_tr,), pin_wo)
            project(fill, 2 * n, tg_v, 0)
            project(fill, 2 * n + 1, tu_v, 1)
            fill.finish()
            return 0
        if 'q' not in SKIP:
            lax.fori_loop(0, jnp.where(i == 0, 4, 0), _scoped('first', first_projection), 0)

        @first
        def _():
            for s in range(2):
                slab_copy(wo_hbm, W_O, s).wait()
            before_start(qkv_v, NB)
            slab_copy(wu_hbm, W_U, 3).start()
            for t in range(4, NQ):
                slab_copy(wg_hbm, W_G, t).start()
                slab_copy(wu_hbm, W_U, t).start()
        if 'v' not in SKIP:
            lax.fori_loop(jnp.where(i == 0, 2, 0), 3, _scoped('proj', projection), 0)

        @first
        def _():
            before_start(qkv_v, 2 * NB)
            for j in range(2):
                wd_copy(j).start()
            for k in range(1, NTILE):
                for j in range(4):
                    x_copy(k, j).start()
        qkw_v[NB:2 * NB, :HIST, :] = qkv_v[NB:2 * NB, :HIST, :]
        following, steps = jnp.minimum(i + 1, NTILE - 1), range(0, MH, RG)
        blocks = [(k, a, r) for k, (a, r) in enumerate((a, r) for r in steps for a in range(4))]

        def gate_up(t, _):
            @first
            def _():
                slab_copy(wg_hbm, W_G, t).wait()
                slab_copy(wu_hbm, W_U, t).wait()
            fill = _Shadow(_room(1, 2, *ROOM_G))
            if 'h' not in SKIP:
                fill.add([functools.partial(h_operands, jnp.maximum(t - 1, 0), r, p)
                          for p in (1, 5, 4, 6, 0, 2, 3) for r in range(0, M, RG)], *SPAN_H, (), pin_ha)
            if 'a' not in SKIP:
                base, nxt = [al(jnp.minimum(n * AROWS, TM - AROWS), 32) for n in (t, t + 1)]
                qk, v = qkw_v, vw_v
                fill.add(windows(v_v, vw_v, range(NB), base), *SPAN_W[0], (), pin_vw)
                fill.add(windows(qk_v, qkw_v, range(2 * NB), nxt), *SPAN_W[1], (), pin_qkw)
                o = o_v.at[:, pl.ds(base, AROWS)]
                groups = range(AROWS // AG)
                parts = [range(n, n + AP) for n in range(0, 8, AP)]
                fill.add([functools.partial(scores, qk, n, ws) for n in groups for ws in parts],
                         *SPAN_A[0], (gate_qkw,), pin_s[0])
                fill.add([functools.partial(logits, i * TM + base + n * AG, n * AG, n) for n in groups],
                         *SPAN_A[1], gate_s[0:1], pin_s[1])
                fill.add([functools.partial(exps, n) for n in groups], *SPAN_A[2], gate_s[1:2], pin_s[2])
                fill.add([functools.partial(reciprocals, range(n, n + RB)) for n in range(0, len(groups), RB)],
                         *SPAN_A[3], gate_s[2:3], pin_s[3])
                fill.add([functools.partial(mix, v, o, n, bs) for n in groups for bs in parts],
                         *SPAN_A[4], (gate_s[2], gate_s[3], gate_vw), pin_o)
            g = {}

            def emit_g(r, c, v, ref):
                if ref is None:
                    ref = tg_v.at[20 + 2 * r + c % 2]
                    ref[...] = v
                g[r, c] = ref

            def emit_u(r, c, v, ref):
                hh_v[2 + 4 * r + c] = g[r, c][...] * v
            for k, (w0, tmp, emit) in enumerate(((W_G, tg_v, emit_g), (W_U, tu_v, emit_u))):
                ops = _rhs2(lambda r, c, dtype: w_v[w0 + t, r * KQ:(r + 1) * KQ, lanes(c)].astype(dtype), b1_v, k)
                _strassen2(lambda n: fill.dot(cat(xa2_v, 2 * n, 2), ops(n)), t2_v, tmp, emit)
            fill.finish()
            return 0
        if 'g' not in SKIP:
            lax.fori_loop(0, NQ, _scoped('gate_up', gate_up), 0)

        @first
        def _():
            for j in range(2):
                wd_copy(j).wait()
            for k in range(1, NTILE):
                for j in range(4):
                    x_copy(k, j).wait()

        def down(j, _):
            fill = _Shadow(_room(1 + len(KSPLIT), 1, *ROOM_D))

            if 'l' not in SKIP:
                args = [(following, j * MH, a, r, k) for k, a, r in blocks]
                if LN_MODE == 0:
                    fill.add([functools.partial(layernorm, *x) for x in args], *SPAN_L[2], (gate_x,), pin_tu)
                elif LN_MODE == 1:
                    fill.add([functools.partial(center, *x) for x in args], *SPAN_L[0], (gate_x,), pin_m[1])
                    fill.add([functools.partial(rescale, *x, bs) for x in args for bs in (range(4), range(4, 8))],
                             *SPAN_L[2], (gate_tu, gate_m[1]), pin_tu)
                else:
                    fill.add([functools.partial(row_mean, *x) for x in args], *SPAN_L[0], (gate_x,), pin_m[0])
                    fill.add([functools.partial(row_scale, *x) for x in args],
                             *SPAN_L[1], (gate_x, gate_m[0]), pin_m[1])
                    fill.add([functools.partial(normalize, *x) for x in args],
                             *SPAN_L[2], (gate_x, gate_m[0], gate_m[1]), pin_tu)
                fill.add([functools.partial(x_operands, j, r, kk, p)
                          for r in steps for kk in range(2) for p in range(7)], *SPAN_L[3], (gate_tu,), pin_xa)

            def weights(r, c, dtype):
                down = wd_v[j, :, lanes(r), lanes(c)].astype(dtype).reshape(NQ * 128, 128)
                proj = wo_v[pl.ds(j * 64 + r * 16, 16), :, lanes(c)].astype(dtype).reshape(KQ, 128)
                return jnp.concatenate([down, proj], axis=0)
            ops = _rhs2(weights, b1d_v)

            def prod(n):
                p, q = divmod(n, 7)
                direct = lambda blk: _comb(L_TERMS[q], lambda r, c: _comb(
                    L_TERMS[p], lambda a, b: blk(2 * a + r, 2 * b + c))).astype(BF16)
                parts = [packed(ha_v, n * (NQ - 1) + t) for t in range(NQ - 1)]
                parts.append(direct(lambda a, c: hh_v[2 + 4 * a + c]))
                parts += [direct(lambda a, c: o_v[2 * c + kk, a * M:(a + 1) * M, :]) for kk in range(2)]
                if not KSPLIT:
                    return fill.dot(jnp.concatenate(parts, axis=1), ops(n))
                b, out = ops(n), None
                for k, (lo, hi) in enumerate(zip((0,) + KSPLIT, KSPLIT + (len(parts),))):
                    y = fill.dot(jnp.concatenate(parts[lo:hi], axis=1), b[lo * 128:hi * 128])
                    out = y if out is None else y + t3_v[k - 1, :M]
                    if hi < len(parts):
                        t3_v[k, :M] = out
                return out

            def emit(r, c, v, ref):
                x = x_v[4 * i + r, :, pl.ds(al(j * 512 + c * 128, 128), 128)]
                out_v[2 * i + j, r, :, lanes(c)] = (v + x.astype(F32)).astype(BF16)
                if r % 2 == 1 and c % 2 == 1 - SWAP[(6, 2, 3, 5)[r // 2 * 2 + c // 2]]:
                    out_copy(i, j, r // 2, c // 2).start()
            _strassen2(prod, t2_v, tg_v, emit)
            fill.finish()
            return 0
        if 'd' not in SKIP:
            lax.fori_loop(0, 2, _scoped('down', down), 0)
        return 0

    x_rows = lambda i, j, a, r: x_v.at[4 * i + a, pl.ds(al(j, MQ), MH if r >= MQ else MQ)][r:r + RG, :].astype(F32)

    def row_mean(i, j, a, r, n):
        m1_v[2 + n] = jnp.broadcast_to(jnp.mean(x_rows(i, j, a, r), axis=-1, keepdims=True), (RG, 128))

    def row_scale(i, j, a, r, n):
        xc = x_rows(i, j, a, r) - jnp.tile(m1_v[2 + n], (1, NB))
        m2_v[2 + n] = jnp.broadcast_to(jnp.mean(xc * xc, axis=-1, keepdims=True), (RG, 128))

    def layernorm(i, j, a, r, n):
        x = x_rows(i, j, a, r)
        xc = x - jnp.mean(x, axis=-1, keepdims=True)
        y = xc * lax.rsqrt(jnp.mean(xc * xc, axis=-1, keepdims=True) + 1e-5)
        for b in range(NB):
            tu_v[2 + 4 * a + b // 2, pl.ds((b % 2) * MH + r, RG), :] = y[:, lanes(b)]

    def center(i, j, a, r, n):
        x = x_rows(i, j, a, r)
        xc = x - jnp.mean(x, axis=-1, keepdims=True)
        m2_v[2 + n] = jnp.broadcast_to(jnp.mean(xc * xc, axis=-1, keepdims=True), (RG, 128))
        for b in range(NB):
            tu_v[2 + 4 * a + b // 2, pl.ds((b % 2) * MH + r, RG), :] = xc[:, lanes(b)]

    def rescale(i, j, a, r, n, bs):
        scale = lax.rsqrt(m2_v[2 + n] + 1e-5)
        for b in bs:
            at = (2 + 4 * a + b // 2, pl.ds((b % 2) * MH + r, RG))
            tu_v[at] = tu_v[at] * scale

    def normalize(i, j, a, r, n):
        x, m, scale = x_rows(i, j, a, r), m1_v[2 + n], lax.rsqrt(m2_v[2 + n] + 1e-5)
        for b in range(NB):
            tu_v[2 + 4 * a + b // 2, pl.ds((b % 2) * MH + r, RG), :] = (x[:, lanes(b)] - m) * scale
    m1_v[1, 8:, :] = m2_v[2 + TM // RG, :8, :] = jnp.zeros((8, 128), F32)
    pin_m = [lambda: m1_v[origin() + 1, 8:, :], lambda: m2_v[2 + TM // RG, :8, :]]
    gate_m = [gate_to(ref, lambda: (origin() + 1,)) for ref in (m1_v, m2_v)]
    pin_tu = lambda: tu_v[origin() + 20, :8, :]
    gate_tu = gate_to(tu_v, lambda: (origin() + 1,))

    def first_operands(j, _):
        x_copy(0, j).wait()
        start_next(j)
        for n, (a, r) in enumerate((a, r) for r in range(0, MQ, RG) for a in range(4)):
            row_mean(0, j * MQ, a, r, n)
            row_scale(0, j * MQ, a, r, n)

        def operands(u, _):
            rows = pl.ds(al(j * MQ + u * RG, RG), RG)
            stats = [(m1_v[2 + 4 * u + a], lax.rsqrt(m2_v[2 + 4 * u + a] + 1e-5)) for a in range(4)]
            for kk in range(2):
                y = {(a, c): (x_v[a, rows, lanes(2 * c + kk)].astype(F32) - stats[a][0]) * stats[a][1]
                     for a in range(4) for c in range(4)}
                for p in range(7):
                    for q, v in enumerate(_lhs2(lambda a, c: y[a, c], p)[1]):
                        xa2_v[2 * (7 * p + q) + kk, rows, :] = v
            return 0
        lax.fori_loop(0, MQ // RG, operands, 0, unroll=UNROLL)
        return 0

    def first_weights(j, _):
        wq_copy(j).wait()
        start_next(4 + j)
        ks = lambda u: pl.ds(al(j % 2 * 512 + u * 128, 128), 128)
        for u in range(4):
            for c in range(4):
                stash(u, c, wa_v[j // 2, ks(u), lanes(c)].T.astype(F32))
        for u in range(4):
            for d in range(DH):
                wt_v[2 * d + j // 2, :, ks(u)] = gather(u, d)
        return 0
    if 'f' not in SKIP:
        lax.fori_loop(0, 4, _scoped('start', first_operands), 0)
        lax.fori_loop(0, 4, _scoped('start', first_weights), 0)
    lax.fori_loop(0, NTILE, tile, 0)
    pltpu.make_async_copy(o_hbm, o_hbm, sem_out.at[0]).wait()


@jax.jit
def pallas_parallel_sum__sliding_local_dilated__glu_gated_bilinear__prompt_kernel(
        A_x, A_wqkv, A_wo, B_x, B_w_gate, B_w_up, B_w_down):
    B, S, D = A_x.shape
    F = B_w_gate.shape[1]
    NB, NQ, M, NTILE = D // 128, F // 512, TM // 4, S // TM
    groups = _attention_rows(NQ) // AG
    V = pltpu.VMEM
    out = pl.pallas_call(
        _kernel,
        out_shape=jax.ShapeDtypeStruct((NTILE, 4, M, D), BF16),
        in_specs=[pl.BlockSpec(memory_space=pl.ANY)] * 6,
        out_specs=pl.BlockSpec(memory_space=pl.ANY),
        scratch_shapes=[
            V((4 * NTILE + 1, M, D), BF16),
            V((2 * NTILE, 4, M, 512), BF16),
            V((2 * NQ, D, 512), BF16),
            V((9, D, 512), BF16),
            V((6 * 32 + 1, 16, D), BF16),
            V((2 * 64 + 1, 16, 512), BF16),
            V((2, NQ, 512, 512), BF16),
            V((2 + 8, 16 * PITCH, 128), F32),
            V((99, M, 128), BF16), V((49 * (NQ - 1) + 1, M, 128), BF16),
            V((3 * NB, TM + HIST, 128), F32), V((NB + 1, TM, 128), F32),
            V((18, M, 128), F32), V((5, M, 128), F32), V((5, 2 * M, 128), F32),
            V((28, M, 128), F32), V((21, M, 128), F32),
            V((8, D // 4, 128), F32), V((8, 128, D // 4), F32), V((8, NQ * 128 + D // 4, 128), F32),
            V((2 * NB + 1, groups * AG + HIST + PAD, 128), F32), V((NB + 1, groups * AG + HIST + PAD, 128), F32),
            *[V((2 + groups, n, AG, 128), F32) for n in (WIN, WIN + 1, WIN + 1, 1)],
            V((2 + TM // RG, RG, 128), F32), V((3 + TM // RG, RG, 128), F32),
            pltpu.SMEM((1,), jnp.int32),
            pltpu.SemaphoreType.DMA((2 * NQ + 10 + 4 * NTILE,)), pltpu.SemaphoreType.DMA((5,)),
        ],
        compiler_params=pltpu.CompilerParams(vmem_limit_bytes=126 << 20, flags=FLAGS, disable_bounds_checks=NOCHECK),
    )(A_x.reshape(NTILE, 4, M, D), A_wqkv, A_wo, B_w_gate, B_w_up, B_w_down.reshape(NQ, 512, D))
    return out.reshape(B, S, D)
```

```python
import functools
import math
import jax
import jax.numpy as jnp
from jax import lax
import jax.experimental.pallas as pl
import jax.experimental.pallas.tpu as pltpu

H, WIN, DIL = 32, 8, 2
TM = 1024
RG = 16
AG = 8
HIST = 16
PITCH = 33
STEPS = 8
SKIP = ''
AP, RB, KSPLIT = 2, 1, (4,)
SPAN_H = (0, 84, 3)
SPAN_A = ((0, 50, 5), (6, 64, 7), (14, 72, 6), (31, 80, 5), (50, 93, 5))
SPAN_L = ((0, 68, 4), (6, 74, 4), (12, 80, 3), (26, 94, 3))
LN_MODE = 2
KEPT = {4: ((0, 0), (0, 1), (1, 0), (1, 1)), 3: ((0, 0), (1, 0), (1, 1)), 2: ((0, 0), (1, 1)), 1: ((0, 0),), 0: ()}
K_T, K_Q, K_G, K_D = 4, 2, 1, 2
GM = '12345678'
NOCHECK = True
UNROLL = False
T_MODE = (1, 1, 0)
WCUT = 88
PIN_TILE, PIN_SPAN = 0, 6
ROOM_D, ROOM_G = (1.0, 0), (0.54, 5)
LAG_T, LAG_W = (5, 2), (5, 5)
FLAGS = None
SPAN_W = ((0, 37, 4), (58, 94, 4))
AHEAD = 4
PAD = 24
SCOPES = False
LAST_T = 47
FIRST_T = 0
F32, BF16 = jnp.float32, jnp.bfloat16
NN = (((1,), (0,)), ((), ()))
NT = (((1,), (1,)), ((), ()))

L_TERMS = (((0, 0), (1, 1), 1), ((1, 0), (1, 1), 1), ((0, 0),), ((1, 1),),
           ((0, 0), (0, 1), 1), ((1, 0), (0, 0), -1), ((0, 1), (1, 1), -1))
R_TERMS = (((0, 0), (1, 1), 1), ((0, 0),), ((0, 1), (1, 1), -1), ((1, 0), (0, 0), -1),
           ((1, 1),), ((0, 0), (0, 1), 1), ((1, 0), (1, 1), 1))
ORDER = (1, 3, 4, 2, 0, 6, 5)
SWAP = (0, 1, 0, 0, 1, 1, 1)


def _comb(term, get):
    if len(term) == 1:
        return get(*term[0])
    a, b = get(*term[0]), get(*term[1])
    return a + b if term[2] > 0 else a - b


def _scoped(name, f):
    def g(*args):
        with jax.named_scope(name):
            return f(*args)
    return g if SCOPES else f


def _attention_rows(steps):
    return pl.cdiv(TM // 32, steps) * 32


def _tree(f, xs):
    return xs[0] if len(xs) == 1 else f(_tree(f, xs[:len(xs) // 2]), _tree(f, xs[len(xs) // 2:]))


class _Shadow:
    def __init__(self, room=None):
        self.room = room
        self.calls, self.tasks, self.zeros, self.late = 0, [], {}, []

    def add(self, fns, first, last, lag, gates, pin):
        for n, fn in enumerate(fns):
            self.tasks.append((self.warp(first + n * (last - first) / len(fns)), fn, lag, gates, pin))
        self.tasks.sort(key=lambda task: task[0])

    def warp(self, at):
        if self.room is None:
            return at
        at *= sum(self.room) / len(self.room)
        for n, room in enumerate(self.room):
            if at < room:
                return n + at / room
            at -= room

    def dot(self, a, b, dims=NN):
        self.late += self.zeros.pop(self.calls, [])
        if self.late and b.dtype == F32:
            rows = [[b[r:r + 8, c:c + 128] for c in range(0, b.shape[1], 128)] for r in range(0, b.shape[0], 8)]
            tiles = b.size // (128 * 128)
            for step, zero in self.late:
                tile = tiles - 1 - (step * PIN_TILE) % tiles
                r, c = (16 * tile, 0) if len(rows[0]) == 1 else (0, tile)
                rows[r + 14 - 2 * (step * PIN_SPAN // STEPS)][c] += zero
            self.late = []
            b = jnp.concatenate([jnp.concatenate(row, axis=1) for row in rows], axis=0)
        out = lax.dot_general(a, b.astype(BF16), dims, preferred_element_type=F32)
        events = []
        while self.tasks and self.tasks[0][0] < self.calls + 1:
            events.append(self.tasks.pop(0))
        for step in range(STEPS):
            group = [task for task in events if int((task[0] - self.calls) * STEPS) == step]
            row = step * out.shape[0] // STEPS
            for gate in {gate: None for task in group for gate in task[3]}:
                gate(out[row:row + 8])
            for task in group:
                task[1]()
            for lag, pin in {(task[2], task[4]): None for task in group if task[4]}:
                self.zeros.setdefault(self.calls + lag, []).append((step, pin()))
        self.calls += 1
        return out

    def finish(self):
        assert not self.tasks


def _level(prod, tmp, emit, keep=None):
    tmp[0] = prod(1)
    c21 = tmp[0] + prod(3)
    emit(1, 0, c21)
    if keep is None:
        tmp[3] = c21
    tmp[1] = prod(4)
    c12 = tmp[1] + prod(2)
    emit(0, 1, c12)
    if keep is None:
        tmp[4] = c12
    tmp[2] = prod(0) - tmp[0] - tmp[1]
    emit(0, 0, (tmp[3] if keep is None else keep(1, 0)) + tmp[2] + prod(6))
    emit(1, 1, (tmp[4] if keep is None else keep(0, 1)) + tmp[2] + prod(5))


def _strassen2(prod, t2, t1, emit):
    def run(p, e, keep=None):
        _level(lambda q: prod(7 * p + q), t2, lambda r, c, v: e(r, c ^ SWAP[p], v),
               keep and (lambda r, c: keep(r, c ^ SWAP[p])))

    def put(i):
        def f(r, c, v):
            t1[4 * i + 2 * r + c] = v
        return f
    get = lambda i, r, c: t1[4 * i + 2 * r + c]

    def c21(r, c, v):
        v = get(0, r, c) + v
        put(3)(r, c, v)
        emit(2 + r, c, v, t1.at[12 + 2 * r + c])

    def c12(r, c, v):
        v = get(1, r, c) + v
        put(4)(r, c, v)
        emit(r, 2 + c, v, t1.at[16 + 2 * r + c])
    run(1, put(0), functools.partial(get, 0))
    run(3, c21)
    run(4, put(1), functools.partial(get, 1))
    run(2, c12)
    run(0, lambda r, c, v: put(2)(r, c, v - get(0, r, c) - get(1, r, c)))
    run(6, lambda r, c, v: emit(r, c, get(3, r, c) + get(2, r, c) + v, None))
    run(5, lambda r, c, v: emit(2 + r, 2 + c, get(4, r, c) + get(2, r, c) + v, None))


def _room(calls, count, busy, shift):
    heavy = [len(R_TERMS[p]) > 1 and k < 4 for p in ORDER for k in range(7)]
    return [busy if heavy[(n + shift) // calls % 49] else 1.0 for n in range(49 * calls * count)]


def _rhs2(w, b1, slot, kept):
    slots = {}

    def get(n):
        p, q = divmod(n, 7)
        if len(R_TERMS[p]) == 1:
            a, b = R_TERMS[p][0]
            dtype = BF16 if len(R_TERMS[q]) == 1 else F32
            return _comb(R_TERMS[q], lambda r, c: w(2 * a + r, 2 * b + (c ^ SWAP[p]), dtype))
        level1 = lambda r, c: _comb(R_TERMS[p], lambda a, b: w(2 * a + r, 2 * b + (c ^ SWAP[p]), F32))
        if p not in slots:
            slots[p] = 4 * ((slot + len(slots)) % 2)
            for r, c in kept:
                b1[slots[p] + 2 * r + c] = level1(r, c)
        return _comb(R_TERMS[q], lambda r, c: b1[slots[p] + 2 * r + c] if (r, c) in kept else level1(r, c))
    return get


def _lhs2(blk, p):
    l1 = {(r, c): _comb(L_TERMS[p], lambda a, b: blk(2 * a + r, 2 * b + c)) for r in range(2) for c in range(2)}
    return l1, [_comb(L_TERMS[q], lambda r, c: l1[r, c]).astype(BF16) for q in range(7)]


def _kernel(x_hbm, wqkv_hbm, wo_hbm, wg_hbm, wu_hbm, wd_hbm, o_hbm,
            x_v, out_v, w_v, wa_v, wt_v, wo_v, wd_v, tr_v, xa2_v, ha_v, qkv_v, o_v,
            hh_v, t2_v, t3_v, tg_v, tu_v, b1_v, b1t_v, b1d_v, qkw_v, vw_v, s1_v, s2_v, s3_v, s4_v, m1_v, m2_v, opaque, sem_in, sem_out):
    S, D = x_hbm.shape[0] * TM, x_hbm.shape[-1]
    F = wg_hbm.shape[1]
    NTILE, NB, DH, NQ = S // TM, D // 128, D // H, F // 512
    M, KQ = TM // 4, D // 4
    MH, MQ = M // 2, M // 4
    AROWS = _attention_rows(NQ)
    W_G, W_U, W_QKV, W_O = 0, NQ, 2 * NQ, 2 * NQ + 6
    al = pl.multiple_of
    qk_v, v_v = qkv_v.at[:2 * NB], qkv_v.at[2 * NB:]
    lanes = lambda n: slice(n * 128, (n + 1) * 128)

    def slab_copy(src, base, s):
        dst = w_v.at[base + s] if base < W_QKV else wa_v.at[base - W_QKV + s]
        return pltpu.make_async_copy(src.at[:, pl.ds(al(s * 512, 512), 512)], dst, sem_in.at[base + s])

    def wq_copy(n):
        rows = pl.ds(al(n % 2 * 512, 512), 512)
        return pltpu.make_async_copy(wqkv_hbm.at[rows, pl.ds(al(n // 2 * 512, 512), 512)], wa_v.at[n // 2, rows],
                                     sem_out.at[1 + n])

    def wd_copy(j):
        return pltpu.make_async_copy(wd_hbm.at[:, :, pl.ds(j * 512, 512)], wd_v.at[j], sem_in.at[W_O + 2 + j])

    def x_copy(i, j):
        rows = pl.ds(al(j * MQ, MQ), MQ)
        return pltpu.make_async_copy(x_hbm.at[i, :, rows], x_v.at[pl.ds(4 * i, 4), rows],
                                     sem_in.at[W_O + 4 + 4 * i + j])

    def out_copy(i, j, a, b):
        return pltpu.make_async_copy(out_v.at[2 * i + j, a, :, lanes(b)],
                                     o_hbm.at[i, a, :, pl.ds(al(j * 512 + b * 128, 128), 128)], sem_out.at[0])

    early = [x_copy(0, j) for j in range(4)] + [wq_copy(j) for j in range(4)]
    early += [slab_copy(wqkv_hbm, W_QKV, s) for s in range(2, 3)]
    for cp in early[:AHEAD]:
        cp.start()

    def start_next(step):
        for n in range(AHEAD, len(early)):
            pl.when(step == min(n - AHEAD, 7))(early[n].start)

    opaque[0] = 0
    origin = lambda: opaque[0]
    for ref in (o_v.at[NB], tu_v.at[20], tr_v.at[0], s1_v.at[0, 0], s2_v.at[0, 0], s3_v.at[0, 0], s4_v.at[0, 0]):
        ref[:8, :] = jnp.zeros((8, 128), F32)
    for ref in (ha_v.at[49 * (NQ - 1)], xa2_v.at[98], wt_v.at[6 * 32], wo_v.at[2 * 64]):
        ref[:16, :128] = jnp.zeros((16, 128), BF16)
    for ref in (t2_v, t3_v, tg_v, tu_v, b1_v, b1t_v, b1d_v):
        ref[origin(), :8, :128] = jnp.zeros((8, 128), F32)
    pin_ha = lambda: ha_v.bitcast(F32)[49 * (NQ - 1), :8, :]
    pin_xa = lambda: xa2_v.bitcast(F32)[98, :8, :]
    pin_wt = lambda: wt_v[6 * 32, :, :128].astype(F32)[:8]
    pin_wo = lambda: wo_v[origin() + 2 * 64, :, :128].astype(F32)[:8]
    pin_o = lambda: o_v[NB, :8, :]
    pin_hh, pin_tr = [lambda ref=ref: ref[origin(), :8, :] for ref in (hh_v, tr_v)]
    pin_s = [lambda ref=ref: ref[origin(), 0, :8, :] for ref in (s1_v, s2_v, s3_v, s4_v)]

    def gate_to(ref, at):
        def gate(v):
            if ref.dtype == F32:
                ref[at() + (slice(0, 8), slice(0, 128))] = v
            else:
                ref[at() + (slice(0, 16), slice(0, 128))] = jnp.concatenate([v, v], axis=0).astype(BF16)
        return gate
    gate_hh, gate_tr = [gate_to(ref, lambda: (origin() + 1,)) for ref in (hh_v, tr_v)]
    gate_s = [gate_to(ref, lambda: (origin() + 1, 0)) for ref in (s1_v, s2_v, s3_v, s4_v)]
    gate_qkw, gate_vw = gate_to(qkw_v, lambda: (origin() + 2 * NB,)), gate_to(vw_v, lambda: (origin() + NB,))
    pin_qkw, pin_vw = lambda: qkw_v[origin() + 2 * NB, 8:16, :], lambda: vw_v[origin() + NB, 8:16, :]
    qkw_v[2 * NB, 8:16, :] = vw_v[NB, 8:16, :] = jnp.zeros((8, 128), F32)
    gate_x = gate_to(x_v, lambda: (4 * NTILE,))
    gate_wqkv, gate_wo = gate_to(wa_v, lambda: (8,)), gate_to(wa_v, lambda: (origin() + 8,))
    packed = lambda ref, n: pltpu.bitcast(ref.bitcast(F32)[n], BF16)
    cat = lambda ref, lo, n: jnp.concatenate([packed(ref, lo + k) for k in range(n)], axis=1)

    def x_operands(j, r, kk, p):
        rows = pl.ds(al(j * MH + r, RG), RG)
        l1, l2 = _lhs2(lambda a, c: tu_v[2 + 4 * a + c, pl.ds(kk * MH + r, RG), :], p)
        for q, v in enumerate(l2):
            xa2_v[2 * (7 * p + q) + kk, rows, :] = v

    def h_operands(t, r, p):
        for q, v in enumerate(_lhs2(lambda a, c: hh_v[2 + 4 * a + c, r:r + RG, :], p)[1]):
            ha_v[(7 * p + q) * (NQ - 1) + t, r:r + RG, :] = v

    def window(src, dst, b, base, lo, hi):
        dst[b, lo:hi, :] = src.at[:, pl.ds(base, AROWS + HIST)][b, lo:hi, :]

    def windows(src, dst, planes, base):
        cuts = [*range(0, AROWS + HIST, WCUT), AROWS + HIST]
        return [functools.partial(window, src, dst, b, base, lo, hi) for lo, hi in zip(cuts, cuts[1:]) for b in planes]

    def scores(qk, n, ws):
        r0 = n * AG
        qs = [qk[b, pl.ds(r0 + HIST, AG), :] for b in range(NB)]
        for w in ws:
            s1_v[2 + n, w] = _tree(jnp.add, [qs[b] * qk[NB + b, pl.ds(r0 + HIST - DIL * w, AG), :]
                                             for b in range(NB)])

    def logits(pos, may_mask, n):
        ls = []
        for w in range(WIN):
            t = s1_v[2 + n, w]
            t = t + pltpu.roll(t, 64, 1)
            t = t + pltpu.roll(t, 32, 1)
            if may_mask < DIL * w:
                t = jnp.where(pos + lax.broadcasted_iota(jnp.int32, (AG, 128), 0) >= DIL * w, t, -1e9 * DH ** 0.5)
            ls.append(t)
        for w, t in enumerate(ls + [_tree(jnp.maximum, ls)]):
            s2_v[2 + n, w] = t

    def exps(n):
        m = s2_v[2 + n, WIN]
        es = [jnp.exp2((s2_v[2 + n, w] - m) * (DH ** -0.5 * math.log2(math.e))) for w in range(WIN)]
        for w, e in enumerate(es + [_tree(jnp.add, es)]):
            s3_v[2 + n, w] = e

    def reciprocals(ns):
        for n in ns:
            s4_v[2 + n, 0] = 1.0 / s3_v[2 + n, WIN]

    def mix(v, o, n, bs):
        r0 = n * AG
        es = [s3_v[2 + n, w] for w in range(WIN)]
        for b in bs:
            o[b, pl.ds(r0, AG), :] = s4_v[2 + n, 0] * _tree(
                jnp.add, [es[w] * v[b, pl.ds(r0 + HIST - DIL * w, AG), :] for w in range(WIN)])

    def stash(slot, c, v):
        for h in range(4):
            tr_v[2 + slot, pl.ds((4 * c + h) * PITCH, DH), :] = v[h * DH:(h + 1) * DH]

    def gather(slot, d):
        return tr_v[2 + slot, pl.ds(d, 16, stride=PITCH), :].astype(BF16)

    def reorder(shadow, first, last, lags, spread, units, block, put, gates, gates_tr, pin):
        def spill(n, c):
            stash(n % STASH, c, block(units[n], c))

        def fill(n, d0):
            for d in range(d0, d0 + 8):
                put(units[n], d, gather(n % STASH, d))
        step = (last - first - lags[0]) / (len(units) + 1)
        assert lags[0] + 2 * step <= STASH * step
        for n in range(len(units)):
            shadow.add([functools.partial(spill, n, c) for c in range(4)], first + n * step, first + (n + spread) * step,
                       lags[0], gates, pin_tr if gates_tr else pin_s[0])
            shadow.add([functools.partial(fill, n, 8 * c) for c in range(4)],
                       first + lags[0] + (n + 1) * step, first + lags[0] + (n + 2) * step, lags[1], gates_tr, pin)
    STASH = tr_v.shape[0] - 2

    def before_start(ref, base):
        for b in range(base, base + NB):
            ref[b, :HIST, :] = jnp.broadcast_to(ref[b, HIST:HIST + 1, :], (HIST, 128))

    def tile(i, _):
        def first(f):
            pl.when(i == 0)(f)

        def wt(row, k0, kn, dtype):
            return wt_v[pl.ds(row, 8), :, k0:k0 + kn].astype(dtype).reshape(128, kn)

        @pl.when(i > 0)
        def _():
            qkv_v[NB:, :HIST, :] = qkv_v[NB:, TM:TM + HIST, :]

        def project(fill, n, tmp, slot, kept):
            ops = _rhs2(lambda r, c, dtype: wt(n * 32 + c * 8, r * KQ, KQ, dtype), b1t_v, slot, KEPT[kept])

            def emit(r, c, v, ref):
                qkv_v[4 * n + c, HIST + r * M:HIST + (r + 1) * M, :] = v
                if r == 0:
                    qkw_v[jnp.minimum(4 * n + c, 2 * NB), HIST:HIST + AROWS, :] = v[:AROWS]
            _strassen2(lambda m: fill.dot(cat(xa2_v, 2 * m, 2), ops(m), NT), t2_v, tmp, emit)

        def first_projection(n, _):
            if not FIRST_T:
                slab_copy(wqkv_hbm, W_QKV, n + 2).wait()
            pl.when(n < 3)(lambda: slab_copy(wqkv_hbm, W_QKV, n + 3).start())
            pl.when(n < 2)(lambda: slab_copy(wo_hbm, W_O, n).start())
            slab_copy(wg_hbm, W_G, n).start()
            pl.when(n > 0)(lambda: slab_copy(wu_hbm, W_U, n - 1).start())
            fill = _Shadow()

            def put(kb, d, v):
                wt_v[64 * (n // 2 + 1) + 2 * d + n % 2, :, lanes(kb)] = v
            if FIRST_T:
                fill.add([slab_copy(wqkv_hbm, W_QKV, n + 2).wait], FIRST_T - 0.01, FIRST_T, 0, (), None)
            reorder(fill, FIRST_T, LAST_T, LAG_T, T_MODE[0], range(NB),
                    lambda kb, c: wa_v[n + 2, lanes(kb), lanes(c)].T.astype(F32) if T_MODE[1] else wa_v[n + 2, lanes(kb), lanes(c)].astype(F32).T,
                    put, (gate_wqkv,), (gate_tr,) * T_MODE[2], pin_wt)
            project(fill, n, tg_v, 0, K_T)
            fill.finish()
            return 0

        def projection(n, _):
            fill = _Shadow()

            def put(unit, d, v):
                wo_v[unit[0] * 64 + 2 * d + unit[2], :, lanes(unit[1])] = v
            reorder(fill, 0, 92, LAG_W, 1, [(j, c, s) for j in range(2) for c in range(4) for s in range(2)],
                    lambda unit, k: wa_v[6 + unit[0], lanes(4 * unit[2] + k), lanes(unit[1])].astype(F32),
                    put, (gate_wo,), (gate_tr,), pin_wo)
            project(fill, 2 * n, tg_v, 0, K_Q)
            project(fill, 2 * n + 1, tu_v, 1, K_Q)
            fill.finish()
            return 0
        if 'q' not in SKIP:
            lax.fori_loop(0, jnp.where(i == 0, 4, 0), _scoped('first', first_projection), 0)

        @first
        def _():
            for s in range(2):
                slab_copy(wo_hbm, W_O, s).wait()
            before_start(qkv_v, NB)
            slab_copy(wu_hbm, W_U, 3).start()
            for t in range(4, NQ):
                slab_copy(wg_hbm, W_G, t).start()
                slab_copy(wu_hbm, W_U, t).start()
        if 'v' not in SKIP:
            lax.fori_loop(jnp.where(i == 0, 2, 0), 3, _scoped('proj', projection), 0)

        @first
        def _():
            before_start(qkv_v, 2 * NB)
            for j in range(2):
                wd_copy(j).start()
            for k in range(1, NTILE):
                for j in range(4):
                    x_copy(k, j).start()
        qkw_v[NB:2 * NB, :HIST, :] = qkv_v[NB:2 * NB, :HIST, :]
        following, steps = jnp.minimum(i + 1, NTILE - 1), range(0, MH, RG)
        blocks = [(k, a, r) for k, (a, r) in enumerate((a, r) for r in steps for a in range(4))]

        def gate_up(t, _):
            @first
            def _():
                slab_copy(wg_hbm, W_G, t).wait()
                slab_copy(wu_hbm, W_U, t).wait()
            fill = _Shadow(_room(1, 2, *ROOM_G))
            if 'h' not in SKIP:
                fill.add([functools.partial(h_operands, jnp.maximum(t - 1, 0), r, p)
                          for p in (1, 5, 4, 6, 0, 2, 3) for r in range(0, M, RG)], *SPAN_H, (), pin_ha)
            if 'a' not in SKIP:
                base, nxt = [al(jnp.minimum(n * AROWS, TM - AROWS), 32) for n in (t, t + 1)]
                qk, v = qkw_v, vw_v
                fill.add(windows(v_v, vw_v, range(NB), base), *SPAN_W[0], (), pin_vw)
                fill.add(windows(qk_v, qkw_v, range(2 * NB), nxt), *SPAN_W[1], (), pin_qkw)
                o = o_v.at[:, pl.ds(base, AROWS)]
                groups = range(AROWS // AG)
                parts = [range(n, n + AP) for n in range(0, 8, AP)]
                fill.add([functools.partial(scores, qk, n, ws) for n in groups for ws in parts],
                         *SPAN_A[0], (gate_qkw,) * ('1' in GM), pin_s[0])
                fill.add([functools.partial(logits, i * TM + base + n * AG, n * AG, n) for n in groups],
                         *SPAN_A[1], gate_s[0:1] * ('2' in GM), pin_s[1])
                fill.add([functools.partial(exps, n) for n in groups], *SPAN_A[2], gate_s[1:2] * ('3' in GM), pin_s[2])
                fill.add([functools.partial(reciprocals, range(n, n + RB)) for n in range(0, len(groups), RB)],
                         *SPAN_A[3], gate_s[2:3] * ('4' in GM), pin_s[3])
                fill.add([functools.partial(mix, v, o, n, bs) for n in groups for bs in parts],
                         *SPAN_A[4], [g for g, k in zip((gate_s[2], gate_s[3], gate_vw), '567') if k in GM], pin_o)
            g = {}

            def emit_g(r, c, v, ref):
                if ref is None:
                    ref = tg_v.at[20 + 2 * r + c % 2]
                    ref[...] = v
                g[r, c] = ref

            def emit_u(r, c, v, ref):
                hh_v[2 + 4 * r + c] = g[r, c][...] * v
            for k, (w0, tmp, emit) in enumerate(((W_G, tg_v, emit_g), (W_U, tu_v, emit_u))):
                ops = _rhs2(lambda r, c, dtype: w_v[w0 + t, r * KQ:(r + 1) * KQ, lanes(c)].astype(dtype), b1_v, k, KEPT[K_G])
                _strassen2(lambda n: fill.dot(cat(xa2_v, 2 * n, 2), ops(n)), t2_v, tmp, emit)
            fill.finish()
            return 0
        if 'g' not in SKIP:
            lax.fori_loop(0, NQ, _scoped('gate_up', gate_up), 0)

        @first
        def _():
            for j in range(2):
                wd_copy(j).wait()
            for k in range(1, NTILE):
                for j in range(4):
                    x_copy(k, j).wait()

        def down(j, _):
            fill = _Shadow(_room(1 + len(KSPLIT), 1, *ROOM_D))

            if 'l' not in SKIP:
                args = [(following, j * MH, a, r, k) for k, a, r in blocks]
                if LN_MODE == 0:
                    fill.add([functools.partial(layernorm, *x) for x in args], *SPAN_L[2], (gate_x,), pin_tu)
                elif LN_MODE == 1:
                    fill.add([functools.partial(center, *x) for x in args], *SPAN_L[0], (gate_x,), pin_m[1])
                    fill.add([functools.partial(rescale, *x, bs) for x in args for bs in (range(4), range(4, 8))],
                             *SPAN_L[2], (gate_tu, gate_m[1]), pin_tu)
                else:
                    fill.add([functools.partial(row_mean, *x) for x in args], *SPAN_L[0], (gate_x,), pin_m[0])
                    fill.add([functools.partial(row_scale, *x) for x in args],
                             *SPAN_L[1], (gate_x, gate_m[0]), pin_m[1])
                    fill.add([functools.partial(normalize, *x) for x in args],
                             *SPAN_L[2], (gate_x, gate_m[0], gate_m[1]), pin_tu)
                fill.add([functools.partial(x_operands, j, r, kk, p)
                          for r in steps for kk in range(2) for p in range(7)], *SPAN_L[3], (gate_tu,), pin_xa)

            def weights(r, c, dtype):
                down = wd_v[j, :, lanes(r), lanes(c)].astype(dtype).reshape(NQ * 128, 128)
                proj = wo_v[pl.ds(j * 64 + r * 16, 16), :, lanes(c)].astype(dtype).reshape(KQ, 128)
                return jnp.concatenate([down, proj], axis=0)
            ops = _rhs2(weights, b1d_v, 0, KEPT[K_D])

            def prod(n):
                p, q = divmod(n, 7)
                direct = lambda blk: _comb(L_TERMS[q], lambda r, c: _comb(
                    L_TERMS[p], lambda a, b: blk(2 * a + r, 2 * b + c))).astype(BF16)
                parts = [packed(ha_v, n * (NQ - 1) + t) for t in range(NQ - 1)]
                parts.append(direct(lambda a, c: hh_v[2 + 4 * a + c]))
                parts += [direct(lambda a, c: o_v[2 * c + kk, a * M:(a + 1) * M, :]) for kk in range(2)]
                if not KSPLIT:
                    return fill.dot(jnp.concatenate(parts, axis=1), ops(n))
                b, out = ops(n), None
                for k, (lo, hi) in enumerate(zip((0,) + KSPLIT, KSPLIT + (len(parts),))):
                    y = fill.dot(jnp.concatenate(parts[lo:hi], axis=1), b[lo * 128:hi * 128])
                    out = y if out is None else y + t3_v[k - 1, :M]
                    if hi < len(parts):
                        t3_v[k, :M] = out
                return out

            def emit(r, c, v, ref):
                x = x_v[4 * i + r, :, pl.ds(al(j * 512 + c * 128, 128), 128)]
                out_v[2 * i + j, r, :, lanes(c)] = (v + x.astype(F32)).astype(BF16)
                out_copy(i, j, r, c).start()
            _strassen2(prod, t2_v, tg_v, emit)
            fill.finish()
            return 0
        if 'd' not in SKIP:
            lax.fori_loop(0, 2, _scoped('down', down), 0)
        return 0

    x_rows = lambda i, j, a, r: x_v.at[4 * i + a, pl.ds(al(j, MQ), MH if r >= MQ else MQ)][r:r + RG, :].astype(F32)

    def row_mean(i, j, a, r, n):
        m1_v[2 + n] = jnp.broadcast_to(jnp.mean(x_rows(i, j, a, r), axis=-1, keepdims=True), (RG, 128))

    def row_scale(i, j, a, r, n):
        xc = x_rows(i, j, a, r) - jnp.tile(m1_v[2 + n], (1, NB))
        m2_v[2 + n] = jnp.broadcast_to(jnp.mean(xc * xc, axis=-1, keepdims=True), (RG, 128))

    def layernorm(i, j, a, r, n):
        x = x_rows(i, j, a, r)
        xc = x - jnp.mean(x, axis=-1, keepdims=True)
        y = xc * lax.rsqrt(jnp.mean(xc * xc, axis=-1, keepdims=True) + 1e-5)
        for b in range(NB):
            tu_v[2 + 4 * a + b // 2, pl.ds((b % 2) * MH + r, RG), :] = y[:, lanes(b)]

    def center(i, j, a, r, n):
        x = x_rows(i, j, a, r)
        xc = x - jnp.mean(x, axis=-1, keepdims=True)
        m2_v[2 + n] = jnp.broadcast_to(jnp.mean(xc * xc, axis=-1, keepdims=True), (RG, 128))
        for b in range(NB):
            tu_v[2 + 4 * a + b // 2, pl.ds((b % 2) * MH + r, RG), :] = xc[:, lanes(b)]

    def rescale(i, j, a, r, n, bs):
        scale = lax.rsqrt(m2_v[2 + n] + 1e-5)
        for b in bs:
            at = (2 + 4 * a + b // 2, pl.ds((b % 2) * MH + r, RG))
            tu_v[at] = tu_v[at] * scale

    def normalize(i, j, a, r, n):
        x, m, scale = x_rows(i, j, a, r), m1_v[2 + n], lax.rsqrt(m2_v[2 + n] + 1e-5)
        for b in range(NB):
            tu_v[2 + 4 * a + b // 2, pl.ds((b % 2) * MH + r, RG), :] = (x[:, lanes(b)] - m) * scale
    m1_v[1, 8:, :] = m2_v[2 + TM // RG, :8, :] = jnp.zeros((8, 128), F32)
    pin_m = [lambda: m1_v[origin() + 1, 8:, :], lambda: m2_v[2 + TM // RG, :8, :]]
    gate_m = [gate_to(ref, lambda: (origin() + 1,)) for ref in (m1_v, m2_v)]
    pin_tu = lambda: tu_v[origin() + 20, :8, :]
    gate_tu = gate_to(tu_v, lambda: (origin() + 1,))

    def first_operands(j, _):
        x_copy(0, j).wait()
        start_next(j)
        for n, (a, r) in enumerate((a, r) for r in range(0, MQ, RG) for a in range(4)):
            row_mean(0, j * MQ, a, r, n)
            row_scale(0, j * MQ, a, r, n)

        def operands(u, _):
            rows = pl.ds(al(j * MQ + u * RG, RG), RG)
            stats = [(m1_v[2 + 4 * u + a], lax.rsqrt(m2_v[2 + 4 * u + a] + 1e-5)) for a in range(4)]
            for kk in range(2):
                y = {(a, c): (x_v[a, rows, lanes(2 * c + kk)].astype(F32) - stats[a][0]) * stats[a][1]
                     for a in range(4) for c in range(4)}
                for p in range(7):
                    for q, v in enumerate(_lhs2(lambda a, c: y[a, c], p)[1]):
                        xa2_v[2 * (7 * p + q) + kk, rows, :] = v
            return 0
        lax.fori_loop(0, MQ // RG, operands, 0, unroll=UNROLL)
        return 0

    def first_weights(j, _):
        wq_copy(j).wait()
        start_next(4 + j)
        ks = lambda u: pl.ds(al(j % 2 * 512 + u * 128, 128), 128)
        for u in range(4):
            for c in range(4):
                stash(u, c, wa_v[j // 2, ks(u), lanes(c)].T.astype(F32))
        for u in range(4):
            for d in range(DH):
                wt_v[2 * d + j // 2, :, ks(u)] = gather(u, d)
        return 0
    if 'f' not in SKIP:
        lax.fori_loop(0, 4, _scoped('start', first_operands), 0)
        lax.fori_loop(0, 4, _scoped('start', first_weights), 0)
    lax.fori_loop(0, NTILE, tile, 0)
    pltpu.make_async_copy(o_hbm, o_hbm, sem_out.at[0]).wait()


@jax.jit
def pallas_parallel_sum__sliding_local_dilated__glu_gated_bilinear__prompt_kernel(
        A_x, A_wqkv, A_wo, B_x, B_w_gate, B_w_up, B_w_down):
    B, S, D = A_x.shape
    F = B_w_gate.shape[1]
    NB, NQ, M, NTILE = D // 128, F // 512, TM // 4, S // TM
    groups = _attention_rows(NQ) // AG
    V = pltpu.VMEM
    out = pl.pallas_call(
        _kernel,
        out_shape=jax.ShapeDtypeStruct((NTILE, 4, M, D), BF16),
        in_specs=[pl.BlockSpec(memory_space=pl.ANY)] * 6,
        out_specs=pl.BlockSpec(memory_space=pl.ANY),
        scratch_shapes=[
            V((4 * NTILE + 1, M, D), BF16),
            V((2 * NTILE, 4, M, 512), BF16),
            V((2 * NQ, D, 512), BF16),
            V((9, D, 512), BF16),
            V((6 * 32 + 1, 16, D), BF16),
            V((2 * 64 + 1, 16, 512), BF16),
            V((2, NQ, 512, 512), BF16),
            V((2 + 8, 16 * PITCH, 128), F32),
            V((99, M, 128), BF16), V((49 * (NQ - 1) + 1, M, 128), BF16),
            V((3 * NB, TM + HIST, 128), F32), V((NB + 1, TM, 128), F32),
            V((18, M, 128), F32), V((5, M, 128), F32), V((5, 2 * M, 128), F32),
            V((28, M, 128), F32), V((21, M, 128), F32),
            V((8, D // 4, 128), F32), V((8, 128, D // 4), F32), V((8, NQ * 128 + D // 4, 128), F32),
            V((2 * NB + 1, groups * AG + HIST + PAD, 128), F32), V((NB + 1, groups * AG + HIST + PAD, 128), F32),
            *[V((2 + groups, n, AG, 128), F32) for n in (WIN, WIN + 1, WIN + 1, 1)],
            V((2 + TM // RG, RG, 128), F32), V((3 + TM // RG, RG, 128), F32),
            pltpu.SMEM((1,), jnp.int32),
            pltpu.SemaphoreType.DMA((2 * NQ + 10 + 4 * NTILE,)), pltpu.SemaphoreType.DMA((5,)),
        ],
        compiler_params=pltpu.CompilerParams(vmem_limit_bytes=126 << 20, flags=FLAGS, disable_bounds_checks=NOCHECK),
    )(A_x.reshape(NTILE, 4, M, D), A_wqkv, A_wo, B_w_gate, B_w_up, B_w_down.reshape(NQ, 512, D))
    return out.reshape(B, S, D)
```

```python
import functools
import math

import jax
import jax.numpy as jnp
from jax import lax
import jax.experimental.pallas as pl
import jax.experimental.pallas.tpu as pltpu

H, WIN, DIL = 32, 8, 2
TM = 1024
RG = 16
AG = 8
HIST = 16
PITCH = 33
STASH = 8
F32, BF16 = jnp.float32, jnp.bfloat16
NN = (((1,), (0,)), ((), ()))
NT = (((1,), (1,)), ((), ()))

STEPS, PIN_SPAN, PAD, WCUT, AHEAD = 8, 6, 24, 88, 3
SPAN_H = (0, 84, 3)
SPAN_A = ((0, 50, 5), (6, 64, 7), (14, 72, 6), (31, 80, 5), (50, 93, 5))
SPAN_W = ((0, 37, 4), (58, 94, 4))
SPAN_L = ((0, 68, 4), (6, 74, 4), (12, 80, 3), (26, 94, 3))
START_L = ((2, 3.5, 3), (5, 6.5, 3), (0, 4, 2), (1, 7.9, 2))
START_T, FIRST_T, PROJ_T = (0, 7, (1.5, 3), 0), (0, 47, (5, 2), 1), (0, 92, (5, 5), 1)
ROOM_G = (0.54, 5)
K_T, K_Q, K_G, K_D = 4, 2, 1, 2

L_TERMS = (((0, 0), (1, 1), 1), ((1, 0), (1, 1), 1), ((0, 0),), ((1, 1),),
           ((0, 0), (0, 1), 1), ((1, 0), (0, 0), -1), ((0, 1), (1, 1), -1))
R_TERMS = (((0, 0), (1, 1), 1), ((0, 0),), ((0, 1), (1, 1), -1), ((1, 0), (0, 0), -1),
           ((1, 1),), ((0, 0), (0, 1), 1), ((1, 0), (1, 1), 1))
ORDER = (1, 3, 4, 2, 0, 6, 5)
SWAP = (0, 1, 0, 0, 1, 1, 1)


def _comb(term, get):
    if len(term) == 1:
        return get(*term[0])
    a, b = get(*term[0]), get(*term[1])
    return a + b if term[2] > 0 else a - b


def _tree(f, xs):
    return xs[0] if len(xs) == 1 else f(_tree(f, xs[:len(xs) // 2]), _tree(f, xs[len(xs) // 2:]))


def _lanes(n):
    return slice(n * 128, (n + 1) * 128)


def _attention_rows(steps):
    return pl.cdiv(TM // 32, steps) * 32


class _Shadow:
    def __init__(self, room=None):
        self.room, self.calls, self.tasks, self.zeros, self.late = room, 0, [], {}, []

    def add(self, fns, first, last, lag, gates, pin):
        for n, fn in enumerate(fns):
            self.tasks.append((self.warp(first + n * (last - first) / len(fns)), fn, lag, gates, pin))
        self.tasks.sort(key=lambda task: task[0])

    def warp(self, at):
        if self.room is None:
            return at
        at *= sum(self.room) / len(self.room)
        for n, room in enumerate(self.room):
            if at < room:
                return n + at / room
            at -= room

    def dot(self, a, b, dims=NN):
        self.late += self.zeros.pop(self.calls, [])
        if self.late and b.dtype == F32:
            rows = [[b[r:r + 8, _lanes(c)] for c in range(b.shape[1] // 128)] for r in range(0, b.shape[0], 8)]
            for step, zero in self.late:
                rows[-2 - 2 * (step * PIN_SPAN // STEPS)][-1] += zero
            self.late = []
            b = jnp.concatenate([jnp.concatenate(row, axis=1) for row in rows], axis=0)
        out = lax.dot_general(a, b.astype(BF16), dims, preferred_element_type=F32)
        events = []
        while self.tasks and self.tasks[0][0] < self.calls + 1:
            events.append(self.tasks.pop(0))
        for step in range(STEPS):
            group = [task for task in events if int((task[0] - self.calls) * STEPS) == step]
            row = step * out.shape[0] // STEPS
            for gate in {gate: None for task in group for gate in task[3]}:
                gate(out[row:row + 8])
            for task in group:
                task[1]()
            for lag, pin in {(task[2], task[4]): None for task in group}:
                self.zeros.setdefault(self.calls + lag, []).append((step, pin()))
        self.calls += 1
        return out

    def finish(self):
        assert not self.tasks


def _level(prod, tmp, emit, keep=None):
    tmp[0] = prod(1)
    c21 = tmp[0] + prod(3)
    emit(1, 0, c21)
    if keep is None:
        tmp[3] = c21
    tmp[1] = prod(4)
    c12 = tmp[1] + prod(2)
    emit(0, 1, c12)
    if keep is None:
        tmp[4] = c12
    tmp[2] = prod(0) - tmp[0] - tmp[1]
    emit(0, 0, (tmp[3] if keep is None else keep(1, 0)) + tmp[2] + prod(6))
    emit(1, 1, (tmp[4] if keep is None else keep(0, 1)) + tmp[2] + prod(5))


def _strassen2(prod, t2, t1, emit):
    def run(p, e, keep=None):
        _level(lambda q: prod(7 * p + q), t2, lambda r, c, v: e(r, c ^ SWAP[p], v),
               keep and (lambda r, c: keep(r, c ^ SWAP[p])))

    def get(i, r, c):
        return t1[4 * i + 2 * r + c]

    def put(i, r, c, v):
        t1[4 * i + 2 * r + c] = v

    def c21(r, c, v):
        v = get(0, r, c) + v
        put(3, r, c, v)
        emit(2 + r, c, v, t1.at[12 + 2 * r + c])

    def c12(r, c, v):
        v = get(1, r, c) + v
        put(4, r, c, v)
        emit(r, 2 + c, v, t1.at[16 + 2 * r + c])
    run(1, functools.partial(put, 0), functools.partial(get, 0))
    run(3, c21)
    run(4, functools.partial(put, 1), functools.partial(get, 1))
    run(2, c12)
    run(0, lambda r, c, v: put(2, r, c, v - get(0, r, c) - get(1, r, c)))
    run(6, lambda r, c, v: emit(r, c, get(3, r, c) + get(2, r, c) + v, None))
    run(5, lambda r, c, v: emit(2 + r, 2 + c, get(4, r, c) + get(2, r, c) + v, None))


def _right_operands(w, b1, slot, keep):
    slots, kept = {}, sorted(((0, 0), (1, 1), (1, 0), (0, 1))[:keep])

    def get(n):
        p, q = divmod(n, 7)
        if len(R_TERMS[p]) == 1:
            a, b = R_TERMS[p][0]
            dtype = BF16 if len(R_TERMS[q]) == 1 else F32
            return _comb(R_TERMS[q], lambda r, c: w(2 * a + r, 2 * b + (c ^ SWAP[p]), dtype))
        level1 = lambda r, c: _comb(R_TERMS[p], lambda a, b: w(2 * a + r, 2 * b + (c ^ SWAP[p]), F32))
        if p not in slots:
            slots[p] = 4 * ((slot + len(slots)) % 2)
            for r, c in kept:
                b1[slots[p] + 2 * r + c] = level1(r, c)
        return _comb(R_TERMS[q], lambda r, c: b1[slots[p] + 2 * r + c] if (r, c) in kept else level1(r, c))
    return get


def _left_operands(blk, p):
    l1 = {(r, c): _comb(L_TERMS[p], lambda a, b: blk(2 * a + r, 2 * b + c)) for r in range(2) for c in range(2)}
    return [_comb(L_TERMS[q], lambda r, c: l1[r, c]).astype(BF16) for q in range(7)]


def _kernel(x_hbm, wqkv_hbm, wo_hbm, wg_hbm, wu_hbm, wd_hbm, o_hbm,
            x_v, out_v, w_v, wa_v, wt_v, wo_v, wd_v, tr_v, xa_v, ha_v, qkv_v, o_v, hh_v, t2_v, t3_v, tg_v, tu_v,
            b1_v, b1t_v, b1d_v, qkw_v, vw_v, s1_v, s2_v, s3_v, s4_v, m1_v, m2_v, opaque, sems):
    NTILE, D, NQ = x_hbm.shape[0], x_hbm.shape[-1], wg_hbm.shape[1] // 512
    NB, DH = D // 128, D // H
    M, KQ = TM // 4, D // 4
    MH, MQ = M // 2, M // 4
    AROWS = _attention_rows(NQ)
    al, partial = pl.multiple_of, functools.partial

    def slab_copy(src, dst, s, sem):
        return pltpu.make_async_copy(src.at[:, pl.ds(al(s * 512, 512), 512)], dst, sems.at[sem])
    wg_copy = lambda t: slab_copy(wg_hbm, w_v.at[t], t, t)
    wu_copy = lambda t: slab_copy(wu_hbm, w_v.at[NQ + t], t, t)
    wqkv_copy = lambda s: slab_copy(wqkv_hbm, wa_v.at[s], s, NQ + s % 2)
    wo_copy = lambda s: slab_copy(wo_hbm, wa_v.at[6 + s], s, NQ + 2)
    late_copies = [pltpu.make_async_copy(wd_hbm.at[:, :, pl.ds(j * 512, 512)], wd_v.at[j], sems.at[NQ + 3])
                   for j in range(2)]
    late_copies += [pltpu.make_async_copy(x_hbm.at[i], x_v.at[4 * i:4 * i + 4], sems.at[NQ + 3])
                    for i in range(1, NTILE)]

    def x_copy(j):
        rows = pl.ds(al(j * MQ, MQ), MQ)
        return pltpu.make_async_copy(x_hbm.at[0, :, rows], x_v.at[:4, rows], sems.at[NQ + 4 + j])

    def wq_copy(n):
        rows = pl.ds(al(n % 2 * 512, 512), 512)
        return pltpu.make_async_copy(wqkv_hbm.at[rows, pl.ds(al(n // 2 * 512, 512), 512)], wa_v.at[n // 2, rows],
                                     sems.at[n])

    def wk_copy(n):
        rows = pl.ds(al(n * 256, 256), 256)
        return pltpu.make_async_copy(wqkv_hbm.at[rows, pl.ds(D, 512)], wa_v.at[2, rows], sems.at[NQ + 9 + n])

    def out_copy(i, j, r, c):
        return pltpu.make_async_copy(out_v.at[2 * i + j, r, :, _lanes(c)],
                                     o_hbm.at[i, r, :, pl.ds(al(j * 512 + c * 128, 128), 128)], sems.at[NQ + 8])

    early = [[x_copy(0)]] + [[wq_copy(j)] for j in range(4)] + [[x_copy(j + 1), wk_copy(j)] for j in range(3)]
    early += [[wk_copy(3), wqkv_copy(3)]]

    def start_early(n):
        for cp in early[n]:
            cp.start()

    def start_next(step):
        for n in range(AHEAD + 1, len(early)):
            pl.when(step == n - AHEAD)(partial(start_early, n))
    for n in range(AHEAD):
        start_early(n)

    opaque[0] = 0
    origin = lambda: opaque[0]
    for ref in (o_v.at[NB], tu_v.at[20], tr_v.at[0], s1_v.at[0, 0], s2_v.at[0, 0], s3_v.at[0, 0], s4_v.at[0, 0],
                m2_v.at[2 + TM // RG]):
        ref[:8, :] = jnp.zeros((8, 128), F32)
    for ref in (qkw_v.at[2 * NB], vw_v.at[NB], m1_v.at[1]):
        ref[8:16, :] = jnp.zeros((8, 128), F32)
    for ref in (ha_v.at[49 * (NQ - 1)], xa_v.at[98], wt_v.at[6 * DH], wo_v.at[4 * DH]):
        ref[:16, :128] = jnp.zeros((16, 128), BF16)
    for ref in (t2_v, t3_v, tg_v, tu_v, b1_v, b1t_v, b1d_v):
        ref[origin(), :8, :128] = jnp.zeros((8, 128), F32)
    pin_ha = lambda: ha_v.bitcast(F32)[49 * (NQ - 1), :8, :]
    pin_xa = lambda: xa_v.bitcast(F32)[98, :8, :]
    pin_wt = lambda: wt_v[6 * DH, :, :128].astype(F32)[:8]
    pin_wo = lambda: wo_v[origin() + 4 * DH, :, :128].astype(F32)[:8]
    pin_o = lambda: o_v[NB, :8, :]
    pin_tr = lambda: tr_v[origin(), :8, :]
    pin_tu = lambda: tu_v[origin() + 20, :8, :]
    pin_qkw = lambda: qkw_v[origin() + 2 * NB, 8:16, :]
    pin_vw = lambda: vw_v[origin() + NB, 8:16, :]
    pin_m = [lambda: m1_v[origin() + 1, 8:16, :], lambda: m2_v[2 + TM // RG, :8, :]]
    pin_s = [lambda ref=ref: ref[origin(), 0, :8, :] for ref in (s1_v, s2_v, s3_v, s4_v)]

    def gate_to(ref, at):
        def gate(v):
            if ref.dtype == F32:
                ref[at() + (slice(0, 8), slice(0, 128))] = v
            else:
                ref[at() + (slice(0, 16), slice(0, 128))] = jnp.concatenate([v, v], axis=0).astype(BF16)
        return gate
    gate_tr, gate_tu, *gate_m = [gate_to(ref, lambda: (origin() + 1,)) for ref in (tr_v, tu_v, m1_v, m2_v)]
    gate_s = [gate_to(ref, lambda: (origin() + 1, 0)) for ref in (s1_v, s2_v, s3_v, s4_v)]
    gate_qkw, gate_vw = gate_to(qkw_v, lambda: (origin() + 2 * NB,)), gate_to(vw_v, lambda: (origin() + NB,))
    gate_x = gate_to(x_v, lambda: (4 * NTILE,))
    gate_wqkv, gate_wo = gate_to(wa_v, lambda: (8,)), gate_to(wa_v, lambda: (origin() + 8,))

    packed = lambda ref, n: pltpu.bitcast(ref.bitcast(F32)[n], BF16)
    cat = lambda ref, lo, n: jnp.concatenate([packed(ref, lo + k) for k in range(n)], axis=1)

    def x_rows(i, base, a, r):
        return x_v.at[4 * i + a, pl.ds(al(base, RG), r + RG)][r:r + RG, :].astype(F32)

    def row_mean(i, base, a, r, n):
        m1_v[2 + n] = jnp.broadcast_to(jnp.mean(x_rows(i, base, a, r), axis=-1, keepdims=True), (RG, 128))

    def row_var(i, base, a, r, n):
        xc = x_rows(i, base, a, r) - jnp.tile(m1_v[2 + n], (1, NB))
        m2_v[2 + n] = jnp.broadcast_to(jnp.mean(xc * xc, axis=-1, keepdims=True), (RG, 128))

    def normalize(i, base, a, r, n, plain=False):
        x, mean, scale = x_rows(i, base, a, r), m1_v[2 + n], lax.rsqrt(m2_v[2 + n] + 1e-5)
        for b in range(NB):
            y = (x[:, _lanes(b)] - mean) * scale
            if plain:
                ha_v[b, a * MQ + r:a * MQ + r + RG, :] = y.astype(BF16)
            else:
                tu_v[2 + 4 * a + b // 2, pl.ds((b % 2) * MH + r, RG), :] = y

    def x_operands(base, r, kk, p):
        rows = pl.ds(al(base + r, RG), RG)
        for q, v in enumerate(_left_operands(lambda a, c: tu_v[2 + 4 * a + c, pl.ds(kk * MH + r, RG), :], p)):
            xa_v[2 * (7 * p + q) + kk, rows, :] = v

    def h_operands(t, r, p):
        for q, v in enumerate(_left_operands(lambda a, c: hh_v[2 + 4 * a + c, r:r + RG, :], p)):
            ha_v[(7 * p + q) * (NQ - 1) + t, r:r + RG, :] = v

    def windows(first, dst, planes, base):
        def copy(b, lo, hi):
            dst[b, lo:hi, :] = qkv_v.at[first:, pl.ds(base, AROWS + HIST)][b, lo:hi, :]
        cuts = [*range(0, AROWS + HIST, WCUT), AROWS + HIST]
        return [partial(copy, b, lo, hi) for lo, hi in zip(cuts, cuts[1:]) for b in range(planes)]

    def scores(n, ws):
        qs = [qkw_v[b, pl.ds(n * AG + HIST, AG), :] for b in range(NB)]
        for w in ws:
            s1_v[2 + n, w] = _tree(jnp.add, [qs[b] * qkw_v[NB + b, pl.ds(n * AG + HIST - DIL * w, AG), :]
                                             for b in range(NB)])

    def logits(pos, n):
        ls = []
        for w in range(WIN):
            t = s1_v[2 + n, w]
            t = t + pltpu.roll(t, 64, 1)
            t = t + pltpu.roll(t, 32, 1)
            if n * AG < DIL * w:
                t = jnp.where(pos + lax.broadcasted_iota(jnp.int32, (AG, 128), 0) >= DIL * w, t, -1e9 * DH ** 0.5)
            ls.append(t)
        for w, t in enumerate(ls + [_tree(jnp.maximum, ls)]):
            s2_v[2 + n, w] = t

    def exponentials(n):
        top = s2_v[2 + n, WIN]
        es = [jnp.exp2((s2_v[2 + n, w] - top) * (DH ** -0.5 * math.log2(math.e))) for w in range(WIN)]
        for w, e in enumerate(es + [_tree(jnp.add, es)]):
            s3_v[2 + n, w] = e

    def reciprocal(n):
        s4_v[2 + n, 0] = 1.0 / s3_v[2 + n, WIN]

    def mix(o, n, bs):
        es = [s3_v[2 + n, w] for w in range(WIN)]
        for b in bs:
            o[b, pl.ds(n * AG, AG), :] = s4_v[2 + n, 0] * _tree(
                jnp.add, [es[w] * vw_v[b, pl.ds(n * AG + HIST - DIL * w, AG), :] for w in range(WIN)])

    def before_start(base):
        for b in range(base, base + NB):
            qkv_v[b, :HIST, :] = jnp.broadcast_to(qkv_v[b, HIST:HIST + 1, :], (HIST, 128))

    def stash(slot, c, v):
        for h in range(4):
            tr_v[2 + slot, pl.ds((4 * c + h) * PITCH, DH), :] = v[h * DH:(h + 1) * DH]

    def gather(slot, d):
        return tr_v[2 + slot, pl.ds(d, 16, stride=PITCH), :].astype(BF16)

    def reorder(shadow, first, last, lags, spread, units, block, put, gates, pins):
        def spill(n, c):
            stash(n % STASH, c, block(units[n], c))

        def fill(n, d0):
            for d in range(d0, d0 + 8):
                put(units[n], d, gather(n % STASH, d))
        step = (last - first - lags[0]) / (len(units) + 1)
        assert lags[0] + 2 * step <= STASH * step
        for n in range(len(units)):
            shadow.add([partial(spill, n, c) for c in range(4)], first + n * step, first + (n + spread) * step,
                       lags[0], gates[0], pins[0])
            shadow.add([partial(fill, n, 8 * c) for c in range(4)], first + lags[0] + (n + 1) * step,
                       first + lags[0] + (n + 2) * step, lags[1], gates[1], pins[1])

    def transpose_slab(shadow, s, units, place):
        ks = lambda kb: pl.ds(al(kb * 128, 128), 128)

        def put(kb, d, v):
            wt_v[2 * DH * (s // 2) + 2 * d + s % 2, :, ks(kb)] = v
        reorder(shadow, *place, units, lambda kb, c: wa_v[s, ks(kb), _lanes(c)].T.astype(F32), put,
                ((gate_wqkv,), ()), (pin_s[0], pin_wt))

    def wt(row, k0, kn, dtype):
        return wt_v[pl.ds(row, 8), :, k0:k0 + kn].astype(dtype).reshape(128, kn)

    def project(shadow, n, tmp, slot, keep):
        ops = _right_operands(lambda r, c, dtype: wt(n * DH + c * 8, r * KQ, KQ, dtype), b1t_v, slot, keep)

        def emit(r, c, v, ref):
            qkv_v[4 * n + c, HIST + r * M:HIST + (r + 1) * M, :] = v
            if r == 0:
                qkw_v[jnp.minimum(4 * n + c, 2 * NB), HIST:HIST + AROWS, :] = v[:AROWS]
        _strassen2(lambda m: shadow.dot(cat(xa_v, 2 * m, 2), ops(m), NT), t2_v, tmp, emit)

    quarter = [(n, a, r) for n, (a, r) in enumerate((a, r) for r in range(0, MQ, RG) for a in range(4))]

    def first_weights(j, _):
        wq_copy(j).wait()
        start_next(1 + j)
        ks = lambda u: pl.ds(al(j % 2 * 512 + u * 128, 128), 128)
        for u in range(4):
            for c in range(4):
                stash(u, c, wa_v[j // 2, ks(u), _lanes(c)].T.astype(F32))
        for u in range(4):
            for d in range(DH):
                wt_v[2 * d + j // 2, :, ks(u)] = gather(u, d)
        return 0

    def first_rows(j, _):
        pl.when(j < 3)(lambda: x_copy(j + 1).wait())
        wk_copy(j).wait()
        start_next(5 + j)

        @pl.when(j == 3)
        def _():
            wo_copy(0).start()
            wg_copy(0).start()
        shadow = _Shadow()
        transpose_slab(shadow, 2, [2 * j, 2 * j + 1], START_T)
        rows = [(0, j * MQ, a, r, n + j * len(quarter)) for n, a, r in quarter]
        more = [(0, jnp.minimum(j + 1, 3) * MQ, a, r, n + (j + 1) % 4 * len(quarter)) for n, a, r in quarter]
        for args in rows:
            normalize(*args, True)
        shadow.add([partial(normalize, *args) for args in rows], *START_L[2], (gate_x,), pin_tu)
        shadow.add([partial(row_mean, *args) for args in more], *START_L[0], (gate_x,), pin_m[0])
        shadow.add([partial(row_var, *args) for args in more], *START_L[1], (gate_x, gate_m[0]), pin_m[1])
        shadow.add([partial(x_operands, j * MQ, r, kk, p)
                    for r in range(0, MQ, RG) for kk in range(2) for p in range(7)], *START_L[3], (gate_tu,), pin_xa)
        for c in range(4):
            t2_v[c % 2] = shadow.dot(cat(ha_v, 0, 4), wt(c * 8, 0, 512, F32), NT)
            y = shadow.dot(cat(ha_v, 4, 4), wt(c * 8, 512, 512, F32), NT) + t2_v[c % 2]
            for a in range(4):
                qkv_v[c, pl.ds(al(HIST + a * M + j * MQ, 8), MQ), :] = y[a * MQ:(a + 1) * MQ]
        shadow.finish()
        return 0

    def first_projection(n, _):
        wqkv_copy(n + 2).wait()
        pl.when(n < 3)(lambda: wqkv_copy(n + 3).start())
        pl.when(n < 2)(lambda: wo_copy(n).start())
        wg_copy(n).start()
        wu_copy(n - 1).start()
        shadow = _Shadow()
        transpose_slab(shadow, n + 2, range(NB), FIRST_T)
        project(shadow, n, tg_v, 0, K_T)
        shadow.finish()
        return 0

    def projection(n, _):
        def put(unit, d, v):
            wo_v[2 * DH * unit[0] + 2 * d + unit[2], :, _lanes(unit[1])] = v
        shadow = _Shadow()
        reorder(shadow, *PROJ_T, [(j, c, s) for j in range(2) for c in range(4) for s in range(2)],
                lambda unit, k: wa_v[6 + unit[0], _lanes(4 * unit[2] + k), _lanes(unit[1])].astype(F32),
                put, ((gate_wo,), (gate_tr,)), (pin_tr, pin_wo))
        project(shadow, 2 * n, tg_v, 0, K_Q)
        project(shadow, 2 * n + 1, tu_v, 1, K_Q)
        shadow.finish()
        return 0

    def gate_up(i, t, _):
        @pl.when(i == 0)
        def _():
            wg_copy(t).wait()
            wu_copy(t).wait()
        busy = [len(R_TERMS[p]) > 1 and k < 4 for p in ORDER for k in range(7)]
        shadow = _Shadow([ROOM_G[0] if busy[(n + ROOM_G[1]) % 49] else 1.0 for n in range(98)])
        shadow.add([partial(h_operands, jnp.maximum(t - 1, 0), r, p)
                    for p in (1, 5, 4, 6, 0, 2, 3) for r in range(0, M, RG)], *SPAN_H, (), pin_ha)
        base, ahead = [al(jnp.minimum(n * AROWS, TM - AROWS), 8) for n in (t, t + 1)]
        o = o_v.at[:, pl.ds(base, AROWS)]
        groups, pairs = range(AROWS // AG), [range(n, n + 2) for n in range(0, 8, 2)]
        shadow.add(windows(2 * NB, vw_v, NB, base), *SPAN_W[0], (), pin_vw)
        shadow.add(windows(0, qkw_v, 2 * NB, ahead), *SPAN_W[1], (), pin_qkw)
        shadow.add([partial(scores, n, ws) for n in groups for ws in pairs], *SPAN_A[0], (gate_qkw,), pin_s[0])
        shadow.add([partial(logits, i * TM + base + n * AG, n) for n in groups], *SPAN_A[1], gate_s[0:1], pin_s[1])
        shadow.add([partial(exponentials, n) for n in groups], *SPAN_A[2], gate_s[1:2], pin_s[2])
        shadow.add([partial(reciprocal, n) for n in groups], *SPAN_A[3], gate_s[2:3], pin_s[3])
        shadow.add([partial(mix, o, n, bs) for n in groups for bs in pairs], *SPAN_A[4],
                   (gate_s[2], gate_s[3], gate_vw), pin_o)
        g = {}

        def emit_g(r, c, v, ref):
            if ref is None:
                ref = tg_v.at[20 + 2 * r + c % 2]
                ref[...] = v
            g[r, c] = ref

        def emit_u(r, c, v, ref):
            hh_v[2 + 4 * r + c] = g[r, c][...] * v
        for k, (tmp, emit) in enumerate(((tg_v, emit_g), (tu_v, emit_u))):
            ops = _right_operands(lambda r, c, dtype: w_v[k * NQ + t, r * KQ:(r + 1) * KQ, _lanes(c)].astype(dtype),
                                  b1_v, k, K_G)
            _strassen2(lambda n: shadow.dot(cat(xa_v, 2 * n, 2), ops(n)), t2_v, tmp, emit)
        shadow.finish()
        return 0

    def down(i, j, _):
        shadow = _Shadow()
        rows = [(jnp.minimum(i + 1, NTILE - 1), j * MH, a, r, n)
                for n, (a, r) in enumerate((a, r) for r in range(0, MH, RG) for a in range(4))]
        shadow.add([partial(row_mean, *args) for args in rows], *SPAN_L[0], (gate_x,), pin_m[0])
        shadow.add([partial(row_var, *args) for args in rows], *SPAN_L[1], (gate_x, gate_m[0]), pin_m[1])
        shadow.add([partial(normalize, *args) for args in rows], *SPAN_L[2], (gate_x, *gate_m), pin_tu)
        shadow.add([partial(x_operands, j * MH, r, kk, p)
                    for r in range(0, MH, RG) for kk in range(2) for p in range(7)], *SPAN_L[3], (gate_tu,), pin_xa)

        def weights(r, c, dtype):
            glu = wd_v[j, :, _lanes(r), _lanes(c)].astype(dtype).reshape(NQ * 128, 128)
            att = wo_v[pl.ds(2 * DH * j + r * 16, 16), :, _lanes(c)].astype(dtype).reshape(KQ, 128)
            return jnp.concatenate([glu, att], axis=0)
        ops = _right_operands(weights, b1d_v, 0, K_D)

        def prod(n):
            p, q = divmod(n, 7)
            direct = lambda blk: _comb(L_TERMS[q], lambda r, c: _comb(
                L_TERMS[p], lambda a, b: blk(2 * a + r, 2 * b + c))).astype(BF16)
            parts = [packed(ha_v, n * (NQ - 1) + t) for t in range(NQ - 1)]
            parts.append(direct(lambda a, c: hh_v[2 + 4 * a + c]))
            parts += [direct(lambda a, c: o_v[2 * c + kk, a * M:(a + 1) * M, :]) for kk in range(2)]
            b = ops(n)
            t3_v[0] = shadow.dot(jnp.concatenate(parts[:4], axis=1), b[:512])
            return shadow.dot(jnp.concatenate(parts[4:], axis=1), b[512:]) + t3_v[0]

        def emit(r, c, v, ref):
            x = x_v[4 * i + r, :, pl.ds(al(j * 512 + c * 128, 128), 128)]
            out_v[2 * i + j, r, :, _lanes(c)] = (v + x.astype(F32)).astype(BF16)
            out_copy(i, j, r, c).start()
        _strassen2(prod, t2_v, tg_v, emit)
        shadow.finish()
        return 0

    def tile(i, _):
        @pl.when(i > 0)
        def _():
            qkv_v[NB:, :HIST, :] = qkv_v[NB:, TM:TM + HIST, :]
        lax.fori_loop(jnp.where(i == 0, 2, 0), 3, projection, 0)

        @pl.when(i == 0)
        def _():
            before_start(2 * NB)
            for cp in late_copies:
                cp.start()
        qkw_v[NB:2 * NB, :HIST, :] = qkv_v[NB:2 * NB, :HIST, :]
        lax.fori_loop(0, NQ, partial(gate_up, i), 0)

        @pl.when(i == 0)
        def _():
            for cp in late_copies:
                cp.wait()
        lax.fori_loop(0, 2, partial(down, i), 0)
        return 0

    x_copy(0).wait()
    start_early(AHEAD)
    for n, a, r in quarter:
        row_mean(0, 0, a, r, n)
        row_var(0, 0, a, r, n)
    lax.fori_loop(0, 4, first_weights, 0)
    lax.fori_loop(0, 4, first_rows, 0)
    qkw_v[:4, HIST:HIST + AROWS, :] = qkv_v[:4, HIST:HIST + AROWS, :]
    lax.fori_loop(1, 4, first_projection, 0)
    for s in range(2):
        wo_copy(s).wait()
    before_start(NB)
    wu_copy(3).start()
    for t in range(4, NQ):
        wg_copy(t).start()
        wu_copy(t).start()
    lax.fori_loop(0, NTILE, tile, 0)
    pltpu.make_async_copy(o_hbm, o_hbm, sems.at[NQ + 8]).wait()


@jax.jit
def pallas_parallel_sum__sliding_local_dilated__glu_gated_bilinear__prompt_kernel(
        A_x, A_wqkv, A_wo, B_x, B_w_gate, B_w_up, B_w_down):
    del B_x
    B, S, D = A_x.shape
    F = B_w_gate.shape[1]
    assert B == 1 and D == 1024 and S % TM == 0 and F == 7 * 512
    NB, NQ, M, NTILE = D // 128, F // 512, TM // 4, S // TM
    window = _attention_rows(NQ)
    V = pltpu.VMEM
    out = pl.pallas_call(
        _kernel,
        out_shape=jax.ShapeDtypeStruct((NTILE, 4, M, D), BF16),
        in_specs=[pl.BlockSpec(memory_space=pl.ANY)] * 6,
        out_specs=pl.BlockSpec(memory_space=pl.ANY),
        scratch_shapes=[
            V((4 * NTILE + 1, M, D), BF16),
            V((2 * NTILE, 4, M, 512), BF16),
            V((2 * NQ, D, 512), BF16),
            V((9, D, 512), BF16),
            V((6 * D // H + 1, 16, D), BF16),
            V((4 * D // H + 1, 16, 512), BF16),
            V((2, NQ, 512, 512), BF16),
            V((2 + STASH, 16 * PITCH, 128), F32),
            V((99, M, 128), BF16),
            V((49 * (NQ - 1) + 1, M, 128), BF16),
            V((3 * NB, TM + HIST, 128), F32),
            V((NB + 1, TM, 128), F32),
            V((18, M, 128), F32),
            V((5, M, 128), F32), V((2, M, 128), F32), V((28, M, 128), F32), V((21, M, 128), F32),
            V((8, D // 4, 128), F32), V((8, 128, D // 4), F32), V((8, NQ * 128 + D // 4, 128), F32),
            V((2 * NB + 1, window + HIST + PAD, 128), F32), V((NB + 1, window + HIST + PAD, 128), F32),
            *[V((2 + window // AG, n, AG, 128), F32) for n in (WIN, WIN + 1, WIN + 1, 1)],
            V((2 + TM // RG, RG, 128), F32), V((3 + TM // RG, RG, 128), F32),
            pltpu.SMEM((1,), jnp.int32),
            pltpu.SemaphoreType.DMA((NQ + 13,)),
        ],
        compiler_params=pltpu.CompilerParams(vmem_limit_bytes=126 << 20, disable_bounds_checks=True),
    )(A_x.reshape(NTILE, 4, M, D), A_wqkv, A_wo, B_w_gate, B_w_up, B_w_down.reshape(NQ, 512, D))
    return out.reshape(B, S, D)
```

```python
import functools
import math

import jax
import jax.numpy as jnp
from jax import lax
import jax.experimental.pallas as pl
import jax.experimental.pallas.tpu as pltpu

H, WIN, DIL = 32, 8, 2
TM = 1024
RG = 16
AG = 8
HIST = 16
PITCH = 33
STASH = 8
F32, BF16 = jnp.float32, jnp.bfloat16
NN = (((1,), (0,)), ((), ()))
NT = (((1,), (1,)), ((), ()))

STEPS, PIN_SPAN, PAD, WCUT, AHEAD = 8, 6, 24, 176, 3
SPAN_H = (0, 39.5, 2)
SPAN_A = ((0, 25, 3), (3, 32, 4), (7, 36, 3), (15, 40, 3), (25, 48, 3))
SPAN_W = ((0, 21, 2), (27.5, 43, 3))
SPAN_L = ((0, 68, 4), (6, 74, 4), (12, 80, 3), (26, 94, 3))
START_L = ((2, 3.5, 3), (5, 6.5, 3), (0, 4, 2), (1, 7.9, 2))
START_T, FIRST_T, PROJ_T = (0, 7, (1.5, 3), 0), (0, 47, (5, 2), 1), (0, 92, (5, 5), 1)
ROOM_G = (0.83, 3)
K_T, K_Q, K_G, K_D = 4, 2, 1, 2

L_TERMS = (((0, 0), (1, 1), 1), ((1, 0), (1, 1), 1), ((0, 0),), ((1, 1),),
           ((0, 0), (0, 1), 1), ((1, 0), (0, 0), -1), ((0, 1), (1, 1), -1))
R_TERMS = (((0, 0), (1, 1), 1), ((0, 0),), ((0, 1), (1, 1), -1), ((1, 0), (0, 0), -1),
           ((1, 1),), ((0, 0), (0, 1), 1), ((1, 0), (1, 1), 1))
ORDER = (1, 3, 4, 2, 0, 6, 5)
SWAP = (0, 1, 0, 0, 1, 1, 1)


def _comb(term, get):
    if len(term) == 1:
        return get(*term[0])
    a, b = get(*term[0]), get(*term[1])
    return a + b if term[2] > 0 else a - b


def _tree(f, xs):
    return xs[0] if len(xs) == 1 else f(_tree(f, xs[:len(xs) // 2]), _tree(f, xs[len(xs) // 2:]))


def _lanes(n):
    return slice(n * 128, (n + 1) * 128)


def _attention_rows(steps):
    return pl.cdiv(TM // 32, steps) * 32


class _Shadow:
    def __init__(self, room=None):
        self.room, self.calls, self.tasks, self.zeros, self.late = room, 0, [], {}, []

    def add(self, fns, first, last, lag, gates, pin):
        for n, fn in enumerate(fns):
            self.tasks.append((self.warp(first + n * (last - first) / len(fns)), fn, lag, gates, pin))
        self.tasks.sort(key=lambda task: task[0])

    def warp(self, at):
        if self.room is None:
            return at
        at *= sum(self.room) / len(self.room)
        for n, room in enumerate(self.room):
            if at < room:
                return n + at / room
            at -= room

    def dot(self, a, b, dims=NN):
        self.late += self.zeros.pop(self.calls, [])
        if self.late and b.dtype == F32:
            rows = [[b[r:r + 8, _lanes(c)] for c in range(b.shape[1] // 128)] for r in range(0, b.shape[0], 8)]
            for step, zero in self.late:
                rows[-2 - 2 * (step * PIN_SPAN // STEPS)][-1] += zero
            self.late = []
            b = jnp.concatenate([jnp.concatenate(row, axis=1) for row in rows], axis=0)
        out = lax.dot_general(a, b.astype(BF16), dims, preferred_element_type=F32)
        events = []
        while self.tasks and self.tasks[0][0] < self.calls + 1:
            events.append(self.tasks.pop(0))
        for step in range(STEPS):
            group = [task for task in events if int((task[0] - self.calls) * STEPS) == step]
            row = step * out.shape[0] // STEPS
            for gate in {gate: None for task in group for gate in task[3]}:
                gate(out[row:row + 8, :128])
            for task in group:
                task[1]()
            for lag, pin in {(task[2], task[4]): None for task in group}:
                self.zeros.setdefault(self.calls + lag, []).append((step, pin()))
        self.calls += 1
        return out

    def finish(self):
        assert not self.tasks


def _level(prod, tmp, emit, keep=None):
    tmp[0] = prod(1)
    c21 = tmp[0] + prod(3)
    emit(1, 0, c21)
    if keep is None:
        tmp[3] = c21
    tmp[1] = prod(4)
    c12 = tmp[1] + prod(2)
    emit(0, 1, c12)
    if keep is None:
        tmp[4] = c12
    tmp[2] = prod(0) - tmp[0] - tmp[1]
    emit(0, 0, (tmp[3] if keep is None else keep(1, 0)) + tmp[2] + prod(6))
    emit(1, 1, (tmp[4] if keep is None else keep(0, 1)) + tmp[2] + prod(5))


def _strassen2(prod, t2, t1, emit, early=False):
    def run(p, e, keep=None):
        _level(lambda q: prod(7 * p + q), t2, lambda r, c, v: e(r, c ^ SWAP[p], v),
               keep and (lambda r, c: keep(r, c ^ SWAP[p])))

    def get(i, r, c):
        return t1[4 * i + 2 * r + c]

    def put(i, r, c, v):
        t1[4 * i + 2 * r + c] = v

    def corner(i, r0, c0, r, c, v):
        v = get(i, r, c) + v
        put(3 + i, r, c, v)
        if early:
            emit(r0 + r, c0 + c, v)

    def left(r, c, v):
        c21 = get(3, r, c)
        if not early:
            emit(2 + r, c, c21)
        emit(r, c, c21 + get(2, r, c) + v)

    def right(r, c, v):
        c12 = get(4, r, c)
        if not early:
            emit(r, 2 + c, c12)
        emit(2 + r, 2 + c, c12 + get(2, r, c) + v)
    run(1, functools.partial(put, 0), functools.partial(get, 0))
    run(3, functools.partial(corner, 0, 2, 0))
    run(4, functools.partial(put, 1), functools.partial(get, 1))
    run(2, functools.partial(corner, 1, 0, 2))
    run(0, lambda r, c, v: put(2, r, c, v - get(0, r, c) - get(1, r, c)))
    run(6, left)
    run(5, right)


def _right_operands(w, b1, slot, keep):
    slots, kept = {}, sorted(((0, 0), (1, 1), (1, 0), (0, 1))[:keep])

    def get(n):
        p, q = divmod(n, 7)
        if len(R_TERMS[p]) == 1:
            a, b = R_TERMS[p][0]
            dtype = BF16 if len(R_TERMS[q]) == 1 else F32
            return _comb(R_TERMS[q], lambda r, c: w(2 * a + r, 2 * b + (c ^ SWAP[p]), dtype))
        level1 = lambda r, c: _comb(R_TERMS[p], lambda a, b: w(2 * a + r, 2 * b + (c ^ SWAP[p]), F32))
        if p not in slots:
            slots[p] = 4 * ((slot + len(slots)) % 2)
            for r, c in kept:
                b1[slots[p] + 2 * r + c] = level1(r, c)
        return _comb(R_TERMS[q], lambda r, c: b1[slots[p] + 2 * r + c] if (r, c) in kept else level1(r, c))
    return get


def _left_operands(blk, p):
    l1 = {(r, c): _comb(L_TERMS[p], lambda a, b: blk(2 * a + r, 2 * b + c)) for r in range(2) for c in range(2)}
    return [_comb(L_TERMS[q], lambda r, c: l1[r, c]).astype(BF16) for q in range(7)]


def _kernel(x_hbm, wqkv_hbm, wo_hbm, wg_hbm, wu_hbm, wd_hbm, o_hbm,
            x_v, out_v, w_v, wa_v, wt_v, wo_v, wd_v, tr_v, xa_v, ha_v, qkv_v, o_v, hh_v, t2_v, t3_v, tg_v, tu_v, u2_v, u1_v,
            b1_v, b1t_v, b1d_v, qkw_v, vw_v, s1_v, s2_v, s3_v, s4_v, m1_v, m2_v, opaque, sems):
    NTILE, D, NQ = x_hbm.shape[0], x_hbm.shape[-1], wg_hbm.shape[1] // 512
    NB, DH = D // 128, D // H
    M, KQ = TM // 4, D // 4
    MH, MQ = M // 2, M // 4
    AROWS = _attention_rows(NQ)
    al, partial = pl.multiple_of, functools.partial

    def slab_copy(src, dst, s, sem):
        return pltpu.make_async_copy(src.at[:, pl.ds(al(s * 512, 512), 512)], dst, sems.at[sem])
    wg_copy = lambda t: slab_copy(wg_hbm, w_v.at[t], t, t)
    wu_copy = lambda t: slab_copy(wu_hbm, w_v.at[NQ + t], t, t)
    wqkv_copy = lambda s: slab_copy(wqkv_hbm, wa_v.at[s], s, NQ + s % 2)
    wo_copy = lambda s: slab_copy(wo_hbm, wa_v.at[6 + s], s, NQ + 2)
    late_copies = [pltpu.make_async_copy(wd_hbm.at[:, :, pl.ds(j * 512, 512)], wd_v.at[j], sems.at[NQ + 3])
                   for j in range(2)]
    late_copies += [pltpu.make_async_copy(x_hbm.at[i], x_v.at[4 * i:4 * i + 4], sems.at[NQ + 3])
                    for i in range(1, NTILE)]

    def x_copy(j):
        rows = pl.ds(al(j * MQ, MQ), MQ)
        return pltpu.make_async_copy(x_hbm.at[0, :, rows], x_v.at[:4, rows], sems.at[NQ + 4 + j])

    def wq_copy(n):
        rows = pl.ds(al(n % 2 * 512, 512), 512)
        return pltpu.make_async_copy(wqkv_hbm.at[rows, pl.ds(al(n // 2 * 512, 512), 512)], wa_v.at[n // 2, rows],
                                     sems.at[n])

    def wk_copy(n):
        rows = pl.ds(al(n * 256, 256), 256)
        return pltpu.make_async_copy(wqkv_hbm.at[rows, pl.ds(D, 512)], wa_v.at[2, rows], sems.at[NQ + 9 + n])

    def out_copy(i, j, r, c):
        return pltpu.make_async_copy(out_v.at[2 * i + j, r, :, _lanes(c)],
                                     o_hbm.at[i, r, :, pl.ds(al(j * 512 + c * 128, 128), 128)], sems.at[NQ + 8])

    early = [[x_copy(0)]] + [[wq_copy(j)] for j in range(4)] + [[x_copy(j + 1), wk_copy(j)] for j in range(3)]
    early += [[wk_copy(3), wqkv_copy(3)]]

    def start_early(n):
        for cp in early[n]:
            cp.start()

    def start_next(step):
        for n in range(AHEAD + 1, len(early)):
            pl.when(step == n - AHEAD)(partial(start_early, n))
    for n in range(AHEAD):
        start_early(n)

    opaque[0] = 0
    origin = lambda: opaque[0]
    for ref in (o_v.at[NB], tu_v.at[20], tr_v.at[0], s1_v.at[0, 0], s2_v.at[0, 0], s3_v.at[0, 0], s4_v.at[0, 0],
                m2_v.at[2 + TM // RG]):
        ref[:8, :] = jnp.zeros((8, 128), F32)
    for ref in (qkw_v.at[2 * NB], vw_v.at[NB], m1_v.at[1]):
        ref[8:16, :] = jnp.zeros((8, 128), F32)
    for ref in (ha_v.at[49 * (NQ - 1)], xa_v.at[98], wt_v.at[6 * DH], wo_v.at[4 * DH]):
        ref[:16, :128] = jnp.zeros((16, 128), BF16)
    for ref in (t2_v, t3_v, tg_v, tu_v, u2_v, u1_v, b1_v, b1t_v, b1d_v):
        ref[origin(), :8, :128] = jnp.zeros((8, 128), F32)
    pin_ha = lambda: ha_v.bitcast(F32)[49 * (NQ - 1), :8, :]
    pin_xa = lambda: xa_v.bitcast(F32)[98, :8, :]
    pin_wt = lambda: wt_v[6 * DH, :, :128].astype(F32)[:8]
    pin_wo = lambda: wo_v[origin() + 4 * DH, :, :128].astype(F32)[:8]
    pin_o = lambda: o_v[NB, :8, :]
    pin_tr = lambda: tr_v[origin(), :8, :]
    pin_tu = lambda: tu_v[origin() + 20, :8, :]
    pin_qkw = lambda: qkw_v[origin() + 2 * NB, 8:16, :]
    pin_vw = lambda: vw_v[origin() + NB, 8:16, :]
    pin_m = [lambda: m1_v[origin() + 1, 8:16, :], lambda: m2_v[2 + TM // RG, :8, :]]
    pin_s = [lambda ref=ref: ref[origin(), 0, :8, :] for ref in (s1_v, s2_v, s3_v, s4_v)]

    def gate_to(ref, at):
        def gate(v):
            if ref.dtype == F32:
                ref[at() + (slice(0, 8), slice(0, 128))] = v
            else:
                ref[at() + (slice(0, 16), slice(0, 128))] = jnp.concatenate([v, v], axis=0).astype(BF16)
        return gate
    gate_tr, gate_tu, *gate_m = [gate_to(ref, lambda: (origin() + 1,)) for ref in (tr_v, tu_v, m1_v, m2_v)]
    gate_s = [gate_to(ref, lambda: (origin() + 1, 0)) for ref in (s1_v, s2_v, s3_v, s4_v)]
    gate_qkw, gate_vw = gate_to(qkw_v, lambda: (origin() + 2 * NB,)), gate_to(vw_v, lambda: (origin() + NB,))
    gate_x = gate_to(x_v, lambda: (4 * NTILE,))
    gate_wqkv, gate_wo = gate_to(wa_v, lambda: (8,)), gate_to(wa_v, lambda: (origin() + 8,))

    packed = lambda ref, n: pltpu.bitcast(ref.bitcast(F32)[n], BF16)
    cat = lambda ref, lo, n: jnp.concatenate([packed(ref, lo + k) for k in range(n)], axis=1)

    def x_rows(i, base, a, r):
        return x_v.at[4 * i + a, pl.ds(al(base, RG), r + RG)][r:r + RG, :].astype(F32)

    def row_mean(i, base, a, r, n):
        m1_v[2 + n] = jnp.broadcast_to(jnp.mean(x_rows(i, base, a, r), axis=-1, keepdims=True), (RG, 128))

    def row_var(i, base, a, r, n):
        xc = x_rows(i, base, a, r) - jnp.tile(m1_v[2 + n], (1, NB))
        m2_v[2 + n] = jnp.broadcast_to(jnp.mean(xc * xc, axis=-1, keepdims=True), (RG, 128))

    def normalize(i, base, a, r, n, plain=False):
        x, mean, scale = x_rows(i, base, a, r), m1_v[2 + n], lax.rsqrt(m2_v[2 + n] + 1e-5)
        for b in range(NB):
            y = (x[:, _lanes(b)] - mean) * scale
            if plain:
                ha_v[b, a * MQ + r:a * MQ + r + RG, :] = y.astype(BF16)
            else:
                tu_v[2 + 4 * a + b // 2, pl.ds((b % 2) * MH + r, RG), :] = y

    def x_operands(base, r, kk, p):
        rows = pl.ds(al(base + r, RG), RG)
        for q, v in enumerate(_left_operands(lambda a, c: tu_v[2 + 4 * a + c, pl.ds(kk * MH + r, RG), :], p)):
            xa_v[2 * (7 * p + q) + kk, rows, :] = v

    def h_operands(t, r, p):
        for q, v in enumerate(_left_operands(lambda a, c: hh_v[2 + 4 * a + c, r:r + RG, :], p)):
            ha_v[(7 * p + q) * (NQ - 1) + t, r:r + RG, :] = v

    def windows(first, dst, planes, base):
        def copy(b, lo, hi):
            dst[b, lo:hi, :] = qkv_v.at[first:, pl.ds(base, AROWS + HIST)][b, lo:hi, :]
        cuts = [*range(0, AROWS + HIST, WCUT), AROWS + HIST]
        return [partial(copy, b, lo, hi) for lo, hi in zip(cuts, cuts[1:]) for b in range(planes)]

    def scores(n, ws):
        qs = [qkw_v[b, pl.ds(n * AG + HIST, AG), :] for b in range(NB)]
        for w in ws:
            s1_v[2 + n, w] = _tree(jnp.add, [qs[b] * qkw_v[NB + b, pl.ds(n * AG + HIST - DIL * w, AG), :]
                                             for b in range(NB)])

    def logits(pos, n):
        ls = []
        for w in range(WIN):
            t = s1_v[2 + n, w]
            t = t + pltpu.roll(t, 64, 1)
            t = t + pltpu.roll(t, 32, 1)
            if n * AG < DIL * w:
                t = jnp.where(pos + lax.broadcasted_iota(jnp.int32, (AG, 128), 0) >= DIL * w, t, -1e9 * DH ** 0.5)
            ls.append(t)
        for w, t in enumerate(ls + [_tree(jnp.maximum, ls)]):
            s2_v[2 + n, w] = t

    def exponentials(n):
        top = s2_v[2 + n, WIN]
        es = [jnp.exp2((s2_v[2 + n, w] - top) * (DH ** -0.5 * math.log2(math.e))) for w in range(WIN)]
        for w, e in enumerate(es + [_tree(jnp.add, es)]):
            s3_v[2 + n, w] = e

    def reciprocal(n):
        s4_v[2 + n, 0] = 1.0 / s3_v[2 + n, WIN]

    def mix(o, n, bs):
        es = [s3_v[2 + n, w] for w in range(WIN)]
        for b in bs:
            o[b, pl.ds(n * AG, AG), :] = s4_v[2 + n, 0] * _tree(
                jnp.add, [es[w] * vw_v[b, pl.ds(n * AG + HIST - DIL * w, AG), :] for w in range(WIN)])

    def before_start(base):
        for b in range(base, base + NB):
            qkv_v[b, :HIST, :] = jnp.broadcast_to(qkv_v[b, HIST:HIST + 1, :], (HIST, 128))

    def stash(slot, c, v):
        for h in range(4):
            tr_v[2 + slot, pl.ds((4 * c + h) * PITCH, DH), :] = v[h * DH:(h + 1) * DH]

    def gather(slot, d):
        return tr_v[2 + slot, pl.ds(d, 16, stride=PITCH), :].astype(BF16)

    def reorder(shadow, first, last, lags, spread, units, block, put, gates, pins):
        def spill(n, c):
            stash(n % STASH, c, block(units[n], c))

        def fill(n, d0):
            for d in range(d0, d0 + 8):
                put(units[n], d, gather(n % STASH, d))
        step = (last - first - lags[0]) / (len(units) + 1)
        assert lags[0] + 2 * step <= STASH * step
        for n in range(len(units)):
            shadow.add([partial(spill, n, c) for c in range(4)], first + n * step, first + (n + spread) * step,
                       lags[0], gates[0], pins[0])
            shadow.add([partial(fill, n, 8 * c) for c in range(4)], first + lags[0] + (n + 1) * step,
                       first + lags[0] + (n + 2) * step, lags[1], gates[1], pins[1])

    def transpose_slab(shadow, s, units, place):
        ks = lambda kb: pl.ds(al(kb * 128, 128), 128)

        def put(kb, d, v):
            wt_v[2 * DH * (s // 2) + 2 * d + s % 2, :, ks(kb)] = v
        reorder(shadow, *place, units, lambda kb, c: wa_v[s, ks(kb), _lanes(c)].T.astype(F32), put,
                ((gate_wqkv,), ()), (pin_s[0], pin_wt))

    def wt(row, k0, kn, dtype):
        return wt_v[pl.ds(row, 8), :, k0:k0 + kn].astype(dtype).reshape(128, kn)

    def project(shadow, n, tmp, slot, keep):
        ops = _right_operands(lambda r, c, dtype: wt(n * DH + c * 8, r * KQ, KQ, dtype), b1t_v, slot, keep)

        def emit(r, c, v):
            qkv_v[4 * n + c, HIST + r * M:HIST + (r + 1) * M, :] = v
            if r == 0:
                qkw_v[jnp.minimum(4 * n + c, 2 * NB), HIST:HIST + AROWS, :] = v[:AROWS]
        _strassen2(lambda m: shadow.dot(cat(xa_v, 2 * m, 2), ops(m), NT), t2_v, tmp, emit)

    quarter = [(n, a, r) for n, (a, r) in enumerate((a, r) for r in range(0, MQ, RG) for a in range(4))]

    def first_weights(j, _):
        wq_copy(j).wait()
        start_next(1 + j)
        ks = lambda u: pl.ds(al(j % 2 * 512 + u * 128, 128), 128)
        for u in range(4):
            for c in range(4):
                stash(u, c, wa_v[j // 2, ks(u), _lanes(c)].T.astype(F32))
        for u in range(4):
            for d in range(DH):
                wt_v[2 * d + j // 2, :, ks(u)] = gather(u, d)
        return 0

    def first_rows(j, _):
        pl.when(j < 3)(lambda: x_copy(j + 1).wait())
        wk_copy(j).wait()
        start_next(5 + j)

        @pl.when(j == 3)
        def _():
            wo_copy(0).start()
            wg_copy(0).start()
        shadow = _Shadow()
        transpose_slab(shadow, 2, [2 * j, 2 * j + 1], START_T)
        rows = [(0, j * MQ, a, r, n + j * len(quarter)) for n, a, r in quarter]
        more = [(0, jnp.minimum(j + 1, 3) * MQ, a, r, n + (j + 1) % 4 * len(quarter)) for n, a, r in quarter]
        for args in rows:
            normalize(*args, True)
        shadow.add([partial(normalize, *args) for args in rows], *START_L[2], (gate_x,), pin_tu)
        shadow.add([partial(row_mean, *args) for args in more], *START_L[0], (gate_x,), pin_m[0])
        shadow.add([partial(row_var, *args) for args in more], *START_L[1], (gate_x, gate_m[0]), pin_m[1])
        shadow.add([partial(x_operands, j * MQ, r, kk, p)
                    for r in range(0, MQ, RG) for kk in range(2) for p in range(7)], *START_L[3], (gate_tu,), pin_xa)
        for c in range(4):
            t2_v[c % 2] = shadow.dot(cat(ha_v, 0, 4), wt(c * 8, 0, 512, F32), NT)
            y = shadow.dot(cat(ha_v, 4, 4), wt(c * 8, 512, 512, F32), NT) + t2_v[c % 2]
            for a in range(4):
                qkv_v[c, pl.ds(al(HIST + a * M + j * MQ, 8), MQ), :] = y[a * MQ:(a + 1) * MQ]
        shadow.finish()
        return 0

    def first_projection(n, _):
        wqkv_copy(n + 2).wait()
        pl.when(n < 3)(lambda: wqkv_copy(n + 3).start())
        pl.when(n < 2)(lambda: wo_copy(n).start())
        wg_copy(n).start()
        wu_copy(n - 1).start()
        shadow = _Shadow()
        transpose_slab(shadow, n + 2, range(NB), FIRST_T)
        project(shadow, n, tg_v, 0, K_T)
        shadow.finish()
        return 0

    def projection(n, _):
        def put(unit, d, v):
            wo_v[2 * DH * unit[0] + 2 * d + unit[2], :, _lanes(unit[1])] = v
        shadow = _Shadow()
        reorder(shadow, *PROJ_T, [(j, c, s) for j in range(2) for c in range(4) for s in range(2)],
                lambda unit, k: wa_v[6 + unit[0], _lanes(4 * unit[2] + k), _lanes(unit[1])].astype(F32),
                put, ((gate_wo,), (gate_tr,)), (pin_tr, pin_wo))
        project(shadow, 2 * n, tg_v, 0, K_Q)
        project(shadow, 2 * n + 1, tu_v, 1, K_Q)
        shadow.finish()
        return 0

    def gate_up(i, t, _):
        @pl.when(i == 0)
        def _():
            wg_copy(t).wait()
            wu_copy(t).wait()
        busy = [len(R_TERMS[p]) > 1 and k < 4 for p in ORDER for k in range(7)]
        shadow = _Shadow([ROOM_G[0] if busy[(n + ROOM_G[1]) % 49] else 1.0 for n in range(49)])
        shadow.add([partial(h_operands, jnp.maximum(t - 1, 0), r, p)
                    for p in (1, 5, 4, 0, 2, 6, 3) for r in range(0, M, RG)], *SPAN_H, (), pin_ha)
        base, ahead = [al(jnp.minimum(n * AROWS, TM - AROWS), 8) for n in (t, t + 1)]
        o = o_v.at[:, pl.ds(base, AROWS)]
        groups, pairs = range(AROWS // AG), [range(n, n + 2) for n in range(0, 8, 2)]
        shadow.add(windows(2 * NB, vw_v, NB, base), *SPAN_W[0], (), pin_vw)
        shadow.add(windows(0, qkw_v, 2 * NB, ahead), *SPAN_W[1], (), pin_qkw)
        shadow.add([partial(scores, n, ws) for n in groups for ws in pairs], *SPAN_A[0], (gate_qkw,), pin_s[0])
        shadow.add([partial(logits, i * TM + base + n * AG, n) for n in groups], *SPAN_A[1], gate_s[0:1], pin_s[1])
        shadow.add([partial(exponentials, n) for n in groups], *SPAN_A[2], gate_s[1:2], pin_s[2])
        shadow.add([partial(reciprocal, n) for n in groups], *SPAN_A[3], gate_s[2:3], pin_s[3])
        shadow.add([partial(mix, o, n, bs) for n in groups for bs in pairs], *SPAN_A[4],
                   (gate_s[2], gate_s[3], gate_vw), pin_o)

        def emit(r, c, v):
            hh_v[2 + 4 * r + c] = v[:, :128] * v[:, 128:]
        ops = _right_operands(lambda r, c, dtype: jnp.concatenate(
            [w_v[k * NQ + t, r * KQ:(r + 1) * KQ, _lanes(c)].astype(dtype) for k in range(2)], axis=1), b1_v, 0, K_G)
        _strassen2(lambda n: shadow.dot(cat(xa_v, 2 * n, 2), ops(n)), u2_v, u1_v, emit)
        shadow.finish()
        return 0

    def down(i, j, _):
        shadow = _Shadow()
        rows = [(jnp.minimum(i + 1, NTILE - 1), j * MH, a, r, n)
                for n, (a, r) in enumerate((a, r) for r in range(0, MH, RG) for a in range(4))]
        shadow.add([partial(row_mean, *args) for args in rows], *SPAN_L[0], (gate_x,), pin_m[0])
        shadow.add([partial(row_var, *args) for args in rows], *SPAN_L[1], (gate_x, gate_m[0]), pin_m[1])
        shadow.add([partial(normalize, *args) for args in rows], *SPAN_L[2], (gate_x, *gate_m), pin_tu)
        shadow.add([partial(x_operands, j * MH, r, kk, p)
                    for r in range(0, MH, RG) for kk in range(2) for p in range(7)], *SPAN_L[3], (gate_tu,), pin_xa)

        def weights(r, c, dtype):
            glu = wd_v[j, :, _lanes(r), _lanes(c)].astype(dtype).reshape(NQ * 128, 128)
            att = wo_v[pl.ds(2 * DH * j + r * 16, 16), :, _lanes(c)].astype(dtype).reshape(KQ, 128)
            return jnp.concatenate([glu, att], axis=0)
        ops = _right_operands(weights, b1d_v, 0, K_D)

        def prod(n):
            p, q = divmod(n, 7)
            direct = lambda blk: _comb(L_TERMS[q], lambda r, c: _comb(
                L_TERMS[p], lambda a, b: blk(2 * a + r, 2 * b + c))).astype(BF16)
            parts = [packed(ha_v, n * (NQ - 1) + t) for t in range(NQ - 1)]
            parts.append(direct(lambda a, c: hh_v[2 + 4 * a + c]))
            parts += [direct(lambda a, c: o_v[2 * c + kk, a * M:(a + 1) * M, :]) for kk in range(2)]
            b = ops(n)
            t3_v[0] = shadow.dot(jnp.concatenate(parts[:4], axis=1), b[:512])
            return shadow.dot(jnp.concatenate(parts[4:], axis=1), b[512:]) + t3_v[0]

        def emit(r, c, v):
            x = x_v[4 * i + r, :, pl.ds(al(j * 512 + c * 128, 128), 128)]
            out_v[2 * i + j, r, :, _lanes(c)] = (v + x.astype(F32)).astype(BF16)
            out_copy(i, j, r, c).start()
        _strassen2(prod, t2_v, tg_v, emit, True)
        shadow.finish()
        return 0

    def tile(i, _):
        @pl.when(i > 0)
        def _():
            qkv_v[NB:, :HIST, :] = qkv_v[NB:, TM:TM + HIST, :]
        lax.fori_loop(jnp.where(i == 0, 2, 0), 3, projection, 0)

        @pl.when(i == 0)
        def _():
            before_start(2 * NB)
            for cp in late_copies:
                cp.start()
        qkw_v[NB:2 * NB, :HIST, :] = qkv_v[NB:2 * NB, :HIST, :]
        lax.fori_loop(0, NQ, partial(gate_up, i), 0)

        @pl.when(i == 0)
        def _():
            for cp in late_copies:
                cp.wait()
        lax.fori_loop(0, 2, partial(down, i), 0)
        return 0

    x_copy(0).wait()
    start_early(AHEAD)
    for n, a, r in quarter:
        row_mean(0, 0, a, r, n)
        row_var(0, 0, a, r, n)
    lax.fori_loop(0, 4, first_weights, 0)
    lax.fori_loop(0, 4, first_rows, 0)
    qkw_v[:4, HIST:HIST + AROWS, :] = qkv_v[:4, HIST:HIST + AROWS, :]
    lax.fori_loop(1, 4, first_projection, 0)
    for s in range(2):
        wo_copy(s).wait()
    before_start(NB)
    wu_copy(3).start()
    for t in range(4, NQ):
        wg_copy(t).start()
        wu_copy(t).start()
    lax.fori_loop(0, NTILE, tile, 0)
    pltpu.make_async_copy(o_hbm, o_hbm, sems.at[NQ + 8]).wait()


@jax.jit
def pallas_parallel_sum__sliding_local_dilated__glu_gated_bilinear__prompt_kernel(
        A_x, A_wqkv, A_wo, B_x, B_w_gate, B_w_up, B_w_down):
    del B_x
    B, S, D = A_x.shape
    F = B_w_gate.shape[1]
    assert B == 1 and D == 1024 and S % TM == 0 and F == 7 * 512
    NB, NQ, M, NTILE = D // 128, F // 512, TM // 4, S // TM
    window = _attention_rows(NQ)
    V = pltpu.VMEM
    out = pl.pallas_call(
        _kernel,
        out_shape=jax.ShapeDtypeStruct((NTILE, 4, M, D), BF16),
        in_specs=[pl.BlockSpec(memory_space=pl.ANY)] * 6,
        out_specs=pl.BlockSpec(memory_space=pl.ANY),
        scratch_shapes=[
            V((4 * NTILE + 1, M, D), BF16),
            V((2 * NTILE, 4, M, 512), BF16),
            V((2 * NQ, D, 512), BF16),
            V((9, D, 512), BF16),
            V((6 * D // H + 1, 16, D), BF16),
            V((4 * D // H + 1, 16, 512), BF16),
            V((2, NQ, 512, 512), BF16),
            V((2 + STASH, 16 * PITCH, 128), F32),
            V((99, M, 128), BF16),
            V((49 * (NQ - 1) + 1, M, 128), BF16),
            V((3 * NB, TM + HIST, 128), F32),
            V((NB + 1, TM, 128), F32),
            V((18, M, 128), F32),
            V((5, M, 128), F32), V((2, M, 128), F32), V((20, M, 128), F32), V((21, M, 128), F32),
            V((5, M, 256), F32), V((20, M, 256), F32),
            V((8, D // 4, 256), F32), V((8, 128, D // 4), F32), V((8, NQ * 128 + D // 4, 128), F32),
            V((2 * NB + 1, window + HIST + PAD, 128), F32), V((NB + 1, window + HIST + PAD, 128), F32),
            *[V((2 + window // AG, n, AG, 128), F32) for n in (WIN, WIN + 1, WIN + 1, 1)],
            V((2 + TM // RG, RG, 128), F32), V((3 + TM // RG, RG, 128), F32),
            pltpu.SMEM((1,), jnp.int32),
            pltpu.SemaphoreType.DMA((NQ + 13,)),
        ],
        compiler_params=pltpu.CompilerParams(vmem_limit_bytes=126 << 20, disable_bounds_checks=True),
    )(A_x.reshape(NTILE, 4, M, D), A_wqkv, A_wo, B_w_gate, B_w_up, B_w_down.reshape(NQ, 512, D))
    return out.reshape(B, S, D)
```

```python
import functools
import math

import jax
import jax.numpy as jnp
from jax import lax
import jax.experimental.pallas as pl
import jax.experimental.pallas.tpu as pltpu

H, WIN, DIL = 32, 8, 2
TM = 1024
RG = 16
AG = 8
HIST = 16
PITCH = 33
STASH = 8
F32, BF16 = jnp.float32, jnp.bfloat16
NN = (((1,), (0,)), ((), ()))
NT = (((1,), (1,)), ((), ()))

STEPS, PIN_SPAN, PAD, WCUT, AHEAD = 8, 6, 24, 88, 3
SPAN_H = (0, 39.5, 2)
SPAN_A = ((0, 25, 3), (3, 32, 4), (7, 36, 3), (15, 40, 3), (25, 48, 3))
SPAN_W = ((0, 21, 2), (27.5, 43, 2))
SPAN_L = ((0, 68, 4), (6, 74, 4), (12, 80, 3), (26, 94, 3))
START_L = ((2, 3.5, 3), (5, 6.5, 3), (0, 4, 2), (1, 7.9, 2))
START_T, FIRST_T, PROJ_T = (0, 7, (1.5, 3), 0), (0, 47, (5, 2), 1), (0, 92, (5, 5), 1)
ROOM_G = (0.83, 3)
K_T, K_Q, K_G, K_D = 4, 2, 1, 2

L_TERMS = (((0, 0), (1, 1), 1), ((1, 0), (1, 1), 1), ((0, 0),), ((1, 1),),
           ((0, 0), (0, 1), 1), ((1, 0), (0, 0), -1), ((0, 1), (1, 1), -1))
R_TERMS = (((0, 0), (1, 1), 1), ((0, 0),), ((0, 1), (1, 1), -1), ((1, 0), (0, 0), -1),
           ((1, 1),), ((0, 0), (0, 1), 1), ((1, 0), (1, 1), 1))
ORDER = (1, 3, 4, 2, 0, 6, 5)
SWAP = (0, 1, 0, 0, 1, 1, 1)


def _comb(term, get):
    if len(term) == 1:
        return get(*term[0])
    a, b = get(*term[0]), get(*term[1])
    return a + b if term[2] > 0 else a - b


def _tree(f, xs):
    return xs[0] if len(xs) == 1 else f(_tree(f, xs[:len(xs) // 2]), _tree(f, xs[len(xs) // 2:]))


def _lanes(n):
    return slice(n * 128, (n + 1) * 128)


def _attention_rows(steps):
    return pl.cdiv(TM // 32, steps) * 32


class _Shadow:
    def __init__(self, room=None):
        self.room, self.calls, self.tasks, self.zeros, self.late = room, 0, [], {}, []

    def add(self, fns, first, last, lag, gates, pin):
        for n, fn in enumerate(fns):
            self.tasks.append((self.warp(first + n * (last - first) / len(fns)), fn, lag, gates, pin))
        self.tasks.sort(key=lambda task: task[0])

    def warp(self, at):
        if self.room is None:
            return at
        at *= sum(self.room) / len(self.room)
        for n, room in enumerate(self.room):
            if at < room:
                return n + at / room
            at -= room

    def dot(self, a, b, dims=NN):
        self.late += self.zeros.pop(self.calls, [])
        if self.late and b.dtype == F32:
            rows = [[b[r:r + 8, _lanes(c)] for c in range(b.shape[1] // 128)] for r in range(0, b.shape[0], 8)]
            for step, zero in self.late:
                rows[-2 - 2 * (step * PIN_SPAN // STEPS)][-1] += zero
            self.late = []
            b = jnp.concatenate([jnp.concatenate(row, axis=1) for row in rows], axis=0)
        out = lax.dot_general(a, b.astype(BF16), dims, preferred_element_type=F32)
        events = []
        while self.tasks and self.tasks[0][0] < self.calls + 1:
            events.append(self.tasks.pop(0))
        for step in range(STEPS):
            group = [task for task in events if int((task[0] - self.calls) * STEPS) == step]
            row = step * out.shape[0] // STEPS
            for gate in {gate: None for task in group for gate in task[3]}:
                gate(out[row:row + 8, :128])
            for task in group:
                task[1]()
            for lag, pin in {(task[2], task[4]): None for task in group}:
                self.zeros.setdefault(self.calls + lag, []).append((step, pin()))
        self.calls += 1
        return out

    def finish(self):
        assert not self.tasks


def _level(prod, tmp, emit, keep=None):
    tmp[0] = prod(1)
    c21 = tmp[0] + prod(3)
    emit(1, 0, c21)
    if keep is None:
        tmp[3] = c21
    tmp[1] = prod(4)
    c12 = tmp[1] + prod(2)
    emit(0, 1, c12)
    if keep is None:
        tmp[4] = c12
    tmp[2] = prod(0) - tmp[0] - tmp[1]
    emit(0, 0, (tmp[3] if keep is None else keep(1, 0)) + tmp[2] + prod(6))
    emit(1, 1, (tmp[4] if keep is None else keep(0, 1)) + tmp[2] + prod(5))


def _strassen2(prod, t2, t1, emit, early=False):
    def run(p, e, keep=None):
        _level(lambda q: prod(7 * p + q), t2, lambda r, c, v: e(r, c ^ SWAP[p], v),
               keep and (lambda r, c: keep(r, c ^ SWAP[p])))

    def get(i, r, c):
        return t1[4 * i + 2 * r + c]

    def put(i, r, c, v):
        t1[4 * i + 2 * r + c] = v

    def corner(i, r0, c0, r, c, v):
        v = get(i, r, c) + v
        put(3 + i, r, c, v)
        if early:
            emit(r0 + r, c0 + c, v)

    def left(r, c, v):
        c21 = get(3, r, c)
        if not early:
            emit(2 + r, c, c21)
        emit(r, c, c21 + get(2, r, c) + v)

    def right(r, c, v):
        c12 = get(4, r, c)
        if not early:
            emit(r, 2 + c, c12)
        emit(2 + r, 2 + c, c12 + get(2, r, c) + v)
    run(1, functools.partial(put, 0), functools.partial(get, 0))
    run(3, functools.partial(corner, 0, 2, 0))
    run(4, functools.partial(put, 1), functools.partial(get, 1))
    run(2, functools.partial(corner, 1, 0, 2))
    run(0, lambda r, c, v: put(2, r, c, v - get(0, r, c) - get(1, r, c)))
    run(6, left)
    run(5, right)


def _right_operands(w, b1, slot, keep):
    slots, kept = {}, sorted(((0, 0), (1, 1), (1, 0), (0, 1))[:keep])

    def get(n):
        p, q = divmod(n, 7)
        if len(R_TERMS[p]) == 1:
            a, b = R_TERMS[p][0]
            dtype = BF16 if len(R_TERMS[q]) == 1 else F32
            return _comb(R_TERMS[q], lambda r, c: w(2 * a + r, 2 * b + (c ^ SWAP[p]), dtype))
        level1 = lambda r, c: _comb(R_TERMS[p], lambda a, b: w(2 * a + r, 2 * b + (c ^ SWAP[p]), F32))
        if p not in slots:
            slots[p] = 4 * ((slot + len(slots)) % 2)
            for r, c in kept:
                b1[slots[p] + 2 * r + c] = level1(r, c)
        return _comb(R_TERMS[q], lambda r, c: b1[slots[p] + 2 * r + c] if (r, c) in kept else level1(r, c))
    return get


def _left_operands(blk, p):
    l1 = {(r, c): _comb(L_TERMS[p], lambda a, b: blk(2 * a + r, 2 * b + c)) for r in range(2) for c in range(2)}
    return [_comb(L_TERMS[q], lambda r, c: l1[r, c]).astype(BF16) for q in range(7)]


def _kernel(x_hbm, wqkv_hbm, wo_hbm, wg_hbm, wu_hbm, wd_hbm, o_hbm,
            x_v, out_v, w_v, wa_v, wt_v, wo_v, wd_v, tr_v, xa_v, ha_v, qkv_v, o_v, hh_v, t2_v, t3_v, tg_v, tu_v, u2_v, u1_v,
            b1_v, b1t_v, b1d_v, qkw_v, vw_v, s1_v, s2_v, s3_v, s4_v, m1_v, m2_v, opaque, sems):
    NTILE, D, NQ = x_hbm.shape[0], x_hbm.shape[-1], wg_hbm.shape[1] // 512
    NB, DH = D // 128, D // H
    M, KQ = TM // 4, D // 4
    MH, MQ = M // 2, M // 4
    AROWS = _attention_rows(NQ)
    al, partial = pl.multiple_of, functools.partial

    def slab_copy(src, dst, s, sem):
        return pltpu.make_async_copy(src.at[:, pl.ds(al(s * 512, 512), 512)], dst, sems.at[sem])
    wg_copy = lambda t: slab_copy(wg_hbm, w_v.at[t], t, t)
    wu_copy = lambda t: slab_copy(wu_hbm, w_v.at[NQ + t], t, t)
    wqkv_copy = lambda s: slab_copy(wqkv_hbm, wa_v.at[s], s, NQ + s % 2)
    wo_copy = lambda s: slab_copy(wo_hbm, wa_v.at[6 + s], s, NQ + 2)
    late_copies = [pltpu.make_async_copy(wd_hbm.at[:, :, pl.ds(j * 512, 512)], wd_v.at[j], sems.at[NQ + 3])
                   for j in range(2)]
    late_copies += [pltpu.make_async_copy(x_hbm.at[i], x_v.at[4 * i:4 * i + 4], sems.at[NQ + 3])
                    for i in range(1, NTILE)]

    def x_copy(j):
        rows = pl.ds(al(j * MQ, MQ), MQ)
        return pltpu.make_async_copy(x_hbm.at[0, :, rows], x_v.at[:4, rows], sems.at[NQ + j % 3 + jnp.minimum(j % 3, 1)])

    def wq_copy(n):
        rows = pl.ds(al(n % 2 * 512, 512), 512)
        return pltpu.make_async_copy(wqkv_hbm.at[rows, pl.ds(al(n // 2 * 512, 512), 512)], wa_v.at[n // 2, rows],
                                     sems.at[n])

    def wk_copy(n):
        rows = pl.ds(al(n * 256, 256), 256)
        return pltpu.make_async_copy(wqkv_hbm.at[rows, pl.ds(D, 512)], wa_v.at[2, rows], sems.at[4 + n % 3])

    def out_copy(i, j, r, c):
        return pltpu.make_async_copy(out_v.at[2 * i + j, r, :, _lanes(c)],
                                     o_hbm.at[i, r, :, pl.ds(al(j * 512 + c * 128, 128), 128)], sems.at[NQ + 4])

    early = [[x_copy(0)]] + [[wq_copy(j)] for j in range(4)] + [[x_copy(j + 1), wk_copy(j)] for j in range(3)]
    early += [[wk_copy(3), wqkv_copy(3)]]

    def start_early(n):
        for cp in early[n]:
            cp.start()

    def start_next(step):
        for n in range(AHEAD + 1, len(early)):
            pl.when(step == n - AHEAD)(partial(start_early, n))
    for n in range(AHEAD):
        start_early(n)

    opaque[0] = 0
    origin = lambda: opaque[0]
    for ref in (o_v.at[NB], tu_v.at[20], tr_v.at[0], s1_v.at[0, 0], s2_v.at[0, 0], s3_v.at[0, 0], s4_v.at[0, 0],
                m2_v.at[2 + TM // RG]):
        ref[:8, :] = jnp.zeros((8, 128), F32)
    for ref in (qkw_v.at[2 * NB], vw_v.at[NB], m1_v.at[1]):
        ref[8:16, :] = jnp.zeros((8, 128), F32)
    for ref in (ha_v.at[49 * (NQ - 1)], xa_v.at[98], wt_v.at[6 * DH], wo_v.at[4 * DH]):
        ref[:16, :128] = jnp.zeros((16, 128), BF16)
    for ref in (t2_v, t3_v, tg_v, tu_v, u2_v, u1_v, b1_v, b1t_v, b1d_v):
        ref[origin(), :8, :128] = jnp.zeros((8, 128), F32)
    pin_ha = lambda: ha_v.bitcast(F32)[49 * (NQ - 1), :8, :]
    pin_xa = lambda: xa_v.bitcast(F32)[98, :8, :]
    pin_wt = lambda: wt_v[6 * DH, :, :128].astype(F32)[:8]
    pin_wo = lambda: wo_v[origin() + 4 * DH, :, :128].astype(F32)[:8]
    pin_o = lambda: o_v[NB, :8, :]
    pin_tr = lambda: tr_v[origin(), :8, :]
    pin_tu = lambda: tu_v[origin() + 20, :8, :]
    pin_qkw = lambda: qkw_v[origin() + 2 * NB, 8:16, :]
    pin_vw = lambda: vw_v[origin() + NB, 8:16, :]
    pin_m = [lambda: m1_v[origin() + 1, 8:16, :], lambda: m2_v[2 + TM // RG, :8, :]]
    pin_s = [lambda ref=ref: ref[origin(), 0, :8, :] for ref in (s1_v, s2_v, s3_v, s4_v)]

    def gate_to(ref, at):
        def gate(v):
            if ref.dtype == F32:
                ref[at() + (slice(0, 8), slice(0, 128))] = v
            else:
                ref[at() + (slice(0, 16), slice(0, 128))] = jnp.concatenate([v, v], axis=0).astype(BF16)
        return gate
    gate_tr, gate_tu, *gate_m = [gate_to(ref, lambda: (origin() + 1,)) for ref in (tr_v, tu_v, m1_v, m2_v)]
    gate_s = [gate_to(ref, lambda: (origin() + 1, 0)) for ref in (s1_v, s2_v, s3_v, s4_v)]
    gate_qkw, gate_vw = gate_to(qkw_v, lambda: (origin() + 2 * NB,)), gate_to(vw_v, lambda: (origin() + NB,))
    gate_x = gate_to(x_v, lambda: (4 * NTILE,))
    gate_wqkv, gate_wo = gate_to(wa_v, lambda: (8,)), gate_to(wa_v, lambda: (origin() + 8,))

    packed = lambda ref, n: pltpu.bitcast(ref.bitcast(F32)[n], BF16)
    cat = lambda ref, lo, n: jnp.concatenate([packed(ref, lo + k) for k in range(n)], axis=1)

    def x_rows(i, base, a, r):
        return x_v.at[4 * i + a, pl.ds(al(base, RG), r + RG)][r:r + RG, :].astype(F32)

    def row_mean(i, base, a, r, n):
        m1_v[2 + n] = jnp.broadcast_to(jnp.mean(x_rows(i, base, a, r), axis=-1, keepdims=True), (RG, 128))

    def row_var(i, base, a, r, n):
        xc = x_rows(i, base, a, r) - jnp.tile(m1_v[2 + n], (1, NB))
        m2_v[2 + n] = jnp.broadcast_to(jnp.mean(xc * xc, axis=-1, keepdims=True), (RG, 128))

    def normalize(i, base, a, r, n, plain=False):
        x, mean, scale = x_rows(i, base, a, r), m1_v[2 + n], lax.rsqrt(m2_v[2 + n] + 1e-5)
        for b in range(NB):
            y = (x[:, _lanes(b)] - mean) * scale
            if plain:
                ha_v[b, a * MQ + r:a * MQ + r + RG, :] = y.astype(BF16)
            else:
                tu_v[2 + 4 * a + b // 2, pl.ds((b % 2) * MH + r, RG), :] = y

    def x_operands(base, r, kk, p):
        rows = pl.ds(al(base + r, RG), RG)
        for q, v in enumerate(_left_operands(lambda a, c: tu_v[2 + 4 * a + c, pl.ds(kk * MH + r, RG), :], p)):
            xa_v[2 * (7 * p + q) + kk, rows, :] = v

    def h_operands(t, r, p):
        for q, v in enumerate(_left_operands(lambda a, c: hh_v[2 + 4 * a + c, r:r + RG, :], p)):
            ha_v[(7 * p + q) * (NQ - 1) + t, r:r + RG, :] = v

    def windows(first, dst, planes, base):
        def copy(b, lo, hi):
            dst[b, lo:hi, :] = qkv_v.at[first:, pl.ds(base, AROWS + HIST)][b, lo:hi, :]
        cuts = [*range(0, AROWS + HIST, WCUT), AROWS + HIST]
        return [partial(copy, b, lo, hi) for lo, hi in zip(cuts, cuts[1:]) for b in range(planes)]

    def scores(n, ws):
        qs = [qkw_v[b, pl.ds(n * AG + HIST, AG), :] for b in range(NB)]
        for w in ws:
            s1_v[2 + n, w] = _tree(jnp.add, [qs[b] * qkw_v[NB + b, pl.ds(n * AG + HIST - DIL * w, AG), :]
                                             for b in range(NB)])

    def logits(pos, n):
        ls = []
        for w in range(WIN):
            t = s1_v[2 + n, w]
            t = t + pltpu.roll(t, 64, 1)
            t = t + pltpu.roll(t, 32, 1)
            if n * AG < DIL * w:
                t = jnp.where(pos + lax.broadcasted_iota(jnp.int32, (AG, 128), 0) >= DIL * w, t, -1e9 * DH ** 0.5)
            ls.append(t)
        for w, t in enumerate(ls + [_tree(jnp.maximum, ls)]):
            s2_v[2 + n, w] = t

    def exponentials(n):
        top = s2_v[2 + n, WIN]
        es = [jnp.exp2((s2_v[2 + n, w] - top) * (DH ** -0.5 * math.log2(math.e))) for w in range(WIN)]
        for w, e in enumerate(es + [_tree(jnp.add, es)]):
            s3_v[2 + n, w] = e

    def reciprocal(n):
        s4_v[2 + n, 0] = 1.0 / s3_v[2 + n, WIN]

    def mix(o, n, bs):
        es = [s3_v[2 + n, w] for w in range(WIN)]
        for b in bs:
            o[b, pl.ds(n * AG, AG), :] = s4_v[2 + n, 0] * _tree(
                jnp.add, [es[w] * vw_v[b, pl.ds(n * AG + HIST - DIL * w, AG), :] for w in range(WIN)])

    def before_start(base):
        for b in range(base, base + NB):
            qkv_v[b, :HIST, :] = jnp.broadcast_to(qkv_v[b, HIST:HIST + 1, :], (HIST, 128))

    def stash(slot, c, v):
        for h in range(4):
            tr_v[2 + slot, pl.ds((4 * c + h) * PITCH, DH), :] = v[h * DH:(h + 1) * DH]

    def gather(slot, d):
        return tr_v[2 + slot, pl.ds(d, 16, stride=PITCH), :].astype(BF16)

    def reorder(shadow, first, last, lags, spread, units, block, put, gates, pins):
        def spill(n, c):
            stash(n % STASH, c, block(units[n], c))

        def fill(n, d0):
            for d in range(d0, d0 + 8):
                put(units[n], d, gather(n % STASH, d))
        step = (last - first - lags[0]) / (len(units) + 1)
        assert lags[0] + 2 * step <= STASH * step
        for n in range(len(units)):
            shadow.add([partial(spill, n, c) for c in range(4)], first + n * step, first + (n + spread) * step,
                       lags[0], gates[0], pins[0])
            shadow.add([partial(fill, n, 8 * c) for c in range(4)], first + lags[0] + (n + 1) * step,
                       first + lags[0] + (n + 2) * step, lags[1], gates[1], pins[1])

    def transpose_slab(shadow, s, units, place):
        ks = lambda kb: pl.ds(al(kb * 128, 128), 128)

        def put(kb, d, v):
            wt_v[2 * DH * (s // 2) + 2 * d + s % 2, :, ks(kb)] = v
        reorder(shadow, *place, units, lambda kb, c: wa_v[s, ks(kb), _lanes(c)].T.astype(F32), put,
                ((gate_wqkv,), ()), (pin_s[0], pin_wt))

    def wt(row, k0, kn, dtype):
        return wt_v[pl.ds(row, 8), :, k0:k0 + kn].astype(dtype).reshape(128, kn)

    def project(shadow, n, tmp, slot, keep):
        ops = _right_operands(lambda r, c, dtype: wt(n * DH + c * 8, r * KQ, KQ, dtype), b1t_v, slot, keep)

        def emit(r, c, v):
            qkv_v[4 * n + c, HIST + r * M:HIST + (r + 1) * M, :] = v
            if r == 0:
                qkw_v[jnp.minimum(4 * n + c, 2 * NB), HIST:HIST + AROWS, :] = v[:AROWS]
        _strassen2(lambda m: shadow.dot(cat(xa_v, 2 * m, 2), ops(m), NT), t2_v, tmp, emit)

    quarter = [(n, a, r) for n, (a, r) in enumerate((a, r) for r in range(0, MQ, RG) for a in range(4))]

    def first_weights(j, _):
        wq_copy(j).wait()
        start_next(1 + j)
        ks = lambda u: pl.ds(al(j % 2 * 512 + u * 128, 128), 128)
        for u in range(4):
            for c in range(4):
                stash(u, c, wa_v[j // 2, ks(u), _lanes(c)].T.astype(F32))
        for u in range(4):
            for d in range(DH):
                wt_v[2 * d + j // 2, :, ks(u)] = gather(u, d)
        return 0

    def first_rows(j, _):
        pl.when(j < 3)(lambda: x_copy(j + 1).wait())
        wk_copy(j).wait()
        start_next(5 + j)

        @pl.when(j == 3)
        def _():
            wo_copy(0).start()
            wg_copy(0).start()
        shadow = _Shadow()
        transpose_slab(shadow, 2, [2 * j, 2 * j + 1], START_T)
        rows = [(0, j * MQ, a, r, n + j * len(quarter)) for n, a, r in quarter]
        more = [(0, jnp.minimum(j + 1, 3) * MQ, a, r, n + (j + 1) % 4 * len(quarter)) for n, a, r in quarter]
        for args in rows:
            normalize(*args, True)
        shadow.add([partial(normalize, *args) for args in rows], *START_L[2], (gate_x,), pin_tu)
        shadow.add([partial(row_mean, *args) for args in more], *START_L[0], (gate_x,), pin_m[0])
        shadow.add([partial(row_var, *args) for args in more], *START_L[1], (gate_x, gate_m[0]), pin_m[1])
        shadow.add([partial(x_operands, j * MQ, r, kk, p)
                    for r in range(0, MQ, RG) for kk in range(2) for p in range(7)], *START_L[3], (gate_tu,), pin_xa)
        for c in range(4):
            t2_v[c % 2] = shadow.dot(cat(ha_v, 0, 4), wt(c * 8, 0, 512, F32), NT)
            y = shadow.dot(cat(ha_v, 4, 4), wt(c * 8, 512, 512, F32), NT) + t2_v[c % 2]
            for a in range(4):
                qkv_v[c, pl.ds(al(HIST + a * M + j * MQ, 8), MQ), :] = y[a * MQ:(a + 1) * MQ]
        shadow.finish()
        return 0

    def first_projection(n, _):
        wqkv_copy(n + 2).wait()
        pl.when(n < 3)(lambda: wqkv_copy(n + 3).start())
        pl.when(n < 2)(lambda: wo_copy(n).start())
        wg_copy(n).start()
        wu_copy(n - 1).start()
        shadow = _Shadow()
        transpose_slab(shadow, n + 2, range(NB), FIRST_T)
        project(shadow, n, tg_v, 0, K_T)
        shadow.finish()
        return 0

    def projection(n, _):
        def put(unit, d, v):
            wo_v[2 * DH * unit[0] + 2 * d + unit[2], :, _lanes(unit[1])] = v
        shadow = _Shadow()
        reorder(shadow, *PROJ_T, [(j, c, s) for j in range(2) for c in range(4) for s in range(2)],
                lambda unit, k: wa_v[6 + unit[0], _lanes(4 * unit[2] + k), _lanes(unit[1])].astype(F32),
                put, ((gate_wo,), (gate_tr,)), (pin_tr, pin_wo))
        project(shadow, 2 * n, tg_v, 0, K_Q)
        project(shadow, 2 * n + 1, tu_v, 1, K_Q)
        shadow.finish()
        return 0

    def gate_up(i, t, _):
        @pl.when(i == 0)
        def _():
            wg_copy(t).wait()
            wu_copy(t).wait()
        busy = [len(R_TERMS[p]) > 1 and k < 4 for p in ORDER for k in range(7)]
        shadow = _Shadow([ROOM_G[0] if busy[(n + ROOM_G[1]) % 49] else 1.0 for n in range(49)])
        shadow.add([partial(h_operands, jnp.maximum(t - 1, 0), r, p)
                    for p in (1, 5, 4, 0, 2, 6, 3) for r in range(0, M, RG)], *SPAN_H, (), pin_ha)
        base, ahead = [al(jnp.minimum(n * AROWS, TM - AROWS), 8) for n in (t, t + 1)]
        o = o_v.at[:, pl.ds(base, AROWS)]
        groups, pairs = range(AROWS // AG), [range(n, n + 2) for n in range(0, 8, 2)]
        shadow.add(windows(2 * NB, vw_v, NB, base), *SPAN_W[0], (), pin_vw)
        shadow.add(windows(0, qkw_v, 2 * NB, ahead), *SPAN_W[1], (), pin_qkw)
        shadow.add([partial(scores, n, ws) for n in groups for ws in pairs], *SPAN_A[0], (gate_qkw,), pin_s[0])
        shadow.add([partial(logits, i * TM + base + n * AG, n) for n in groups], *SPAN_A[1], gate_s[0:1], pin_s[1])
        shadow.add([partial(exponentials, n) for n in groups], *SPAN_A[2], gate_s[1:2], pin_s[2])
        shadow.add([partial(reciprocal, n) for n in groups], *SPAN_A[3], gate_s[2:3], pin_s[3])
        shadow.add([partial(mix, o, n, bs) for n in groups for bs in pairs], *SPAN_A[4],
                   (gate_s[2], gate_s[3], gate_vw), pin_o)

        def emit(r, c, v):
            hh_v[2 + 4 * r + c] = v[:, :128] * v[:, 128:]
        ops = _right_operands(lambda r, c, dtype: jnp.concatenate(
            [w_v[k * NQ + t, r * KQ:(r + 1) * KQ, _lanes(c)].astype(dtype) for k in range(2)], axis=1), b1_v, 0, K_G)
        _strassen2(lambda n: shadow.dot(cat(xa_v, 2 * n, 2), ops(n)), u2_v, u1_v, emit)
        shadow.finish()
        return 0

    def down(i, j, _):
        shadow = _Shadow()
        rows = [(jnp.minimum(i + 1, NTILE - 1), j * MH, a, r, n)
                for n, (a, r) in enumerate((a, r) for r in range(0, MH, RG) for a in range(4))]
        shadow.add([partial(row_mean, *args) for args in rows], *SPAN_L[0], (gate_x,), pin_m[0])
        shadow.add([partial(row_var, *args) for args in rows], *SPAN_L[1], (gate_x, gate_m[0]), pin_m[1])
        shadow.add([partial(normalize, *args) for args in rows], *SPAN_L[2], (gate_x, *gate_m), pin_tu)
        shadow.add([partial(x_operands, j * MH, r, kk, p)
                    for r in range(0, MH, RG) for kk in range(2) for p in range(7)], *SPAN_L[3], (gate_tu,), pin_xa)

        def weights(r, c, dtype):
            glu = wd_v[j, :, _lanes(r), _lanes(c)].astype(dtype).reshape(NQ * 128, 128)
            att = wo_v[pl.ds(2 * DH * j + r * 16, 16), :, _lanes(c)].astype(dtype).reshape(KQ, 128)
            return jnp.concatenate([att[128:], glu, att[:128]], axis=0)
        ops = _right_operands(weights, b1d_v, 0, K_D)

        def prod(n):
            p, q = divmod(n, 7)
            direct = lambda blk: _comb(L_TERMS[q], lambda r, c: _comb(
                L_TERMS[p], lambda a, b: blk(2 * a + r, 2 * b + c))).astype(BF16)
            att = [direct(lambda a, c: o_v[2 * c + kk, a * M:(a + 1) * M, :]) for kk in range(2)]
            glu = [packed(ha_v, n * (NQ - 1) + t) for t in range(NQ - 1)] + [direct(lambda a, c: hh_v[2 + 4 * a + c])]
            parts, b = [att[1], *glu, att[0]], ops(n)
            t3_v[0] = shadow.dot(jnp.concatenate(parts[:4], axis=1), b[:512])
            return shadow.dot(jnp.concatenate(parts[4:], axis=1), b[512:]) + t3_v[0]

        def emit(r, c, v):
            x = x_v[4 * i + r, :, pl.ds(al(j * 512 + c * 128, 128), 128)]
            out_v[2 * i + j, r, :, _lanes(c)] = (v + x.astype(F32)).astype(BF16)
            out_copy(i, j, r, c).start()
        _strassen2(prod, t2_v, tg_v, emit, True)
        shadow.finish()
        return 0

    def tile(i, _):
        @pl.when(i > 0)
        def _():
            qkv_v[NB:, :HIST, :] = qkv_v[NB:, TM:TM + HIST, :]
        lax.fori_loop(jnp.where(i == 0, 2, 0), 3, projection, 0)

        @pl.when(i == 0)
        def _():
            before_start(2 * NB)
            for cp in late_copies:
                cp.start()
        qkw_v[NB:2 * NB, :HIST, :] = qkv_v[NB:2 * NB, :HIST, :]
        lax.fori_loop(0, NQ, partial(gate_up, i), 0)

        @pl.when(i == 0)
        def _():
            for cp in late_copies:
                cp.wait()
        lax.fori_loop(0, 2, partial(down, i), 0)
        return 0

    x_copy(0).wait()
    start_early(AHEAD)
    for n, a, r in quarter:
        row_mean(0, 0, a, r, n)
        row_var(0, 0, a, r, n)
    lax.fori_loop(0, 4, first_weights, 0)
    lax.fori_loop(0, 4, first_rows, 0)
    qkw_v[:4, HIST:HIST + AROWS, :] = qkv_v[:4, HIST:HIST + AROWS, :]
    lax.fori_loop(1, 4, first_projection, 0)
    for s in range(2):
        wo_copy(s).wait()
    before_start(NB)
    wu_copy(3).start()
    for t in range(4, NQ):
        wg_copy(t).start()
        wu_copy(t).start()
    lax.fori_loop(0, NTILE, tile, 0)
    pltpu.make_async_copy(o_hbm, o_hbm, sems.at[NQ + 4]).wait()


@jax.jit
def pallas_parallel_sum__sliding_local_dilated__glu_gated_bilinear__prompt_kernel(
        A_x, A_wqkv, A_wo, B_x, B_w_gate, B_w_up, B_w_down):
    del B_x
    B, S, D = A_x.shape
    F = B_w_gate.shape[1]
    assert B == 1 and D == 1024 and S % TM == 0 and F == 7 * 512
    NB, NQ, M, NTILE = D // 128, F // 512, TM // 4, S // TM
    window = _attention_rows(NQ)
    V = pltpu.VMEM
    out = pl.pallas_call(
        _kernel,
        out_shape=jax.ShapeDtypeStruct((NTILE, 4, M, D), BF16),
        in_specs=[pl.BlockSpec(memory_space=pl.ANY)] * 6,
        out_specs=pl.BlockSpec(memory_space=pl.ANY),
        scratch_shapes=[
            V((4 * NTILE + 1, M, D), BF16),
            V((2 * NTILE, 4, M, 512), BF16),
            V((2 * NQ, D, 512), BF16),
            V((9, D, 512), BF16),
            V((6 * D // H + 1, 16, D), BF16),
            V((4 * D // H + 1, 16, 512), BF16),
            V((2, NQ, 512, 512), BF16),
            V((2 + STASH, 16 * PITCH, 128), F32),
            V((99, M, 128), BF16),
            V((49 * (NQ - 1) + 1, M, 128), BF16),
            V((3 * NB, TM + HIST, 128), F32),
            V((NB + 1, TM, 128), F32),
            V((18, M, 128), F32),
            V((5, M, 128), F32), V((2, M, 128), F32),
            V((20, M, 128), F32), V((21, M, 128), F32), V((5, M, 256), F32), V((20, M, 256), F32),
            V((8, D // 4, 256), F32), V((8, 128, D // 4), F32), V((8, NQ * 128 + D // 4, 128), F32),
            V((2 * NB + 1, window + HIST + PAD, 128), F32), V((NB + 1, window + HIST + PAD, 128), F32),
            *[V((2 + window // AG, n, AG, 128), F32) for n in (WIN, WIN + 1, WIN + 1, 1)],
            V((2 + TM // RG, RG, 128), F32), V((3 + TM // RG, RG, 128), F32),
            pltpu.SMEM((1,), jnp.int32),
            pltpu.SemaphoreType.DMA((NQ + 5,)),
        ],
        compiler_params=pltpu.CompilerParams(vmem_limit_bytes=126 << 20, disable_bounds_checks=True),
    )(A_x.reshape(NTILE, 4, M, D), A_wqkv, A_wo, B_w_gate, B_w_up, B_w_down.reshape(NQ, 512, D))
    return out.reshape(B, S, D)
```

```python
import functools
import math

import jax
import jax.numpy as jnp
from jax import lax
import jax.experimental.pallas as pl
import jax.experimental.pallas.tpu as pltpu

H, WIN, DIL = 32, 8, 2
TM = 1024
RG = 16
AG = 8
HIST = 16
PITCH = 33
STASH = 8
F32, BF16 = jnp.float32, jnp.bfloat16
NN = (((1,), (0,)), ((), ()))
NT = (((1,), (1,)), ((), ()))

STEPS, PIN_SPAN, PAD, WCUT = 8, 6, 24, 88
SPAN_H = (0, 39.5, 2)
SPAN_A = ((0, 25, 3), (3, 32, 4), (7, 36, 3), (15, 40, 3), (25, 48, 3))
SPAN_W = ((0, 21, 2), (27.5, 43, 2))
SPAN_L = ((0, 68, 4), (6, 74, 4), (12, 80, 3), (26, 94, 3))
START_L = ((2, 3.5, 3), (5, 6.5, 3), (0, 4, 2), (1, 7.9, 2))
START_T, FIRST_T, PROJ_T = (0, 7, (1.5, 3), 0), (0, 47, (5, 2), 1), (0, 92, (5, 5), 1)
ROOM_G = (0.83, 3)
K_T, K_Q, K_G, K_D = 4, 2, 1, 2

L_TERMS = (((0, 0), (1, 1), 1), ((1, 0), (1, 1), 1), ((0, 0),), ((1, 1),),
           ((0, 0), (0, 1), 1), ((1, 0), (0, 0), -1), ((0, 1), (1, 1), -1))
R_TERMS = (((0, 0), (1, 1), 1), ((0, 0),), ((0, 1), (1, 1), -1), ((1, 0), (0, 0), -1),
           ((1, 1),), ((0, 0), (0, 1), 1), ((1, 0), (1, 1), 1))
ORDER = (1, 3, 4, 2, 0, 6, 5)
SWAP = (0, 1, 0, 0, 1, 1, 1)


def _comb(term, get):
    if len(term) == 1:
        return get(*term[0])
    a, b = get(*term[0]), get(*term[1])
    return a + b if term[2] > 0 else a - b


def _tree(f, xs):
    return xs[0] if len(xs) == 1 else f(_tree(f, xs[:len(xs) // 2]), _tree(f, xs[len(xs) // 2:]))


def _lanes(n):
    return slice(n * 128, (n + 1) * 128)


def _attention_rows(steps):
    return pl.cdiv(TM // 32, steps) * 32


class _Shadow:
    def __init__(self, room=None):
        self.room, self.calls, self.tasks, self.zeros, self.late = room, 0, [], {}, []

    def add(self, fns, first, last, lag, gates, pin):
        for n, fn in enumerate(fns):
            self.tasks.append((self.warp(first + n * (last - first) / len(fns)), fn, lag, gates, pin))
        self.tasks.sort(key=lambda task: task[0])

    def warp(self, at):
        if self.room is None:
            return at
        at *= sum(self.room) / len(self.room)
        for n, room in enumerate(self.room):
            if at < room:
                return n + at / room
            at -= room

    def dot(self, a, b, dims=NN):
        self.late += self.zeros.pop(self.calls, [])
        if self.late and b.dtype == F32:
            rows = [[b[r:r + 8, _lanes(c)] for c in range(b.shape[1] // 128)] for r in range(0, b.shape[0], 8)]
            for step, zero in self.late:
                rows[-2 - 2 * (step * PIN_SPAN // STEPS)][-1] += zero
            self.late = []
            b = jnp.concatenate([jnp.concatenate(row, axis=1) for row in rows], axis=0)
        out = lax.dot_general(a, b.astype(BF16), dims, preferred_element_type=F32)
        events = []
        while self.tasks and self.tasks[0][0] < self.calls + 1:
            events.append(self.tasks.pop(0))
        for step in range(STEPS):
            group = [task for task in events if int((task[0] - self.calls) * STEPS) == step]
            row = step * out.shape[0] // STEPS
            for gate in {gate: None for task in group for gate in task[3]}:
                gate(out[row:row + 8, :128])
            for task in group:
                task[1]()
            for lag, pin in {(task[2], task[4]): None for task in group}:
                self.zeros.setdefault(self.calls + lag, []).append((step, pin()))
        self.calls += 1
        return out

    def finish(self):
        assert not self.tasks


def _level(prod, tmp, emit, keep=None):
    tmp[0] = prod(1)
    c21 = tmp[0] + prod(3)
    emit(1, 0, c21)
    if keep is None:
        tmp[3] = c21
    tmp[1] = prod(4)
    c12 = tmp[1] + prod(2)
    emit(0, 1, c12)
    if keep is None:
        tmp[4] = c12
    tmp[2] = prod(0) - tmp[0] - tmp[1]
    emit(0, 0, (tmp[3] if keep is None else keep(1, 0)) + tmp[2] + prod(6))
    emit(1, 1, (tmp[4] if keep is None else keep(0, 1)) + tmp[2] + prod(5))


def _strassen2(prod, t2, t1, emit, early=False):
    def run(p, e, keep=None):
        _level(lambda q: prod(7 * p + q), t2, lambda r, c, v: e(r, c ^ SWAP[p], v),
               keep and (lambda r, c: keep(r, c ^ SWAP[p])))

    def get(i, r, c):
        return t1[4 * i + 2 * r + c]

    def put(i, r, c, v):
        t1[4 * i + 2 * r + c] = v

    def corner(i, r0, c0, r, c, v):
        v = get(i, r, c) + v
        put(3 + i, r, c, v)
        if early:
            emit(r0 + r, c0 + c, v)

    def left(r, c, v):
        c21 = get(3, r, c)
        if not early:
            emit(2 + r, c, c21)
        emit(r, c, c21 + get(2, r, c) + v)

    def right(r, c, v):
        c12 = get(4, r, c)
        if not early:
            emit(r, 2 + c, c12)
        emit(2 + r, 2 + c, c12 + get(2, r, c) + v)
    run(1, functools.partial(put, 0), functools.partial(get, 0))
    run(3, functools.partial(corner, 0, 2, 0))
    run(4, functools.partial(put, 1), functools.partial(get, 1))
    run(2, functools.partial(corner, 1, 0, 2))
    run(0, lambda r, c, v: put(2, r, c, v - get(0, r, c) - get(1, r, c)))
    run(6, left)
    run(5, right)


def _right_operands(w, b1, slot, keep):
    slots, kept = {}, sorted(((0, 0), (1, 1), (1, 0), (0, 1))[:keep])

    def get(n):
        p, q = divmod(n, 7)
        if len(R_TERMS[p]) == 1:
            a, b = R_TERMS[p][0]
            dtype = BF16 if len(R_TERMS[q]) == 1 else F32
            return _comb(R_TERMS[q], lambda r, c: w(2 * a + r, 2 * b + (c ^ SWAP[p]), dtype))
        level1 = lambda r, c: _comb(R_TERMS[p], lambda a, b: w(2 * a + r, 2 * b + (c ^ SWAP[p]), F32))
        if p not in slots:
            slots[p] = 4 * ((slot + len(slots)) % 2)
            for r, c in kept:
                b1[slots[p] + 2 * r + c] = level1(r, c)
        return _comb(R_TERMS[q], lambda r, c: b1[slots[p] + 2 * r + c] if (r, c) in kept else level1(r, c))
    return get


def _left_operands(blk, p):
    l1 = {(r, c): _comb(L_TERMS[p], lambda a, b: blk(2 * a + r, 2 * b + c)) for r in range(2) for c in range(2)}
    return [_comb(L_TERMS[q], lambda r, c: l1[r, c]).astype(BF16) for q in range(7)]


def _kernel(x_hbm, wqkv_hbm, wo_hbm, wg_hbm, wu_hbm, wd_hbm, o_hbm,
            x_v, out_v, w_v, wa_v, wt_v, wo_v, wd_v, tr_v, xa_v, ha_v, qkv_v, o_v, hh_v, t2_v, t3_v, tg_v, tu_v, u2_v, u1_v,
            b1_v, b1t_v, b1d_v, qkw_v, vw_v, s1_v, s2_v, s3_v, s4_v, m1_v, m2_v, opaque, sems):
    NTILE, D, NQ = x_hbm.shape[0], x_hbm.shape[-1], wg_hbm.shape[1] // 512
    NB, DH = D // 128, D // H
    M, KQ = TM // 4, D // 4
    MH, MQ = M // 2, M // 4
    AROWS = _attention_rows(NQ)
    al, partial = pl.multiple_of, functools.partial

    def slab_copy(src, dst, s, sem):
        return pltpu.make_async_copy(src.at[:, pl.ds(al(s * 512, 512), 512)], dst, sems.at[sem])
    wg_copy = lambda t: slab_copy(wg_hbm, w_v.at[t], t, t)
    wu_copy = lambda t: slab_copy(wu_hbm, w_v.at[NQ + t], t, t)
    wqkv_copy = lambda s: slab_copy(wqkv_hbm, wa_v.at[s], s, NQ + s % 2)
    wo_copy = lambda s: slab_copy(wo_hbm, wa_v.at[6 + s], s, NQ + 2)
    late_copies = [pltpu.make_async_copy(wd_hbm.at[:, :, pl.ds(j * 512, 512)], wd_v.at[j], sems.at[NQ + 3])
                   for j in range(2)]
    late_copies += [pltpu.make_async_copy(x_hbm.at[i], x_v.at[4 * i:4 * i + 4], sems.at[NQ + 3])
                    for i in range(1, NTILE)]

    def x_copy(j):
        rows = pl.ds(al(j * MQ, MQ), MQ)
        return pltpu.make_async_copy(x_hbm.at[0, :, rows], x_v.at[:4, rows], sems.at[NQ + j % 3 + jnp.minimum(j % 3, 1)])

    def wq_copy(n):
        rows = pl.ds(al(n % 2 * 512, 512), 512)
        return pltpu.make_async_copy(wqkv_hbm.at[rows, pl.ds(al(n // 2 * 512, 512), 512)], wa_v.at[n // 2, rows],
                                     sems.at[n])

    def wk_copy(n):
        rows = pl.ds(al(n * 256, 256), 256)
        return pltpu.make_async_copy(wqkv_hbm.at[rows, pl.ds(D, 512)], wa_v.at[2, rows], sems.at[4 + n % 3])

    def out_copy(i, j, r, c):
        return pltpu.make_async_copy(out_v.at[2 * i + j, r, :, _lanes(c)],
                                     o_hbm.at[i, r, :, pl.ds(al(j * 512 + c * 128, 128), 128)], sems.at[NQ + 4])

    early = [[wq_copy(3)]] + [[x_copy(j + 1), wk_copy(j)] for j in range(3)]
    x_copy(0).start()
    for n in range(2):
        wq_copy(n).start()

    opaque[0] = 0
    origin = lambda: opaque[0]
    for ref in (o_v.at[NB], tu_v.at[20], tr_v.at[0], s1_v.at[0, 0], s2_v.at[0, 0], s3_v.at[0, 0], s4_v.at[0, 0],
                m2_v.at[2 + TM // RG]):
        ref[:8, :] = jnp.zeros((8, 128), F32)
    for ref in (qkw_v.at[2 * NB], vw_v.at[NB], m1_v.at[1]):
        ref[8:16, :] = jnp.zeros((8, 128), F32)
    for ref in (ha_v.at[49 * (NQ - 1)], xa_v.at[98], wt_v.at[6 * DH], wo_v.at[4 * DH]):
        ref[:16, :128] = jnp.zeros((16, 128), BF16)
    for ref in (t2_v, t3_v, tg_v, tu_v, u2_v, u1_v, b1_v, b1t_v, b1d_v):
        ref[origin(), :8, :128] = jnp.zeros((8, 128), F32)
    pin_ha = lambda: ha_v.bitcast(F32)[49 * (NQ - 1), :8, :]
    pin_xa = lambda: xa_v.bitcast(F32)[98, :8, :]
    pin_wt = lambda: wt_v[6 * DH, :, :128].astype(F32)[:8]
    pin_wo = lambda: wo_v[origin() + 4 * DH, :, :128].astype(F32)[:8]
    pin_o = lambda: o_v[NB, :8, :]
    pin_tr = lambda: tr_v[origin(), :8, :]
    pin_tu = lambda: tu_v[origin() + 20, :8, :]
    pin_qkw = lambda: qkw_v[origin() + 2 * NB, 8:16, :]
    pin_vw = lambda: vw_v[origin() + NB, 8:16, :]
    pin_m = [lambda: m1_v[origin() + 1, 8:16, :], lambda: m2_v[2 + TM // RG, :8, :]]
    pin_s = [lambda ref=ref: ref[origin(), 0, :8, :] for ref in (s1_v, s2_v, s3_v, s4_v)]

    def gate_to(ref, at):
        def gate(v):
            if ref.dtype == F32:
                ref[at() + (slice(0, 8), slice(0, 128))] = v
            else:
                ref[at() + (slice(0, 16), slice(0, 128))] = jnp.concatenate([v, v], axis=0).astype(BF16)
        return gate
    gate_tr, gate_tu, *gate_m = [gate_to(ref, lambda: (origin() + 1,)) for ref in (tr_v, tu_v, m1_v, m2_v)]
    gate_s = [gate_to(ref, lambda: (origin() + 1, 0)) for ref in (s1_v, s2_v, s3_v, s4_v)]
    gate_qkw, gate_vw = gate_to(qkw_v, lambda: (origin() + 2 * NB,)), gate_to(vw_v, lambda: (origin() + NB,))
    gate_x = gate_to(x_v, lambda: (4 * NTILE,))
    gate_wqkv, gate_wo = gate_to(wa_v, lambda: (8,)), gate_to(wa_v, lambda: (origin() + 8,))

    packed = lambda ref, n: pltpu.bitcast(ref.bitcast(F32)[n], BF16)
    cat = lambda ref, lo, n: jnp.concatenate([packed(ref, lo + k) for k in range(n)], axis=1)

    def x_rows(i, base, a, r):
        return x_v.at[4 * i + a, pl.ds(al(base, RG), r + RG)][r:r + RG, :].astype(F32)

    def row_mean(i, base, a, r, n):
        m1_v[2 + n] = jnp.broadcast_to(jnp.mean(x_rows(i, base, a, r), axis=-1, keepdims=True), (RG, 128))

    def row_var(i, base, a, r, n):
        xc = x_rows(i, base, a, r) - jnp.tile(m1_v[2 + n], (1, NB))
        m2_v[2 + n] = jnp.broadcast_to(jnp.mean(xc * xc, axis=-1, keepdims=True), (RG, 128))

    def normalize(i, base, a, r, n, plain=False):
        x, mean, scale = x_rows(i, base, a, r), m1_v[2 + n], lax.rsqrt(m2_v[2 + n] + 1e-5)
        for b in range(NB):
            y = (x[:, _lanes(b)] - mean) * scale
            if plain:
                ha_v[b, a * MQ + r:a * MQ + r + RG, :] = y.astype(BF16)
            else:
                tu_v[2 + 4 * a + b // 2, pl.ds((b % 2) * MH + r, RG), :] = y

    def x_operands(base, r, kk, p):
        rows = pl.ds(al(base + r, RG), RG)
        for q, v in enumerate(_left_operands(lambda a, c: tu_v[2 + 4 * a + c, pl.ds(kk * MH + r, RG), :], p)):
            xa_v[2 * (7 * p + q) + kk, rows, :] = v

    def h_operands(t, r, p):
        for q, v in enumerate(_left_operands(lambda a, c: hh_v[2 + 4 * a + c, r:r + RG, :], p)):
            ha_v[(7 * p + q) * (NQ - 1) + t, r:r + RG, :] = v

    def windows(first, dst, planes, base):
        def copy(b, lo, hi):
            dst[b, lo:hi, :] = qkv_v.at[first:, pl.ds(base, AROWS + HIST)][b, lo:hi, :]
        cuts = [*range(0, AROWS + HIST, WCUT), AROWS + HIST]
        return [partial(copy, b, lo, hi) for lo, hi in zip(cuts, cuts[1:]) for b in range(planes)]

    def scores(n, ws):
        qs = [qkw_v[b, pl.ds(n * AG + HIST, AG), :] for b in range(NB)]
        for w in ws:
            s1_v[2 + n, w] = _tree(jnp.add, [qs[b] * qkw_v[NB + b, pl.ds(n * AG + HIST - DIL * w, AG), :]
                                             for b in range(NB)])

    def logits(pos, n):
        ls = []
        for w in range(WIN):
            t = s1_v[2 + n, w]
            t = t + pltpu.roll(t, 64, 1)
            t = t + pltpu.roll(t, 32, 1)
            if n * AG < DIL * w:
                t = jnp.where(pos + lax.broadcasted_iota(jnp.int32, (AG, 128), 0) >= DIL * w, t, -1e9 * DH ** 0.5)
            ls.append(t)
        for w, t in enumerate(ls + [_tree(jnp.maximum, ls)]):
            s2_v[2 + n, w] = t

    def exponentials(n):
        top = s2_v[2 + n, WIN]
        es = [jnp.exp2((s2_v[2 + n, w] - top) * (DH ** -0.5 * math.log2(math.e))) for w in range(WIN)]
        for w, e in enumerate(es + [_tree(jnp.add, es)]):
            s3_v[2 + n, w] = e

    def reciprocal(n):
        s4_v[2 + n, 0] = 1.0 / s3_v[2 + n, WIN]

    def mix(o, n, bs):
        es = [s3_v[2 + n, w] for w in range(WIN)]
        for b in bs:
            o[b, pl.ds(n * AG, AG), :] = s4_v[2 + n, 0] * _tree(
                jnp.add, [es[w] * vw_v[b, pl.ds(n * AG + HIST - DIL * w, AG), :] for w in range(WIN)])

    def before_start(base):
        for b in range(base, base + NB):
            qkv_v[b, :HIST, :] = jnp.broadcast_to(qkv_v[b, HIST:HIST + 1, :], (HIST, 128))

    def stash(slot, c, v):
        for h in range(4):
            tr_v[2 + slot, pl.ds((4 * c + h) * PITCH, DH), :] = v[h * DH:(h + 1) * DH]

    def gather(slot, d):
        return tr_v[2 + slot, pl.ds(d, 16, stride=PITCH), :].astype(BF16)

    def reorder(shadow, first, last, lags, spread, units, block, put, gates, pins):
        def spill(n, c):
            stash(n % STASH, c, block(units[n], c))

        def fill(n, d0):
            for d in range(d0, d0 + 8):
                put(units[n], d, gather(n % STASH, d))
        step = (last - first - lags[0]) / (len(units) + 1)
        assert lags[0] + 2 * step <= STASH * step
        for n in range(len(units)):
            shadow.add([partial(spill, n, c) for c in range(4)], first + n * step, first + (n + spread) * step,
                       lags[0], gates[0], pins[0])
            shadow.add([partial(fill, n, 8 * c) for c in range(4)], first + lags[0] + (n + 1) * step,
                       first + lags[0] + (n + 2) * step, lags[1], gates[1], pins[1])

    def transpose_slab(shadow, s, units, place):
        ks = lambda kb: pl.ds(al(kb * 128, 128), 128)

        def put(kb, d, v):
            wt_v[2 * DH * (s // 2) + 2 * d + s % 2, :, ks(kb)] = v
        reorder(shadow, *place, units, lambda kb, c: wa_v[s, ks(kb), _lanes(c)].T.astype(F32), put,
                ((gate_wqkv,), ()), (pin_s[0], pin_wt))

    def wt(row, k0, kn, dtype):
        return wt_v[pl.ds(row, 8), :, k0:k0 + kn].astype(dtype).reshape(128, kn)

    def project(shadow, n, tmp, slot, keep):
        ops = _right_operands(lambda r, c, dtype: wt(n * DH + c * 8, r * KQ, KQ, dtype), b1t_v, slot, keep)

        def emit(r, c, v):
            qkv_v[4 * n + c, HIST + r * M:HIST + (r + 1) * M, :] = v
            if r == 0:
                qkw_v[jnp.minimum(4 * n + c, 2 * NB), HIST:HIST + AROWS, :] = v[:AROWS]
        _strassen2(lambda m: shadow.dot(cat(xa_v, 2 * m, 2), ops(m), NT), t2_v, tmp, emit)

    quarter = [(n, a, r) for n, (a, r) in enumerate((a, r) for r in range(0, MQ, RG) for a in range(4))]

    def first_weights(j, _):
        wq_copy(j).wait()
        for n, copies in enumerate(early):
            @pl.when(j == n)
            def _():
                for cp in copies:
                    cp.start()
        ks = lambda u: pl.ds(al(j % 2 * 512 + u * 128, 128), 128)
        for u in range(4):
            for c in range(4):
                stash(u, c, wa_v[j // 2, ks(u), _lanes(c)].T.astype(F32))
        for u in range(4):
            for d in range(DH):
                wt_v[2 * d + j // 2, :, ks(u)] = gather(u, d)
        return 0

    def first_rows(j, _):
        pl.when(j < 3)(lambda: x_copy(j + 1).wait())
        wk_copy(j).wait()

        @pl.when(j == 0)
        def _():
            wk_copy(3).start()
            wqkv_copy(3).start()
        shadow = _Shadow()
        transpose_slab(shadow, 2, [2 * j, 2 * j + 1], START_T)
        rows = [(0, j * MQ, a, r, n + j * len(quarter)) for n, a, r in quarter]
        more = [(0, jnp.minimum(j + 1, 3) * MQ, a, r, n + (j + 1) % 4 * len(quarter)) for n, a, r in quarter]
        for args in rows:
            normalize(*args, True)
        shadow.add([partial(normalize, *args) for args in rows], *START_L[2], (gate_x,), pin_tu)
        shadow.add([partial(row_mean, *args) for args in more], *START_L[0], (gate_x,), pin_m[0])
        shadow.add([partial(row_var, *args) for args in more], *START_L[1], (gate_x, gate_m[0]), pin_m[1])
        shadow.add([partial(x_operands, j * MQ, r, kk, p)
                    for r in range(0, MQ, RG) for kk in range(2) for p in range(7)], *START_L[3], (gate_tu,), pin_xa)
        for c in range(4):
            t2_v[c % 2] = shadow.dot(cat(ha_v, 0, 4), wt(c * 8, 0, 512, F32), NT)
            y = shadow.dot(cat(ha_v, 4, 4), wt(c * 8, 512, 512, F32), NT) + t2_v[c % 2]
            for a in range(4):
                qkv_v[c, pl.ds(al(HIST + a * M + j * MQ, 8), MQ), :] = y[a * MQ:(a + 1) * MQ]
        shadow.finish()
        return 0

    def first_projection(n, _):
        wqkv_copy(n + 2).wait()
        pl.when(n < 3)(lambda: wqkv_copy(n + 3).start())
        pl.when(n < 3)(lambda: wo_copy(n - 1).start())
        wg_copy(n - 1).start()
        wu_copy(n - 1).start()
        shadow = _Shadow()
        transpose_slab(shadow, n + 2, range(NB), FIRST_T)
        project(shadow, n, tg_v, 0, K_T)
        shadow.finish()
        return 0

    def projection(n, _):
        def put(unit, d, v):
            wo_v[2 * DH * unit[0] + 2 * d + unit[2], :, _lanes(unit[1])] = v
        shadow = _Shadow()
        reorder(shadow, *PROJ_T, [(j, c, s) for j in range(2) for c in range(4) for s in range(2)],
                lambda unit, k: wa_v[6 + unit[0], _lanes(4 * unit[2] + k), _lanes(unit[1])].astype(F32),
                put, ((gate_wo,), (gate_tr,)), (pin_tr, pin_wo))
        project(shadow, 2 * n, tg_v, 0, K_Q)
        project(shadow, 2 * n + 1, tu_v, 1, K_Q)
        shadow.finish()
        return 0

    def gate_up(i, t, _):
        @pl.when(i == 0)
        def _():
            wg_copy(t).wait()
            wu_copy(t).wait()
        busy = [len(R_TERMS[p]) > 1 and k < 4 for p in ORDER for k in range(7)]
        shadow = _Shadow([ROOM_G[0] if busy[(n + ROOM_G[1]) % 49] else 1.0 for n in range(49)])
        shadow.add([partial(h_operands, jnp.maximum(t - 1, 0), r, p)
                    for p in (1, 5, 4, 0, 2, 6, 3) for r in range(0, M, RG)], *SPAN_H, (), pin_ha)
        base, ahead = [al(jnp.minimum(n * AROWS, TM - AROWS), 8) for n in (t, t + 1)]
        o = o_v.at[:, pl.ds(base, AROWS)]
        groups, pairs = range(AROWS // AG), [range(n, n + 2) for n in range(0, 8, 2)]
        shadow.add(windows(2 * NB, vw_v, NB, base), *SPAN_W[0], (), pin_vw)
        shadow.add(windows(0, qkw_v, 2 * NB, ahead), *SPAN_W[1], (), pin_qkw)
        shadow.add([partial(scores, n, ws) for n in groups for ws in pairs], *SPAN_A[0], (gate_qkw,), pin_s[0])
        shadow.add([partial(logits, i * TM + base + n * AG, n) for n in groups], *SPAN_A[1], gate_s[0:1], pin_s[1])
        shadow.add([partial(exponentials, n) for n in groups], *SPAN_A[2], gate_s[1:2], pin_s[2])
        shadow.add([partial(reciprocal, n) for n in groups], *SPAN_A[3], gate_s[2:3], pin_s[3])
        shadow.add([partial(mix, o, n, bs) for n in groups for bs in pairs], *SPAN_A[4],
                   (gate_s[2], gate_s[3], gate_vw), pin_o)

        def emit(r, c, v):
            hh_v[2 + 4 * r + c] = v[:, :128] * v[:, 128:]
        ops = _right_operands(lambda r, c, dtype: jnp.concatenate(
            [w_v[k * NQ + t, r * KQ:(r + 1) * KQ, _lanes(c)].astype(dtype) for k in range(2)], axis=1), b1_v, 0, K_G)
        _strassen2(lambda n: shadow.dot(cat(xa_v, 2 * n, 2), ops(n)), u2_v, u1_v, emit)
        shadow.finish()
        return 0

    def down(i, j, _):
        shadow = _Shadow()
        rows = [(jnp.minimum(i + 1, NTILE - 1), j * MH, a, r, n)
                for n, (a, r) in enumerate((a, r) for r in range(0, MH, RG) for a in range(4))]
        shadow.add([partial(row_mean, *args) for args in rows], *SPAN_L[0], (gate_x,), pin_m[0])
        shadow.add([partial(row_var, *args) for args in rows], *SPAN_L[1], (gate_x, gate_m[0]), pin_m[1])
        shadow.add([partial(normalize, *args) for args in rows], *SPAN_L[2], (gate_x, *gate_m), pin_tu)
        shadow.add([partial(x_operands, j * MH, r, kk, p)
                    for r in range(0, MH, RG) for kk in range(2) for p in range(7)], *SPAN_L[3], (gate_tu,), pin_xa)

        def weights(r, c, dtype):
            glu = wd_v[j, :, _lanes(r), _lanes(c)].astype(dtype).reshape(NQ * 128, 128)
            att = wo_v[pl.ds(2 * DH * j + r * 16, 16), :, _lanes(c)].astype(dtype).reshape(KQ, 128)
            return jnp.concatenate([att[128:], glu, att[:128]], axis=0)
        ops = _right_operands(weights, b1d_v, 0, K_D)

        def prod(n):
            p, q = divmod(n, 7)
            direct = lambda blk: _comb(L_TERMS[q], lambda r, c: _comb(
                L_TERMS[p], lambda a, b: blk(2 * a + r, 2 * b + c))).astype(BF16)
            att = [direct(lambda a, c: o_v[2 * c + kk, a * M:(a + 1) * M, :]) for kk in range(2)]
            glu = [packed(ha_v, n * (NQ - 1) + t) for t in range(NQ - 1)] + [direct(lambda a, c: hh_v[2 + 4 * a + c])]
            parts, b = [att[1], *glu, att[0]], ops(n)
            t3_v[0] = shadow.dot(jnp.concatenate(parts[:4], axis=1), b[:512])
            return shadow.dot(jnp.concatenate(parts[4:], axis=1), b[512:]) + t3_v[0]

        def emit(r, c, v):
            x = x_v[4 * i + r, :, pl.ds(al(j * 512 + c * 128, 128), 128)]
            out_v[2 * i + j, r, :, _lanes(c)] = (v + x.astype(F32)).astype(BF16)
            out_copy(i, j, r, c).start()
        _strassen2(prod, t2_v, tg_v, emit, True)
        shadow.finish()
        return 0

    def tile(i, _):
        @pl.when(i > 0)
        def _():
            qkv_v[NB:, :HIST, :] = qkv_v[NB:, TM:TM + HIST, :]
        lax.fori_loop(jnp.where(i == 0, 2, 0), 3, projection, 0)

        @pl.when(i == 0)
        def _():
            before_start(2 * NB)
            for cp in late_copies:
                cp.start()
        qkw_v[NB:2 * NB, :HIST, :] = qkv_v[NB:2 * NB, :HIST, :]
        lax.fori_loop(0, NQ, partial(gate_up, i), 0)

        @pl.when(i == 0)
        def _():
            for cp in late_copies:
                cp.wait()
        lax.fori_loop(0, 2, partial(down, i), 0)
        return 0

    x_copy(0).wait()
    wq_copy(2).start()
    for n, a, r in quarter:
        row_mean(0, 0, a, r, n)
        row_var(0, 0, a, r, n)
    lax.fori_loop(0, 4, first_weights, 0)
    lax.fori_loop(0, 4, first_rows, 0)
    qkw_v[:4, HIST:HIST + AROWS, :] = qkv_v[:4, HIST:HIST + AROWS, :]
    lax.fori_loop(1, 4, first_projection, 0)
    for s in range(2):
        wo_copy(s).wait()
    before_start(NB)
    for t in range(3, NQ):
        wg_copy(t).start()
        wu_copy(t).start()
    lax.fori_loop(0, NTILE, tile, 0)
    pltpu.make_async_copy(o_hbm, o_hbm, sems.at[NQ + 4]).wait()


@jax.jit
def pallas_parallel_sum__sliding_local_dilated__glu_gated_bilinear__prompt_kernel(
        A_x, A_wqkv, A_wo, B_x, B_w_gate, B_w_up, B_w_down):
    del B_x
    B, S, D = A_x.shape
    F = B_w_gate.shape[1]
    assert B == 1 and D == 1024 and S % TM == 0 and F == 7 * 512
    NB, NQ, M, NTILE = D // 128, F // 512, TM // 4, S // TM
    window = _attention_rows(NQ)
    V = pltpu.VMEM
    out = pl.pallas_call(
        _kernel,
        out_shape=jax.ShapeDtypeStruct((NTILE, 4, M, D), BF16),
        in_specs=[pl.BlockSpec(memory_space=pl.ANY)] * 6,
        out_specs=pl.BlockSpec(memory_space=pl.ANY),
        scratch_shapes=[
            V((4 * NTILE + 1, M, D), BF16),
            V((2 * NTILE, 4, M, 512), BF16),
            V((2 * NQ, D, 512), BF16),
            V((9, D, 512), BF16),
            V((6 * D // H + 1, 16, D), BF16),
            V((4 * D // H + 1, 16, 512), BF16),
            V((2, NQ, 512, 512), BF16),
            V((2 + STASH, 16 * PITCH, 128), F32),
            V((99, M, 128), BF16),
            V((49 * (NQ - 1) + 1, M, 128), BF16),
            V((3 * NB, TM + HIST, 128), F32),
            V((NB + 1, TM, 128), F32),
            V((18, M, 128), F32),
            V((5, M, 128), F32), V((2, M, 128), F32),
            V((20, M, 128), F32), V((21, M, 128), F32), V((5, M, 256), F32), V((20, M, 256), F32),
            V((8, D // 4, 256), F32), V((8, 128, D // 4), F32), V((8, NQ * 128 + D // 4, 128), F32),
            V((2 * NB + 1, window + HIST + PAD, 128), F32), V((NB + 1, window + HIST + PAD, 128), F32),
            *[V((2 + window // AG, n, AG, 128), F32) for n in (WIN, WIN + 1, WIN + 1, 1)],
            V((2 + TM // RG, RG, 128), F32), V((3 + TM // RG, RG, 128), F32),
            pltpu.SMEM((1,), jnp.int32),
            pltpu.SemaphoreType.DMA((NQ + 5,)),
        ],
        compiler_params=pltpu.CompilerParams(vmem_limit_bytes=126 << 20, disable_bounds_checks=True),
    )(A_x.reshape(NTILE, 4, M, D), A_wqkv, A_wo, B_w_gate, B_w_up, B_w_down.reshape(NQ, 512, D))
    return out.reshape(B, S, D)
```
